```python
import jax
import jax.numpy as jnp

def _softmax(x, axis=-1):
    return jax.nn.softmax(x, axis=axis)

def _gelu(x):
    return jax.nn.gelu(x, approximate=True)

def _silu(x):
    return jax.nn.silu(x)

def _sigmoid(x):
    return jax.nn.sigmoid(x)

def _layernorm(x, axis=-1, eps=1e-05):
    m = jnp.mean(x, axis=axis, keepdims=True)
    v = jnp.var(x, axis=axis, keepdims=True)
    return (x - m) / jnp.sqrt(v + eps)

def _scatter_add(tgt, idx, src, axis=0):
    return tgt.at[idx].add(src)

def _segment_sum(src, seg, n):
    return jax.ops.segment_sum(src, seg, n)

class _Rng:

    def __init__(self, key):
        self._k = key

    def _next(self):
        self._k, sub = jax.random.split(self._k)
        return sub

    def normal(self, shape):
        return jax.random.normal(self._next(), shape, dtype=jnp.bfloat16)

    def randint(self, lo, hi, shape):
        return jax.random.randint(self._next(), shape, lo, hi, dtype=jnp.int32)

    def uniform(self, shape, lo=0.0, hi=1.0):
        return jax.random.uniform(self._next(), shape, jnp.bfloat16, lo, hi)

    def permutation(self, n):
        return jax.random.permutation(self._next(), n)
kernel_name = 'parallel_sum__memory_aug_recurrent_mem_tr__mixer_s_mlp__prompt'

def setup_inputs():
    _rng = _Rng(jax.random.key(int.from_bytes(__import__("os").urandom(4), "little")))
    _w = lambda a: (lambda t: t.astype(jnp.bfloat16) if jnp.issubdtype(t.dtype, jnp.floating) else t)(jnp.asarray(a))

    def _A_setup():
        B, S, Dm = (1, 2048, 1024)
        H, Dh = (32, 128)
        M, seg = (8, 32)
        seg = min(seg, S)
        S = S // seg * seg
        return {'x': _w((lambda *s: _rng.normal(s) * 0.05)(B, S, Dm)), 'mem0': _w((lambda *s: _rng.normal(s) * 0.05)(B, M, Dm)), 'Wq': _w((lambda *s: _rng.normal(s) * 0.05)(Dm, H, Dh) * Dm ** (-0.5)), 'Wk': _w((lambda *s: _rng.normal(s) * 0.05)(Dm, H, Dh) * Dm ** (-0.5)), 'Wv': _w((lambda *s: _rng.normal(s) * 0.05)(Dm, H, Dh) * Dm ** (-0.5)), 'Wo': _w((lambda *s: _rng.normal(s) * 0.05)(H, Dh, Dm) * (H * Dh) ** (-0.5)), 'seg_len': seg}
    _A_in = _A_setup()

    def _B_setup():
        B, S, D, F = (1, 2048, 1024, 3584)
        return {'x': _w((lambda *s: _rng.normal(s) * 0.05)(B, S, D)), 'w1': _w((lambda *s: _rng.normal(s) * 0.05)(D, D) * D ** (-0.5)), 'w2': _w((lambda *s: _rng.normal(s) * 0.05)(D, D) * D ** (-0.5)), 'w3': _w((lambda *s: _rng.normal(s) * 0.05)(D, F) * D ** (-0.5)), 'w4': _w((lambda *s: _rng.normal(s) * 0.05)(F, D) * F ** (-0.5))}
    _B_in = _B_setup()
    return {'A_x': _A_in['x'], 'A_mem0': _A_in['mem0'], 'A_Wq': _A_in['Wq'], 'A_Wk': _A_in['Wk'], 'A_Wv': _A_in['Wv'], 'A_Wo': _A_in['Wo'], 'A_seg_len': _A_in['seg_len'], 'B_x': _B_in['x'], 'B_w1': _B_in['w1'], 'B_w2': _B_in['w2'], 'B_w3': _B_in['w3'], 'B_w4': _B_in['w4']}

def reference(A_x, A_mem0, A_Wq, A_Wk, A_Wv, A_Wo, A_seg_len, B_x, B_w1, B_w2, B_w3, B_w4):

    def _A_ref(x, mem0, Wq, Wk, Wv, Wo, seg_len):
        B, S, Dm = x.shape
        H, Dh = (Wq.shape[1], Wq.shape[2])
        M = mem0.shape[1]
        scale = Dh ** (-0.5)
        n_seg = S // seg_len
        L = M + seg_len
        idx = jnp.arange(L)
        mask = (idx[:, None] < M) | (idx[:, None] >= idx[None, :])
        mem = mem0
        outs = []
        for s in range(n_seg):
            xs = x[:, s * seg_len:(s + 1) * seg_len, :].copy()
            h = jnp.concatenate([mem, xs], axis=1)
            q = jnp.einsum('btd,dhe->bhte', h, Wq)
            k = jnp.einsum('btd,dhe->bhte', h, Wk)
            v = jnp.einsum('btd,dhe->bhte', h, Wv)
            scores = jnp.einsum('bhqe,bhke->bhqk', q, k) * scale
            scores = jnp.where(mask[None, None], scores, -1000000000.0)
            p = _softmax(scores, axis=-1)
            o = jnp.einsum('bhqk,bhke->bhqe', p, v)
            o = jnp.einsum('bhte,hed->btd', o, Wo)
            mem = o[:, :M, :].copy()
            outs.append(o[:, M:, :])
        return jnp.concatenate(outs, axis=1)

    def _B_ref(x, w1, w2, w3, w4):
        B, S, D = x.shape
        h = _gelu(_layernorm(x, axis=-1) @ w1)
        c = D // 4
        g0 = jnp.pad(h[:, :, 0 * c:1 * c], ((0, 0), (1, 0), (0, 0)))[:, :S, :]
        g1 = jnp.pad(h[:, :, 1 * c:2 * c], ((0, 0), (0, 1), (0, 0)))[:, 1:, :]
        g2 = jnp.pad(h[:, :, 2 * c:3 * c], ((0, 0), (2, 0), (0, 0)))[:, :S, :]
        g3 = jnp.pad(h[:, :, 3 * c:], ((0, 0), (0, 2), (0, 0)))[:, 2:, :]
        hs = jnp.concatenate([g0, g1, g2, g3], axis=-1) @ w2
        x1 = x + hs
        h2 = _gelu(_layernorm(x1, axis=-1) @ w3) @ w4
        return x1 + h2
    x = A_x
    xn = _layernorm(x, axis=-1)
    return x + _A_ref(xn, A_mem0, A_Wq, A_Wk, A_Wv, A_Wo, A_seg_len) + _B_ref(xn, B_w1, B_w2, B_w3, B_w4)
```

```python
import functools

import jax
import jax.numpy as jnp
from jax import lax
from jax.experimental import pallas as pl
from jax.experimental.pallas import tpu as pltpu

F32 = jnp.float32
BF16 = jnp.bfloat16
U32 = jnp.uint32
LANES = 128
SUB = 8
EPS = 1e-5
TM = 256
FC = 512
HG = 4


def _layernorm(x):
    m = jnp.mean(x, axis=-1, keepdims=True)
    d = x - m
    v = jnp.mean(d * d, axis=-1, keepdims=True)
    return d * lax.rsqrt(v + EPS)


def _gelu(x):
    return jax.nn.gelu(x, approximate=True)


def _dot(a, b):
    return jnp.dot(a, b, preferred_element_type=F32)


def _kernel(
    x_hbm, mem_ref, wq_hbm, wk_hbm, wv_hbm, wo_hbm, w1_hbm, w2_hbm, w3_hbm, w4_hbm,
    out_hbm,
    xb, xn, hb, yb, base, w1, w2, w3, w4, raw, raw_o, wqkv, wo,
    sem_x, sem_w, sem_raw, sem_out,
    *, S, D, H, DH, M, SEG, F,
):
    NT = S // TM
    NCB = D // LANES
    HP = S + 2 * SUB
    PITCH = D // 2 + 1
    DCH = D // NT
    OCH = H * DH // NT
    NF = F // FC

    def x_copy(i):
        rows = pl.ds(i * TM, TM)
        return pltpu.make_async_copy(x_hbm.at[rows], xb.at[rows], sem_x.at[i])

    w1_copy = pltpu.make_async_copy(w1_hbm, w1, sem_w.at[0])
    w2_copy = pltpu.make_async_copy(w2_hbm, w2, sem_w.at[1])
    w3_copy = pltpu.make_async_copy(w3_hbm, w3, sem_w.at[2])
    w4_copy = pltpu.make_async_copy(w4_hbm, w4, sem_w.at[3])

    def raw_copies(i, slot):
        r0 = pl.multiple_of(i * (DCH * H), DCH * H)
        o0 = pl.multiple_of(i * OCH, OCH)
        cps = [
            pltpu.make_async_copy(w.at[pl.ds(r0, DCH * H)], raw.at[slot, j], sem_raw.at[slot, j])
            for j, w in enumerate((wq_hbm, wk_hbm, wv_hbm))
        ]
        cps.append(pltpu.make_async_copy(wo_hbm.at[pl.ds(o0, OCH)], raw_o.at[slot], sem_raw.at[slot, 3]))
        return cps

    x_copy(0).start()
    w1_copy.start()
    for i in range(1, NT):
        x_copy(i).start()
    w2_copy.start()

    for c in range(NCB):
        hb[pl.ds(c * HP, SUB), :] = jnp.zeros((SUB, LANES), F32)
        hb[pl.ds(c * HP + SUB + S, SUB), :] = jnp.zeros((SUB, LANES), F32)

    def norm_tile(i):
        rows = pl.ds(pl.multiple_of(i * TM, TM), TM)
        n = _layernorm(xb[rows, :].astype(F32))
        xn[rows, :] = n
        yb[rows, :] = _layernorm(n).astype(BF16)

    def stage1(i):
        r0 = pl.multiple_of(i * TM, TM)
        h = _gelu(_dot(yb[pl.ds(r0, TM), :], w1[...]))
        for c in range(NCB):
            hb[pl.ds(c * HP + SUB + r0, TM), :] = h[:, c * LANES:(c + 1) * LANES]

    x_copy(0).wait()
    norm_tile(0)
    w1_copy.wait()
    w3_copy.start()
    w4_copy.start()

    def p1(i, carry):
        x_copy(i + 1).wait()
        stage1(i)
        norm_tile(i + 1)
        return carry

    lax.fori_loop(0, NT - 1, p1, 0)

    shifts = (-1, 1, -2, 2)

    def stage2(i):
        r0 = pl.multiple_of(i * TM, TM)
        rows = pl.ds(r0, TM)
        g = jnp.concatenate(
            [hb[pl.ds(c * HP + SUB + shifts[c * 4 // NCB] + r0, TM), :] for c in range(NCB)], axis=1)
        x1 = xn[rows, :] + _dot(g.astype(BF16), w2[...])
        yb[rows, :] = _layernorm(x1).astype(BF16)
        base[rows, :] = x1 + xb[rows, :].astype(F32)

    def stage3(i):
        rows = pl.ds(pl.multiple_of(i * TM, TM), TM)
        y = yb[rows, :]
        g = jnp.concatenate(
            [_gelu(_dot(y, w3[:, f * FC:(f + 1) * FC])).astype(BF16) for f in range(NF)], axis=1)
        base[rows, :] += _dot(g, w4[...])

    def relayout(i, slot):
        j0 = i * (DCH // 2)
        for w in range(3):
            for j in range(DCH // 2):
                for half in range(H // 16):
                    ev = pltpu.bitcast(raw[slot, w, pl.ds((2 * j) * H + half * 16, 16), :], U32)
                    od = pltpu.bitcast(raw[slot, w, pl.ds((2 * j + 1) * H + half * 16, 16), :], U32)
                    lo = (ev & 0xFFFF) | (od << 16)
                    hi = (ev >> 16) | (od & jnp.uint32(0xFFFF0000))
                    s_lo = w * H + half * SUB
                    s_hi = s_lo + H // 2
                    wqkv[pl.ds(s_lo * PITCH + j + j0, SUB, stride=PITCH), :] = lo
                    wqkv[pl.ds(s_hi * PITCH + j + j0, SUB, stride=PITCH), :] = hi
        o0 = pl.multiple_of(i * (OCH // 2), OCH // 2)
        for c in range(NCB):
            wo[c, pl.ds(o0, OCH // 2), :] = pltpu.bitcast(raw_o[slot, :, c * LANES:(c + 1) * LANES], U32)

    for cp in raw_copies(0, 0):
        cp.start()
    w2_copy.wait()
    stage1(NT - 1)
    stage2(0)
    w3_copy.wait()
    w4_copy.wait()

    def p3(i, carry):
        slot = i % 2
        for cp in raw_copies(i + 1, 1 - slot):
            cp.start()
        for cp in raw_copies(i, slot):
            cp.wait()
        stage3(i)
        stage2(i + 1)
        relayout(i, slot)
        return carry

    lax.fori_loop(0, NT - 1, p3, 0)
    for cp in raw_copies(NT - 1, (NT - 1) % 2):
        cp.wait()
    stage3(NT - 1)
    relayout(NT - 1, (NT - 1) % 2)

    L = M + SEG
    row = lax.broadcasted_iota(jnp.int32, (L, L), 0)
    col = lax.broadcasted_iota(jnp.int32, (L, L), 1)
    mask = (row < M) | (row >= col)
    scale = DH ** -0.5

    def w_in(w, head):
        slot = w * H + (head % 2) * (H // 2) + head // 2
        return pltpu.bitcast(wqkv[pl.ds(slot * PITCH, D // 2), :], BF16)

    def w_out(c, h0):
        return pltpu.bitcast(wo[c, pl.ds(h0 * DH // 2, HG * DH // 2), :], BF16)

    def segment(s, mem):
        rows = pl.ds(pl.multiple_of(s * SEG, SEG), SEG)
        h = jnp.concatenate([mem, xn[rows, :]], axis=0)
        qkv, prob, att = {}, {}, {}
        acc = None

        def project(i):
            r = _dot(h, jnp.concatenate([w_in(0, i), w_in(1, i), w_in(2, i)], axis=1))
            qkv[i] = (r[:, :DH], r[:, DH:2 * DH], r[:, 2 * DH:])

        def scores(i):
            q, k, _ = qkv[i]
            z = lax.dot_general(q, k, (((1,), (1,)), ((), ())), preferred_element_type=F32)
            z = jnp.where(mask, z * scale, -1e9)
            e = jnp.exp(z - jnp.max(z, axis=-1, keepdims=True))
            prob[i] = (e, 1.0 / jnp.sum(e, axis=-1, keepdims=True))

        def attend(i):
            e, inv = prob[i]
            att[i] = _dot(e, qkv[i][2]) * inv

        ng = H // HG
        for t in range(ng + 3):
            for j in range(HG):
                if t < ng:
                    project(t * HG + j)
                if 0 <= t - 1 < ng:
                    scores((t - 1) * HG + j)
                if 0 <= t - 2 < ng:
                    attend((t - 2) * HG + j)
            if 0 <= t - 3 < ng:
                g = t - 3
                o = jnp.concatenate([att[g * HG + j] for j in range(HG)], axis=1)
                r = _dot(o, jnp.concatenate([w_out(c, g * HG) for c in range(NCB)], axis=1))
                acc = r if acc is None else acc + r
        xb[rows, :] = (base[rows, :] + acc[M:]).astype(BF16)
        pltpu.make_async_copy(xb.at[rows], out_hbm.at[rows], sem_out).start()
        return acc[:M]

    lax.fori_loop(0, S // SEG, segment, mem_ref[...].astype(F32))
    pltpu.make_async_copy(xb, out_hbm, sem_out).wait()


@functools.partial(jax.jit, static_argnames=("A_seg_len",))
def pallas_parallel_sum__memory_aug_recurrent_mem_tr__mixer_s_mlp__prompt_kernel(
    A_x: jax.Array,
    A_mem0: jax.Array,
    A_Wq: jax.Array,
    A_Wk: jax.Array,
    A_Wv: jax.Array,
    A_Wo: jax.Array,
    A_seg_len: int,
    B_x: jax.Array,
    B_w1: jax.Array,
    B_w2: jax.Array,
    B_w3: jax.Array,
    B_w4: jax.Array,
):
    del B_x
    B, S, D = A_x.shape
    _, H, DH = A_Wq.shape
    M = A_mem0.shape[1]
    F = B_w3.shape[1]
    SEG = int(A_seg_len)
    assert B == 1 and DH == LANES and S % TM == 0 and S % SEG == 0
    NT = S // TM
    pitch = D // 2 + 1

    hbm = pl.BlockSpec(memory_space=pl.ANY)
    out = pl.pallas_call(
        functools.partial(_kernel, S=S, D=D, H=H, DH=DH, M=M, SEG=SEG, F=F),
        out_shape=jax.ShapeDtypeStruct((S, D), A_x.dtype),
        in_specs=[hbm, pl.BlockSpec(memory_space=pltpu.VMEM)] + [hbm] * 8,
        out_specs=hbm,
        scratch_shapes=[
            pltpu.VMEM((S, D), BF16),
            pltpu.VMEM((S, D), F32),
            pltpu.VMEM((D // LANES * (S + 2 * SUB), LANES), F32),
            pltpu.VMEM((S, D), BF16),
            pltpu.VMEM((S, D), F32),
            pltpu.VMEM((D, D), BF16),
            pltpu.VMEM((D, D), BF16),
            pltpu.VMEM((D, F), BF16),
            pltpu.VMEM((F, D), BF16),
            pltpu.VMEM((2, 3, D // NT * H, LANES), BF16),
            pltpu.VMEM((2, H * DH // NT, D), BF16),
            pltpu.VMEM((-(-3 * H * pitch // SUB) * SUB, LANES), U32),
            pltpu.VMEM((D // LANES, H * DH // 2, LANES), U32),
            pltpu.SemaphoreType.DMA((NT,)),
            pltpu.SemaphoreType.DMA((4,)),
            pltpu.SemaphoreType.DMA((2, 4)),
            pltpu.SemaphoreType.DMA(()),
        ],
        compiler_params=pltpu.CompilerParams(vmem_limit_bytes=120 * 1024 * 1024),
    )(
        A_x.reshape(S, D),
        A_mem0.reshape(M, D),
        A_Wq.reshape(D * H, DH),
        A_Wk.reshape(D * H, DH),
        A_Wv.reshape(D * H, DH),
        A_Wo.reshape(H * DH, D),
        B_w1, B_w2, B_w3, B_w4,
    )
    return out.reshape(B, S, D)
```

```python
import contextlib
import functools
import itertools

import jax
import jax.numpy as jnp
from jax import lax
from jax.experimental import pallas as pl
from jax.experimental.pallas import tpu as pltpu

F32 = jnp.float32
BF16 = jnp.bfloat16
U32 = jnp.uint32
LANES = 128
SUB = 8
EPS = 1e-5
R1 = 128
R3 = 256
FC = 512
NORM = 16
NORM3 = 32
KB = 64
PG = 4
PERIOD = 3
TAIL = (2, 4, 2)
SCOPES = False
PARTS = "13A"
FLAGS = None


def _scope(name):
    return jax.named_scope(name) if SCOPES else contextlib.nullcontext()


def _layernorm(x):
    m = jnp.mean(x, axis=-1, keepdims=True)
    d = x - m
    v = jnp.mean(d * d, axis=-1, keepdims=True)
    return d * lax.rsqrt(v + EPS)


def _gelu(x):
    return jax.nn.gelu(x, approximate=True)


def _softmax_rows(q, k, mask, scale):
    z = lax.dot_general(q, k, (((1,), (1,)), ((), ())), preferred_element_type=F32)
    z = jnp.where(mask, z * scale, -1e9)
    e = jnp.exp(z - jnp.max(z, axis=-1, keepdims=True))
    s = jnp.sum(e, axis=-1, keepdims=True)
    r = pl.reciprocal(s, approx=True)
    return e * (r * (2.0 - s * r))


def _dot(a, b):
    return jnp.dot(a, b, preferred_element_type=F32)


def _put(ref, idx, v):
    ref[idx] = pltpu.bitcast(v.astype(BF16), U32)


def _get(ref, idx):
    return pltpu.bitcast(ref[idx], BF16)


def _words(*shape):
    return pltpu.VMEM(shape + (LANES,), U32)


def _lanes(v, c):
    return v[:, c * LANES:(c + 1) * LANES]


_LHS = (((0, 0), (1, 1), 1), ((1, 0), (1, 1), 1), ((0, 0),), ((1, 1),),
        ((0, 0), (0, 1), 1), ((1, 0), (0, 0), -1), ((0, 1), (1, 1), -1))
_RHS = (((0, 0), (1, 1), 1), ((0, 0),), ((0, 1), (1, 1), -1), ((1, 0), (0, 0), -1),
        ((1, 1),), ((0, 0), (0, 1), 1), ((1, 0), (1, 1), 1))
_OUT = (((0, 1), (3, 1)), ((2, 1), (3, -1)), ((1, 1), (3, 1)), ((0, 1), (2, 1)),
        ((0, -1), (1, 1)), ((3, 1),), ((0, 1),))
_ORDER = (0, 3, 1, 2, 4, 5, 6)


def _operand(terms, block):
    if len(terms) == 1:
        return block(*terms[0])
    u, v = block(*terms[0]), block(*terms[1])
    return u + v if terms[2] > 0 else u - v


def _operands(table, blocks):
    return [_operand(terms, lambda a, b: blocks[2 * a + b]) for terms in table]


def _fold(c, i, m):
    for k, sign in _OUT[i]:
        if c[k] is None:
            c[k] = m if sign > 0 else -m
        else:
            c[k] = c[k] + m if sign > 0 else c[k] - m


def _load7(ref, i, rows=slice(None)):
    return jnp.concatenate([_get(ref, (i, c, rows)) for c in range(ref.shape[1])], axis=1)


_ALL, _LO, _HI = (0, 2), (0, 1), (1, 1)
_STEP_PRODUCTS = (
    ((0, _ALL), (1, _LO), (2, _LO), (3, _LO)),
    ((1, _HI), (3, _HI), (5, _LO), (6, _LO)),
    ((4, _ALL), (2, _HI), (5, _HI), (6, _HI)),
)


def _mem_lhs(m1, m2):
    s = m1 + m2
    return (s, s, m1, m2, s, m1, m2)


def _mem_out(step, m):
    if step == 0:
        return m[1] + m[3], m[2] + m[0] - m[1]
    if step == 1:
        c1 = m[1] + m[3]
        return c1, m[5] + m[6] - c1
    c2 = m[2] + m[4]
    return m[5] + m[6] - c2, c2


def _token_out(step, m, ld, st):
    if step == 0:
        q = m[1].shape[0]
        lo, hi = m[0][:q], m[0][q:]
        st(0, 0, 0, lo + m[3])
        st(0, 1, 0, m[2])
        st(1, 0, 0, m[1] + m[3])
        st(1, 1, 0, lo - m[1] + m[2])
        st(0, 0, 1, hi)
    elif step == 1:
        st(0, 0, 0, ld(0, 0, 0) + m[6])
        st(1, 1, 0, ld(1, 1, 0) + m[5])
        t = ld(0, 0, 1)
        st(0, 0, 1, t + m[3])
        st(1, 0, 1, m[1] + m[3])
        st(1, 1, 1, t - m[1])
    else:
        q = m[2].shape[0]
        lo, hi = m[4][:q], m[4][q:]
        st(0, 0, 0, ld(0, 0, 0) - lo)
        st(0, 1, 0, ld(0, 1, 0) + lo)
        st(0, 0, 1, ld(0, 0, 1) + m[6] - hi)
        st(0, 1, 1, m[2] + hi)
        st(1, 1, 1, ld(1, 1, 1) + m[2] + m[5])


def _share(jobs, k, n):
    return jobs[len(jobs) * k // n:len(jobs) * (k + 1) // n]


def _mix(*lists):
    keyed = [((n + 0.5) / len(l), k, n) for k, l in enumerate(lists) for n in range(len(l))]
    return [lists[k][n] for _, k, n in sorted(keyed)]


def _jobs(fn, *ranges):
    return [functools.partial(fn, *k) for k in itertools.product(*ranges)]


def _run(jobs):
    for job in jobs:
        job(lambda v: v)


def _never(ref):
    return jnp.abs(ref[0:SUB, 0:LANES].astype(F32)) < 0.0


def _paced_dot(a, b, side, never):
    m = _dot(a, b)
    rounds = max(a.shape[1] * m.shape[1] // (4 * LANES * LANES), 1)
    tokens = [
        m[r:r + SUB, c:c + LANES]
        for c in range(0, m.shape[1], m.shape[1] // rounds) for r in range(0, m.shape[0], SUB)
    ]

    def gate(mine, v):
        n = v.shape[0] // SUB
        rows = []
        for r in range(n):
            t = lax.bitcast_convert_type(tokens[mine[0] + (mine[1] - mine[0]) * r // n], v.dtype)
            rows.append(jnp.concatenate([
                jnp.where(never, t, v[r * SUB:(r + 1) * SUB, c:c + LANES])
                for c in range(0, v.shape[1], LANES)], axis=1))
        return jnp.concatenate(rows, axis=0)

    for n, job in enumerate(side):
        job(functools.partial(gate, (len(tokens) * n // len(side), len(tokens) * (n + 1) // len(side))))
    return m


def _strassen(lhs, w, side, never, order=_ORDER):
    c = [None] * 4
    for n, i in enumerate(order):
        _fold(c, i, _paced_dot(lhs(i), _load7(w, i), _share(side, n, 7), never))
    return c


def _lhs_from(block):
    return lambda i: _operand(_LHS[i], block).astype(BF16)


def _rhs_jobs(dst, src, kh, nh, which=range(7)):
    def job(c, k0, gate):
        @functools.cache
        def block(a, b):
            return gate(src(pl.ds(a * kh + k0, KB), pl.ds(b * nh + c * LANES, LANES)).astype(F32))

        for i in which:
            _put(dst, (i, c, pl.ds(k0 // 2, KB // 2)), _operand(_RHS[i], block))

    return _jobs(job, range(nh // LANES), range(0, kh, KB))


def _kernel(
    x_hbm, mem_hbm, wq_hbm, wk_hbm, wv_hbm, wo_hbm, w1_hbm, w2_hbm, w3_hbm, w4_hbm,
    out_hbm,
    xb, xn, base, wqkv, yc, w3c, r3, r4, raw, mid, raw_o, mem0, sem_f, sem_a, sem_m,
    *, S, D, H, DH, M, SEG, F,
):
    HD = D // 2
    NCB = D // LANES
    NP = H // 2
    T1 = 2 * R1
    NT = S // T1
    NF = F // FC
    NPART = NF + 1
    DP = HD // NPART
    OP = NP // NPART

    def w3_copy(f):
        cols = pl.ds(pl.multiple_of(f * FC, FC), FC)
        return pltpu.make_async_copy(w3_hbm.at[:, cols], r3.at[f % 2], sem_f.at[0, f % 2])

    def w4_copy(f):
        rows = pl.ds(pl.multiple_of(f * FC, FC), FC)
        return pltpu.make_async_copy(w4_hbm.at[rows], r4.at[f % 2], sem_f.at[1, f % 2])

    def qkv_copies(part):
        return [
            pltpu.make_async_copy(
                w.at[pl.ds(pl.multiple_of((a * HD + part * DP) * H, DP * H), DP * H)],
                raw.at[part % 2, 2 * j + a], sem_a.at[part % 2, 2 * j + a])
            for j, w in enumerate((wq_hbm, wk_hbm, wv_hbm)) for a in range(2)
        ]

    def wo_copy(part):
        rows = pl.ds(pl.multiple_of(part * (2 * OP * DH), 2 * OP * DH), 2 * OP * DH)
        return pltpu.make_async_copy(wo_hbm.at[rows], raw_o.at[part % 2], sem_a.at[part % 2, 6])

    mem_copy = pltpu.make_async_copy(mem_hbm, mem0, sem_m)

    def qkv_jobs(part):
        def transpose(j, a, g, gate):
            rows = gate(jnp.concatenate([
                pltpu.bitcast(raw[part % 2, 2 * j + a, pl.ds(d * H + g * 16, 16), :], U32)
                for d in range(DP)], axis=0))
            for d in range(DP):
                mid[2 * j + a, pl.ds(g * SUB * (DP + 1) + d, SUB, stride=DP + 1), :] = rows[d * SUB:(d + 1) * SUB]

        def combine(j, p, gate):
            blocks = []
            for a in range(2):
                v = gate(mid[2 * j + a, pl.ds(p * (DP + 1), DP), :])
                blocks.append(pltpu.bitcast(v << 16, F32))
                blocks.append(pltpu.bitcast(v & jnp.uint32(0xFFFF0000), F32))
            k0 = pl.multiple_of(part * (DP // 2), DP // 2)
            for i, v in enumerate(_operands(_RHS, blocks)):
                _put(wqkv, (i, j, p, pl.ds(k0, DP // 2)), v)

        tr = [_jobs(transpose, [j], range(2), range(NP // SUB)) for j in range(3)]
        cb = [_jobs(combine, [j], range(NP)) for j in range(3)]
        return tr[0] + _mix(tr[1], cb[0]) + _mix(tr[2], cb[1]) + cb[2]

    def wo_jobs(wo, part):
        def combine(j, c, k, gate):
            blocks = [
                gate(raw_o[part % 2, pl.ds((2 * j + a) * DH + k, KB), pl.ds(b * HD + c * LANES, LANES)].astype(F32))
                for a in range(2) for b in range(2)
            ]
            k0 = pl.multiple_of(((part * OP + j) * DH + k) // 2, KB // 2)
            for i, v in enumerate(_operands(_RHS, blocks)):
                _put(wo, (i, c, pl.ds(k0, KB // 2)), v)

        return _jobs(combine, range(OP), range(HD // LANES), range(0, DH, KB))

    def token_mixing(r12, w1c, w2c, y0, c1, c2, hb, sem_x, sem_w):
        shifts = (-1, 1, -2, 2)
        pieces = range(0, R1, NORM)

        def x_copy(t):
            rows = pl.ds(pl.multiple_of(t * T1, T1), T1)
            return pltpu.make_async_copy(x_hbm.at[rows], xb.at[rows], sem_x.at[t])

        def w1_copy(a, b):
            idx = (pl.ds(a * HD, HD), pl.ds(b * HD, HD))
            return pltpu.make_async_copy(w1_hbm.at[idx], r12.at[(0,) + idx], sem_w.at[2 * a + b])

        w2_copy = pltpu.make_async_copy(w2_hbm, r12.at[1], sem_w.at[4])

        def tile_rows(t, a, lo):
            return pl.ds(pl.multiple_of(t * T1 + a * R1 + lo, NORM), NORM)

        def normalizing(t, slot):
            def job(lo, a, gate):
                rows = tile_rows(t, a, lo)
                n = _layernorm(gate(xb[rows, :].astype(F32)))
                xn[rows, :] = n.astype(BF16)
                base[rows, :] = n
                y0[slot, a, pl.ds(lo, NORM), :] = _layernorm(n)

            return _jobs(job, pieces, range(2))

        def keep(dst, c):
            for k, v in enumerate(c):
                dst[k // 2, :, pl.ds(k % 2 * HD, HD)] = v

        def lhs1(slot):
            return _lhs_from(lambda a, b: y0[slot, a, :, pl.ds(b * HD, HD)])

        def stage1(slot, side):
            keep(c1, _strassen(lhs1(slot), w1c, side, never))

        def activating(t):
            def job(a, c, gate):
                hb[c, pl.ds(SUB + t * T1 + a * R1, R1), :] = _gelu(gate(c1[a, :, pl.ds(c * LANES, LANES)]))

            return _jobs(job, range(2), range(NCB))

        def stage2(t, side):
            keep(c2, _strassen(_lhs_from(lambda a, b: jnp.concatenate([
                hb[c, pl.ds(SUB + t * T1 + a * R1 + shifts[c * 4 // NCB], R1), :]
                for c in range(b * NCB // 2, (b + 1) * NCB // 2)], axis=1)), w2c, side, never))

        def renormalizing(t):
            def job(lo, gate):
                ys = []
                for a in range(2):
                    rows = tile_rows(t, a, lo)
                    x1 = base[rows, :] + gate(c2[a, pl.ds(lo, NORM), :])
                    base[rows, :] = x1 + xb[rows, :].astype(F32)
                    y = _layernorm(x1)
                    ys += [y[:, :HD], y[:, HD:]]
                half = pl.multiple_of((t * R1 + lo) // 2, NORM // 2)
                for i, v in enumerate(_operands(_LHS, ys)):
                    for c in range(NCB // 2):
                        _put(yc, (i, c, pl.ds(half, NORM // 2)), _lanes(v, c))

            return _jobs(job, pieces)

        arrival = (((0, 0), (1,)), ((1, 1), (4, 0)), ((0, 1), (2, 5)), ((1, 0), (3, 6)))
        for cp in [x_copy(0)] + [w1_copy(*q) for q, _ in arrival] + [x_copy(1), x_copy(2), w2_copy]:
            cp.start()
        for c in range(NCB):
            hb[c, pl.ds(0, SUB), :] = jnp.zeros((SUB, LANES), F32)
            hb[c, pl.ds(SUB + S, SUB), :] = jnp.zeros((SUB, LANES), F32)
        pad = xn.shape[0] - S
        xn[pl.ds(S, pad), :] = jnp.zeros((pad, D), BF16)
        with _scope("wait_x0"):
            x_copy(0).wait()
        never = _never(xb)
        with _scope("tile0"):
            _run(normalizing(0, 1))
            c = [None] * 4
            for q, ready in arrival:
                w1_copy(*q).wait()
                _run(_rhs_jobs(w1c, lambda r, k: r12[0, r, k], HD, HD, ready))
                for i in ready:
                    _fold(c, i, _dot(lhs1(1)(i), _load7(w1c, i)))
            keep(c1, c)
            x_copy(1).wait()
            _run(normalizing(1, 0))
        with _scope("tile1"):
            for t in range(3, NT):
                x_copy(t).start()
            x_copy(2).wait()
            stage1(0, _mix(activating(0), normalizing(2, 1)))
            for cp in [w3_copy(0)] + qkv_copies(0) + [w3_copy(1), w4_copy(0), wo_copy(0)] + qkv_copies(1):
                cp.start()
            mem_copy.start()
            w2_copy.wait()
            x_copy(3).wait()
            stage1(1, _mix(activating(1), _rhs_jobs(w2c, lambda r, k: r12[1, r, k], HD, HD)))
            stage2(0, normalizing(3, 0))

        def slot(u, carry):
            x_copy(u + 1).wait()
            with _scope("slot"):
                stage1(0, _mix(activating(u - 1), renormalizing(u - 3)))
                stage2(u - 2, normalizing(u + 1, 0))
            return carry

        lax.fori_loop(3, NT - 1, slot, 0)
        for cp in [w3_copy(0)] + qkv_copies(0):
            cp.wait()
        late = _rhs_jobs(w3c, lambda r, k: r3[0, r, k], HD, FC // 2) + qkv_jobs(0)
        with _scope("tile7"):
            stage1(0, _mix(activating(NT - 2), renormalizing(NT - 4)))
            stage2(NT - 3, _mix(activating(NT - 1), _share(late, 0, 3)))
            stage2(NT - 2, _mix(renormalizing(NT - 3), _share(late, 1, 3)))
            stage2(NT - 1, _mix(renormalizing(NT - 2), _share(late, 2, 3)))
            _run(renormalizing(NT - 1))

    def ffn(wo, w4c, g):
        N3 = S // 2 // R3
        never = _never(xb)

        def chunk(f, carry):
            @pl.when(f + 2 < NF)
            def _():
                w3_copy(f + 2).start()

            @pl.when(f + 1 < NF)
            def _():
                w4_copy(f + 1).start()
                for cp in qkv_copies(f + 2):
                    cp.start()
                w3_copy(f + 1).wait()

            wo_copy(f + 1).start()
            for cp in qkv_copies(f + 1) + [w4_copy(f), wo_copy(f)]:
                cp.wait()
            pre, post = {}, {}

            def up(t, side):
                pre[t] = _strassen(lambda i: _load7(yc, i, pl.ds(t * R3 // 2, R3 // 2)), w3c, side, never)

            def activate(t, lo, gate):
                for k, v in enumerate(pre[t]):
                    g[t % 2, k // 2, pl.ds(lo, NORM3), pl.ds(k % 2 * FC // 2, FC // 2)] = _gelu(gate(v[lo:lo + NORM3]))

            def down(t, side):
                post[t] = _strassen(
                    _lhs_from(lambda a, b: g[t % 2, a, :, pl.ds(b * FC // 2, FC // 2)]), w4c, side, never)

            def accumulate(t, lo, gate):
                j, r = divmod(t * R3 + lo, R1)
                for k, v in enumerate(post[t]):
                    base[pl.ds(j * T1 + k // 2 * R1 + r, NORM3), pl.ds(k % 2 * HD, HD)] += gate(v[lo:lo + NORM3])

            def rows_of(fn, t):
                return _jobs(fn, [t], range(0, R3, NORM3))

            side = _mix(qkv_jobs(f + 1), wo_jobs(wo, f))
            with _scope("chunk"):
                up(0, _rhs_jobs(w4c, lambda r, k: r4[f % 2, r, k], FC // 2, HD))
                up(1, rows_of(activate, 0))
                for t in range(N3 - 2):
                    down(t, rows_of(activate, t + 1))
                    up(t + 2, _mix(rows_of(accumulate, t), _share(side, t, N3 - 1)))
                down(N3 - 2, _mix(
                    rows_of(activate, N3 - 1), _rhs_jobs(w3c, lambda r, k: r3[(f + 1) % 2, r, k], HD, FC // 2)))
                down(N3 - 1, _mix(rows_of(accumulate, N3 - 2), _share(side, N3 - 2, N3 - 1)))
                _run(rows_of(accumulate, N3 - 1))
            return carry

        lax.fori_loop(0, NF, chunk, 0)

    def recurrence(wo, xc, gq, fq, ob, oc, go, sem_out):
        NG = NP // PG
        L = M + SEG
        PR = PERIOD * SEG
        HR = PR // 2
        QR = PR // 4
        NPER = (S // SEG - 1) // PERIOD
        assert NPER * PR + SEG == S
        scale = DH ** -0.5
        row = lax.broadcasted_iota(jnp.int32, (L, L), 0)
        col = lax.broadcasted_iota(jnp.int32, (L, L), 1)
        mask = (row < M) | (row >= col)

        def w_in(i, p, which=(0, 1, 2)):
            return jnp.concatenate([_get(wqkv, (i, j, p)) for j in which], axis=1)

        def w_out(i, g):
            return _load7(wo, i, pl.ds(g * PG * DH // 2, PG * DH // 2))

        def token_lhs(r0):
            blocks = [xn[pl.ds(r0 + a * HR, HR), pl.ds(b * HD, HD)].astype(F32) for a in range(2) for b in range(2)]
            for i, v in enumerate(_operands(_LHS, blocks)):
                xc[i] = v

        def out_copy(r0, n):
            return pltpu.make_async_copy(xb.at[pl.ds(r0, n)], out_hbm.at[pl.ds(r0, n)], sem_out)

        def emit(r0):
            xb[pl.ds(r0, PR), :] = (base[pl.ds(r0, PR), :] + go[...]).astype(BF16)

        def quarter(a, half):
            return pl.ds(a * HR + half * QR, QR)

        wo_copy(NF).wait()
        mem_copy.wait()
        with _scope("a_pro"):
            never = _never(xb)
            side = wo_jobs(wo, NF)
            token_lhs(0)
            for p in range(NP):
                c = [None] * 4
                for i in _ORDER:
                    _fold(c, i, _paced_dot(xc[i], w_in(i, p), _share(side, p, NP) if i == 0 else [], never))
                for j in range(3):
                    for k, v in enumerate(c):
                        gq[j, 2 * p + k % 2, pl.ds(k // 2 * HR, HR), :] = _lanes(v, j)
            ob[...] = jnp.zeros(ob.shape, F32)
            go[...] = jnp.zeros(go.shape, F32)

        def period(it, mem):
            done = pl.multiple_of(jnp.maximum(it - 2, 0) * PR, PR)
            token_lhs(pl.multiple_of((it + 1) * PR, HR))
            emit(done)
            for step, products in enumerate(_STEP_PRODUCTS):
                mem = segment(step, products, mem)

            @pl.when(it >= 2)
            def _():
                out_copy(done, PR).start()

            return mem

        def segment(step, products, mem):
            rows = pl.ds(step * SEG, SEG)
            ml = _mem_lhs(mem[:, :HD], mem[:, HD:])
            lhs = {
                i: jnp.concatenate([ml[i], xc[i, pl.ds(s * QR, n * QR), :]], axis=0)
                for i, (s, n) in products
            }
            qkv_mem, prob, att_mem, acc = {}, {}, {}, {}

            def project(p):
                if step == 0:
                    for j in range(3):
                        for b in range(2):
                            fq[j, 2 * p + b] = gq[j, 2 * p + b]
                    blocks = [ob[2 * p + b, pl.ds(a * HR, HR), :] for a in range(2) for b in range(2)]
                    for i, v in enumerate(_operands(_LHS, blocks)):
                        oc[i, p, pl.ds(0, HR), :] = v
                r = {i: _dot(lhs[i], w_in(i, p)) for i, _ in products}
                qkv_mem[2 * p], qkv_mem[2 * p + 1] = _mem_out(step, {i: v[:M] for i, v in r.items()})
                for j in range(3):
                    def ld(a, b, half):
                        return gq[j, 2 * p + b, quarter(a, half), :]

                    def st(a, b, half, v):
                        gq[j, 2 * p + b, quarter(a, half), :] = v

                    _token_out(step, {i: _lanes(v[M:], j) for i, v in r.items()}, ld, st)

            def part(j, h):
                return jnp.concatenate([_lanes(qkv_mem[h], j), fq[j, h, rows, :]], axis=0)

            def scores(h):
                prob[h] = _softmax_rows(part(0, h), part(1, h), mask, scale)

            def attend(h):
                o = _dot(prob[h], part(2, h))
                att_mem[h] = o[:M]
                ob[h, rows, :] = o[M:]

            def outproj(g, k):
                i, (s, n) = products[k]
                a = jnp.concatenate([
                    jnp.concatenate(
                        [_mem_lhs(att_mem[2 * p], att_mem[2 * p + 1])[i], oc[i, p, pl.ds(s * QR, n * QR), :]],
                        axis=0)
                    for p in range(g * PG, (g + 1) * PG)], axis=1)
                r = _dot(a, w_out(i, g))
                acc[i] = acc[i] + r if i in acc else r

            todo = [(g, k) for g in range(NG) for k in range(4)]
            for t in range(NP + 2):
                if t < NP:
                    project(t)
                else:
                    for _ in range(TAIL[t - NP]):
                        outproj(*todo.pop(0))
                if 0 <= t - 1 < NP:
                    scores(2 * (t - 1))
                    scores(2 * (t - 1) + 1)
                if 0 <= t - 2:
                    attend(2 * (t - 2))
                    attend(2 * (t - 2) + 1)
                for _ in range(2):
                    if t < NP and len(todo) > sum(TAIL) + 4 and (todo[0][0] + 1) * PG <= t - 2:
                        outproj(*todo.pop(0))
            for job in todo:
                outproj(*job)

            def ld(a, b, half):
                return go[quarter(a, half), pl.ds(b * HD, HD)]

            def st(a, b, half, v):
                go[quarter(a, half), pl.ds(b * HD, HD)] = v

            _token_out(step, {i: v[M:] for i, v in acc.items()}, ld, st)
            return jnp.concatenate(_mem_out(step, {i: v[:M] for i, v in acc.items()}), axis=1)

        with _scope("a_loop"):
            mem = lax.fori_loop(0, NPER, period, mem0[...].astype(F32))

        with _scope("a_epi"):
            emit((NPER - 2) * PR)
            out_copy((NPER - 2) * PR, PR).start()
            ml = _mem_lhs(mem[:, :HD], mem[:, HD:])
            rows = pl.ds(0, SEG)
            ER = (PR + SEG) // 2
            kv_mem, prob, acc = {}, {}, {}

            def part(j, h):
                return jnp.concatenate([_lanes(kv_mem[h], j - 1), gq[j, h, rows, :]], axis=0)

            def outproj(g, i):
                a = jnp.concatenate([oc[i, p] for p in range(g * PG, (g + 1) * PG)], axis=1)
                r = _dot(a, w_out(i, g))
                acc[i] = acc[i] + r if i in acc else r

            todo = [(g, i) for g in range(NG) for i in _ORDER]
            for t in range(NP + 4):
                if t < NP:
                    kv_mem[2 * t], kv_mem[2 * t + 1] = _mem_out(
                        1, {i: _dot(ml[i], w_in(i, t, (1, 2))) for i, _ in _STEP_PRODUCTS[1]})
                if 0 <= t - 2 < NP:
                    for h in (2 * (t - 2), 2 * (t - 2) + 1):
                        prob[h] = _softmax_rows(gq[0, h, rows, :], part(1, h), mask[M:], scale)
                if 0 <= t - 4:
                    p = t - 4
                    new = [_dot(prob[h], part(2, h)) for h in (2 * p, 2 * p + 1)]
                    top = [ob[2 * p + b, pl.ds(0, ER), :] for b in range(2)]
                    bot = [jnp.concatenate([ob[2 * p + b, pl.ds(ER, PR - ER), :], new[b]], axis=0) for b in range(2)]
                    for i, v in enumerate(_operands(_LHS, top + bot)):
                        oc[i, p] = v
                if t >= NP - 1:
                    for _ in range(3):
                        outproj(*todo.pop(0))
            for job in todo:
                outproj(*job)
            c = [None] * 4
            for i in _ORDER:
                _fold(c, i, acc[i])
            r0 = (NPER - 1) * PR
            for k, v in enumerate(c):
                idx = (pl.ds(r0 + k // 2 * ER, ER), pl.ds(k % 2 * HD, HD))
                xb[idx] = (base[idx] + v).astype(BF16)
            out_copy(r0, 2 * ER).start()
        with _scope("tail"):
            out_copy(0, S).wait()

    if "1" in PARTS:
        pl.run_scoped(
            token_mixing,
            pltpu.VMEM((2, D, D), BF16),
            _words(7, HD // LANES, HD // 2),
            _words(7, HD // LANES, HD // 2),
            pltpu.VMEM((2, 2, R1, D), F32),
            pltpu.VMEM((2, R1, D), F32),
            pltpu.VMEM((2, R1, D), F32),
            pltpu.VMEM((NCB, S + 2 * SUB, LANES), F32),
            pltpu.SemaphoreType.DMA((NT,)),
            pltpu.SemaphoreType.DMA((5,)),
        )

    def rest(wo):
        PR = PERIOD * SEG
        if "3" in PARTS:
            pl.run_scoped(
                functools.partial(ffn, wo),
                _words(7, HD // LANES, FC // 4),
                pltpu.VMEM((2, 2, R3, FC), F32),
            )
        if "A" not in PARTS:
            k = xb[0:8, 0:128].astype(jnp.int32)[0, 0]
            k16 = pl.ds(pl.multiple_of(k * 16, 16), 16)
            xb[0:16, 0:128] = (_get(wqkv, (k, k, k, pl.ds(0, 8))) + _get(wo, (k, k, pl.ds(0, 8))) + _get(yc, (k, k, pl.ds(0, 8)))
                               + _get(w3c, (k, k, pl.ds(0, 8))) + xn[k16, 0:128] + base[k16, 0:128].astype(BF16))
            pltpu.sync_copy(xb, out_hbm)
            return
        pl.run_scoped(
            functools.partial(recurrence, wo),
            pltpu.VMEM((7, PR // 2, HD), F32),
            pltpu.VMEM((3, H, PR, DH), F32),
            pltpu.VMEM((3, H, PR, DH), F32),
            pltpu.VMEM((H, PR, DH), F32),
            pltpu.VMEM((7, NP, (PR + SEG) // 2, DH), F32),
            pltpu.VMEM((PR, D), F32),
            pltpu.SemaphoreType.DMA(()),
        )

    pl.run_scoped(rest, _words(7, HD // LANES, H * DH // 4))


@functools.partial(jax.jit, static_argnames=("A_seg_len",))
def pallas_parallel_sum__memory_aug_recurrent_mem_tr__mixer_s_mlp__prompt_kernel(
    A_x: jax.Array,
    A_mem0: jax.Array,
    A_Wq: jax.Array,
    A_Wk: jax.Array,
    A_Wv: jax.Array,
    A_Wo: jax.Array,
    A_seg_len: int,
    B_x: jax.Array,
    B_w1: jax.Array,
    B_w2: jax.Array,
    B_w3: jax.Array,
    B_w4: jax.Array,
):
    del B_x
    B, S, D = A_x.shape
    _, H, DH = A_Wq.shape
    M = A_mem0.shape[1]
    F = B_w3.shape[1]
    SEG = int(A_seg_len)
    assert B == 1 and DH == LANES
    HD = D // 2
    parts = F // FC + 1

    hbm = pl.BlockSpec(memory_space=pl.ANY)
    out = pl.pallas_call(
        functools.partial(_kernel, S=S, D=D, H=H, DH=DH, M=M, SEG=SEG, F=F),
        out_shape=jax.ShapeDtypeStruct((S, D), A_x.dtype),
        in_specs=[hbm] * 10,
        out_specs=hbm,
        scratch_shapes=[
            pltpu.VMEM((S, D), BF16),
            pltpu.VMEM((S + (PERIOD - 1) * SEG, D), BF16),
            pltpu.VMEM((S, D), F32),
            _words(7, 3, H // 2, HD // 2),
            _words(7, HD // LANES, S // 4),
            _words(7, FC // 2 // LANES, HD // 2),
            pltpu.VMEM((2, D, FC), BF16),
            pltpu.VMEM((2, FC, D), BF16),
            pltpu.VMEM((2, 6, HD // parts * H, LANES), BF16),
            _words(6, H // 2 * (HD // parts + 1)),
            pltpu.VMEM((2, H * DH // parts, D), BF16),
            pltpu.VMEM((M, D), BF16),
            pltpu.SemaphoreType.DMA((2, 2)),
            pltpu.SemaphoreType.DMA((2, 7)),
            pltpu.SemaphoreType.DMA(()),
        ],
        compiler_params=pltpu.CompilerParams(vmem_limit_bytes=127 * 1024 * 1024, flags=FLAGS),
    )(
        A_x.reshape(S, D),
        A_mem0.reshape(M, D),
        A_Wq.reshape(D * H, DH),
        A_Wk.reshape(D * H, DH),
        A_Wv.reshape(D * H, DH),
        A_Wo.reshape(H * DH, D),
        B_w1, B_w2, B_w3, B_w4,
    )
    return out.reshape(B, S, D)
```

```python
import contextlib
import functools
import itertools
import math

import jax
import jax.numpy as jnp
from jax import lax
from jax.experimental import pallas as pl
from jax.experimental.pallas import tpu as pltpu

F32 = jnp.float32
BF16 = jnp.bfloat16
U32 = jnp.uint32
LANES = 128
SUB = 8
EPS = 1e-5
R1 = 128
R3 = 256
FC = 512
NORM = 16
NORM3 = 32
KB = 64
PG = 4
PERIOD = 3
TAIL = (2, 4, 2)
SPLIT = (5, 6)
DUE = 2
SPREAD = 5
SPLIT7 = 4
SPREAD1 = 6
LU = 2
LD = 2
RU = 64
RD = 32
W3F = False
W4F = False
AF = False
WU = 3
WD = 1
WE = 3
W1 = 1
CW = 2
WQF = False
SCOPES = False
PARTS = "13A"
FLAGS = None


def _scope(name):
    return jax.named_scope(name) if SCOPES else contextlib.nullcontext()


def _layernorm(x):
    m = jnp.mean(x, axis=-1, keepdims=True)
    d = x - m
    v = jnp.mean(d * d, axis=-1, keepdims=True)
    r = lax.rsqrt(v + EPS)
    return d * r, v * r * r


def _gelu(x):
    return 0.5 * _gelu2(x)


def _gelu2(x):
    c = math.sqrt(2 / math.pi)
    return x + x * jnp.tanh(x * (c + (c * 0.044715) * (x * x)))


def _softmax_rows(q, k, mask, scale):
    z = lax.dot_general(q, k, (((1,), (1,)), ((), ())), preferred_element_type=F32)
    z = jnp.where(mask, z * scale, -1e9)
    e = jnp.exp(z - jnp.max(z, axis=-1, keepdims=True))
    s = jnp.sum(e, axis=-1, keepdims=True)
    r = pl.reciprocal(s, approx=True)
    return e * (r * (2.0 - s * r))


def _dot(a, b):
    return jnp.dot(a, b, preferred_element_type=F32)


def _put(ref, idx, v):
    if ref.dtype != U32:
        if len(idx) == len(ref.shape) - 1:
            r = idx[-1]
            idx = idx[:-1] + (pl.ds(2 * r.start, 2 * r.size),)
        ref[idx] = v.astype(ref.dtype)
        return
    ref[idx] = pltpu.bitcast(v.astype(BF16), U32)


def _get(ref, idx):
    if ref.dtype == F32:
        return ref[idx]
    if ref.dtype == BF16:
        return pltpu.bitcast(ref.bitcast(U32)[idx], BF16)
    return pltpu.bitcast(ref[idx], BF16)


def _words(*shape, f32=False):
    if f32:
        return pltpu.VMEM(shape[:-1] + (2 * shape[-1], LANES), F32 if f32 is True else BF16)
    return pltpu.VMEM(shape + (LANES,), U32)


def _lanes(v, c):
    return v[:, c * LANES:(c + 1) * LANES]


_LHS = (((0, 0), (1, 1), 1), ((1, 0), (1, 1), 1), ((0, 0),), ((1, 1),),
        ((0, 0), (0, 1), 1), ((1, 0), (0, 0), -1), ((0, 1), (1, 1), -1))
_RHS = (((0, 0), (1, 1), 1), ((0, 0),), ((0, 1), (1, 1), -1), ((1, 0), (0, 0), -1),
        ((1, 1),), ((0, 0), (0, 1), 1), ((1, 0), (1, 1), 1))
_OUT = (((0, 1), (3, 1)), ((2, 1), (3, -1)), ((1, 1), (3, 1)), ((0, 1), (2, 1)),
        ((0, -1), (1, 1)), ((3, 1),), ((0, 1),))
_ORDER = (0, 3, 1, 2, 4, 5, 6)


def _operand(terms, block):
    if len(terms) == 1:
        return block(*terms[0])
    u, v = block(*terms[0]), block(*terms[1])
    return u + v if terms[2] > 0 else u - v


def _operands(table, blocks):
    return [_operand(terms, lambda a, b: blocks[2 * a + b]) for terms in table]


def _fold(c, i, m):
    for k, sign in _OUT[i]:
        if c[k] is None:
            c[k] = m if sign > 0 else -m
        else:
            c[k] = c[k] + m if sign > 0 else c[k] - m


def _load7(ref, i, rows=slice(None)):
    return jnp.concatenate([_get(ref, (i, c, rows)) for c in range(ref.shape[1])], axis=1)


_ALL, _LO, _HI = (0, 2), (0, 1), (1, 1)
_STEP_PRODUCTS = (
    ((0, _ALL), (1, _LO), (2, _LO), (3, _LO)),
    ((1, _HI), (3, _HI), (5, _LO), (6, _LO)),
    ((4, _ALL), (2, _HI), (5, _HI), (6, _HI)),
)


def _mem_lhs(m1, m2):
    s = m1 + m2
    return (s, s, m1, m2, s, m1, m2)


def _mem_out(step, m):
    if step == 0:
        return m[1] + m[3], m[2] + m[0] - m[1]
    if step == 1:
        c1 = m[1] + m[3]
        return c1, m[5] + m[6] - c1
    c2 = m[2] + m[4]
    return m[5] + m[6] - c2, c2


def _token_out(step, m, ld, st):
    if step == 0:
        q = m[1].shape[0]
        lo, hi = m[0][:q], m[0][q:]
        st(0, 0, 0, lo + m[3])
        st(0, 1, 0, m[2])
        st(1, 0, 0, m[1] + m[3])
        st(1, 1, 0, lo - m[1] + m[2])
        st(0, 0, 1, hi)
    elif step == 1:
        st(0, 0, 0, ld(0, 0, 0) + m[6])
        st(1, 1, 0, ld(1, 1, 0) + m[5])
        t = ld(0, 0, 1)
        st(0, 0, 1, t + m[3])
        st(1, 0, 1, m[1] + m[3])
        st(1, 1, 1, t - m[1])
    else:
        q = m[2].shape[0]
        lo, hi = m[4][:q], m[4][q:]
        st(0, 0, 0, ld(0, 0, 0) - lo)
        st(0, 1, 0, ld(0, 1, 0) + lo)
        st(0, 0, 1, ld(0, 0, 1) + m[6] - hi)
        st(0, 1, 1, m[2] + hi)
        st(1, 1, 1, ld(1, 1, 1) + m[2] + m[5])


def _share(jobs, k, n):
    return jobs[len(jobs) * k // n:len(jobs) * (k + 1) // n]


def _mix(*lists):
    keyed = [((n + 0.5) / len(l), k, n) for k, l in enumerate(lists) for n in range(len(l))]
    return [lists[k][n] for _, k, n in sorted(keyed)]


def _jobs(fn, *ranges):
    return [functools.partial(fn, *k) for k in itertools.product(*ranges)]


def _run(jobs):
    for job in jobs:
        job(lambda v: v)


def _never(ref):
    return jnp.abs(ref[0:SUB, 0:LANES].astype(F32)) < 0.0


class _Pacer:
    def __init__(self, never):
        self.never = never
        self.tokens = []

    def dot(self, a, b):
        m = _dot(a, b)
        rounds = min(max(a.shape[1] * m.shape[1] // (4 * LANES * LANES), 1), m.shape[1] // LANES)
        self.tokens += [
            m[r:r + SUB, c:c + LANES]
            for c in range(0, m.shape[1], m.shape[1] // rounds) for r in range(0, m.shape[0], SUB)
        ]
        return m

    def run(self, *job_lists):
        tokens, self.tokens = self.tokens, []

        def gate(k, count, v):
            n = v.shape[0] // SUB
            rows = []
            for r in range(n):
                t = lax.bitcast_convert_type(tokens[len(tokens) * (k * n + r) // (count * n)], v.dtype)
                rows.append(jnp.concatenate([
                    jnp.where(self.never, t, v[r * SUB:(r + 1) * SUB, c:c + LANES])
                    for c in range(0, v.shape[1], LANES)], axis=1))
            return jnp.concatenate(rows, axis=0)

        due = []
        for job in _mix(*[
            [functools.partial(job, functools.partial(gate, k, len(jobs))) for k, job in enumerate(jobs)]
            for jobs in job_lists
        ]):
            due += job() or []
        return due


def _paced_dot(a, b, side, never):
    pacer = _Pacer(never)
    return pacer.dot(a, b), pacer.run(side)


def _strassen(lhs, w, side, never, spread=7, order=_ORDER):
    c = [None] * 4
    due = [[]] * DUE
    for n, i in enumerate(order):
        m, late = _paced_dot(lhs(i, due.pop(0), never), _load7(w, i), _share(side, n, spread) if n < spread else [], never)
        due.append(late)
        _fold(c, i, m)
    return c


def _lhs_from(block):
    def lhs(i, due=(), never=None):
        a = _operand(_LHS[i], block)
        if due:
            rows = [a[r:r + SUB] for r in range(0, a.shape[0], SUB)]
            for n, v in enumerate(due):
                r = len(rows) // 2 + n * len(rows) // 2 // len(due)
                rows[r] = jnp.concatenate([jnp.where(never, v, rows[r][:, :LANES]), rows[r][:, LANES:]], axis=1)
            a = jnp.concatenate(rows, axis=0)
        return a if AF else a.astype(BF16)

    return lhs


def _rhs_jobs(dst, src, kh, nh, which=range(7)):
    def job(c, k0, gate):
        @functools.cache
        def block(a, b):
            return gate(src(pl.ds(a * kh + k0, KB), pl.ds(b * nh + c * LANES, LANES)).astype(F32))

        for i in which:
            _put(dst, (i, c, pl.ds(k0 // 2, KB // 2)), _operand(_RHS[i], block))

    return _jobs(job, range(nh // LANES), range(0, kh, KB))


def _rhs2_jobs(dst, src, kq, nq):
    @functools.cache
    def block(c, k0, a, b):
        return src(pl.ds(a * kq + k0, KB2), pl.ds(b * nq + c * LANES, LANES)).astype(F32)

    def job(c, k0, i, gate):
        outer = functools.cache(lambda a, b: gate(_operand(_RHS[i], lambda u, v: block(c, k0, 2 * u + a, 2 * v + b))))
        for j in range(7):
            _put(dst, (7 * i + j, c, pl.ds(k0 // 2, KB2 // 2)), _operand(_RHS[j], outer))

    KB2 = 16
    return _jobs(job, range(nq // LANES), range(0, kq, KB2), range(7))


def _strassen2(outer, w, pacer, cols=None):
    c = [[None] * 4 for _ in range(4)]
    for i in _ORDER:
        block = functools.cache(functools.partial(outer, i))
        inner = [None] * 4
        for j in _ORDER:
            b = _load7(w, 7 * i + j) if cols is None else _get(w, (7 * i + j, cols))
            _fold(inner, j, pacer.dot(_operand(_LHS[j], block).astype(F32 if AF else BF16), b))
        for q in range(4):
            _fold(c[q], i, inner[q])
    return [[c[q][k] for q in range(4)] for k in range(4)]


def _qkv_part(D, F):
    return -(-D // 2 // 16 // (F // FC)) * 16


def _kernel(
    x_hbm, mem_hbm, wq_hbm, wk_hbm, wv_hbm, wo_hbm, w1_hbm, w2_hbm, w3_hbm, w4_hbm,
    out_hbm,
    xb, xn, macc, wqkv, raw_o, mem0, sem_m, sem_o,
    *, S, D, H, DH, M, SEG, F,
):
    HD = D // 2
    NCB = D // LANES
    NP = H // 2
    T1 = 2 * R1
    NT = S // T1
    NF = F // FC
    DP = _qkv_part(D, F)
    OR = H * DH // (NF + 1)

    def wo_copy(part):
        rows = pl.ds(pl.multiple_of(part * OR, OR), OR)
        return pltpu.make_async_copy(wo_hbm.at[rows], raw_o.at[rows], sem_o)

    mem_copy = pltpu.make_async_copy(mem_hbm, mem0, sem_m)

    def wo_jobs(wo):
        def combine(p, c, k, gate):
            blocks = [
                gate(raw_o[pl.ds((2 * p + a) * DH + k, KB), pl.ds(b * HD + c * LANES, LANES)].astype(F32))
                for a in range(2) for b in range(2)
            ]
            for i, v in enumerate(_operands(_RHS, blocks)):
                _put(wo, (i, c, pl.ds((p * DH + k) // 2, KB // 2)), v)

        return _jobs(combine, range(NP), range(HD // LANES), range(0, DH, KB))

    def mixer(yc, w3c, r3, r4, raw, sem_f, sem_a):
        def w3_copy(f):
            cols = pl.ds(pl.multiple_of(f * FC, FC), FC)
            return pltpu.make_async_copy(w3_hbm.at[:, cols], r3.at[f % 2], sem_f.at[0, f % 2])

        def w4_copy(f):
            rows = pl.ds(pl.multiple_of(f * FC, FC), FC)
            return pltpu.make_async_copy(w4_hbm.at[rows], r4.at[f % 2], sem_f.at[1, f % 2])

        def qkv_start(part):
            return jnp.minimum(part * DP, HD - DP)

        def qkv_copies(part):
            return [
                pltpu.make_async_copy(
                    w.at[pl.ds(pl.multiple_of((a * HD + qkv_start(part)) * H, 16 * H), DP * H)],
                    raw.at[part % 2, 2 * j + a], sem_a.at[part % 2, 2 * j + a])
                for j, w in enumerate((wq_hbm, wk_hbm, wv_hbm)) for a in range(2)
            ]

        def qkv_jobs(part, mid):
            dst = wqkv.at[:, :, :, pl.ds(pl.multiple_of(qkv_start(part), 16), DP)] if WQF else wqkv.at[:, :, :, pl.ds(pl.multiple_of(qkv_start(part) // 2, SUB), DP // 2)]

            def transpose(j, a, g, gate):
                rows = gate(jnp.concatenate([
                    pltpu.bitcast(raw[part % 2, 2 * j + a, pl.ds(d * H + g * 16, 16), :], U32)
                    for d in range(DP)], axis=0))
                for d in range(DP):
                    mid[2 * j + a, pl.ds(g * SUB * (DP + 1) + d, SUB, stride=DP + 1), :] = rows[d * SUB:(d + 1) * SUB]

            def combine(j, p, gate):
                blocks = []
                for a in range(2):
                    v = gate(mid[2 * j + a, pl.ds(p * (DP + 1), DP), :])
                    blocks.append(pltpu.bitcast(v << 16, F32))
                    blocks.append(pltpu.bitcast(v & jnp.uint32(0xFFFF0000), F32))
                for i, v in enumerate(_operands(_RHS, blocks)):
                    _put(dst, (i, j, p), v)

            tr = [_jobs(transpose, [j], range(2), range(NP // SUB)) for j in range(3)]
            cb = [_jobs(combine, [j], range(NP)) for j in range(3)]
            return tr[0] + _mix(tr[1], cb[0]) + _mix(tr[2], cb[1]) + cb[2]

        def w3_jobs(f):
            return (_rhs_jobs, _rhs2_jobs)[LU - 1](w3c.at[f % 2], lambda r, k: r3[f % 2, r, k], HD // LU, FC // 2 // LU)

        def token_mixing(r12, y0, c1, c2, hb, sem_x, sem_w):
            w1c, w2c = (wqkv.at[:, j, pl.ds(0, NCB // 2)] for j in range(2))
            shifts = (-1, 1, -2, 2)
            pieces = range(0, R1, NORM)

            def x_copy(t):
                rows = pl.ds(pl.multiple_of(t * T1, T1), T1)
                return pltpu.make_async_copy(x_hbm.at[rows], xb.at[rows], sem_x.at[t])

            def w1_copy(a, b):
                idx = (pl.ds(a * HD, HD), pl.ds(b * HD, HD))
                return pltpu.make_async_copy(w1_hbm.at[idx], r12.at[(0,) + idx], sem_w.at[2 * a + b])

            w2_copy = pltpu.make_async_copy(w2_hbm, r12.at[1], sem_w.at[4])

            def tile(ref, t):
                return ref.at[pl.ds(pl.multiple_of(t * T1, T1), T1)]

            def normalizing(t, slot):
                xb_t, xn_t = tile(xb, t), tile(xn, t)

                def job(lo, a, gate):
                    rows = pl.ds(a * R1 + lo, 2 * NORM)
                    n, var = _layernorm(gate(xb_t[rows, :].astype(F32)))
                    xn_t[rows, :] = n.astype(BF16)
                    y = n * lax.rsqrt(var + EPS)
                    y0[slot, a, pl.ds(lo, 2 * NORM), :] = y
                    return [y[r:r + SUB, :LANES] for r in range(0, 2 * NORM, SUB)]

                return _jobs(job, pieces[::2], range(2))

            def keep(dst, c):
                for k, v in enumerate(c):
                    dst[k // 2, :, pl.ds(k % 2 * HD, HD)] = v

            def lhs1(slot):
                return _lhs_from(lambda a, b: y0[slot, a, :, pl.ds(b * HD, HD)])

            def stage1(slot, side):
                keep(c1, _strassen(lhs1(slot), w1c, side, never, SPREAD1))

            def activating(t):
                hb_t = hb.at[:, pl.ds(pl.multiple_of(SUB + t * T1, SUB), T1)]

                def job(a, c, gate):
                    hb_t[c, pl.ds(a * R1, R1), :] = _gelu(gate(c1[a, :, pl.ds(c * LANES, LANES)]))

                return _jobs(job, range(2), range(NCB))

            def stage2(t, side):
                hb_t = hb.at[:, pl.ds(pl.multiple_of(t * T1, SUB), T1 + 2 * SUB)]
                keep(c2, _strassen(_lhs_from(lambda a, b: jnp.concatenate([
                    hb_t[c, pl.ds(SUB + a * R1 + shifts[c * 4 // NCB], R1), :]
                    for c in range(b * NCB // 2, (b + 1) * NCB // 2)], axis=1)), w2c, side, never, SPREAD))

            def renormalizing(t):
                xb_t, xn_t = tile(xb, t), tile(xn, t)
                acc_t = macc.at[:, pl.ds(pl.multiple_of(t * R1, R1), R1)]
                if LU == 2:
                    yc_t = yc.at[:, pl.ds(pl.multiple_of(t * R1, R1), R1)]
                else:
                    yc_t = yc.at[:, :, pl.ds(pl.multiple_of(t * (R1 // 2), R1 // 2), R1 // 2)]

                def job(lo, gate):
                    x1, z = [], []
                    for a in range(2):
                        rows = pl.ds(a * R1 + lo, NORM)
                        x1.append(xn_t[rows, :].astype(F32) + gate(c2[a, pl.ds(lo, NORM), :]))
                        z.append(2.0 * (x1[a] + xb_t[rows, :].astype(F32)))
                    z11, z12, z21, z22 = z[0][:, :HD], z[0][:, HD:], z[1][:, :HD], z[1][:, HD:]
                    for i, v in ((6, z11), (2, z12), (1, z21), (5, z22 - z12 + z21)):
                        acc_t[i, pl.ds(lo, NORM), :] = v
                    y, _ = _layernorm(jnp.concatenate(x1, axis=0))
                    ys = [y[a * NORM:(a + 1) * NORM, b * HD:(b + 1) * HD] for a in range(2) for b in range(2)]
                    for i, v in enumerate(_operands(_LHS, ys)):
                        if LU == 2:
                            yc_t[i, pl.ds(lo, NORM), :] = v
                            continue
                        for c in range(NCB // 2):
                            _put(yc_t, (i, c, pl.ds(lo // 2, NORM // 2)), _lanes(v, c))
                    return [y[r:r + SUB, :LANES] for r in range(0, 2 * NORM, SUB)]

                return _jobs(job, pieces)

            arrival = (((0, 0), (1,)), ((1, 1), (4, 0)), ((0, 1), (2, 5)), ((1, 0), (3, 6)))
            queue = [w1_copy(*q) for q, _ in arrival] + [x_copy(1), x_copy(2)]
            x_copy(0).start()
            queue.pop(0).start()
            for c in range(NCB):
                hb[c, pl.ds(0, SUB), :] = jnp.zeros((SUB, LANES), F32)
                hb[c, pl.ds(SUB + S, SUB), :] = jnp.zeros((SUB, LANES), F32)
            for i in (0, 3, 4):
                macc[i] = jnp.zeros(macc.shape[1:], F32)
            pad = xn.shape[0] - S
            xn[pl.ds(S, pad), :] = jnp.zeros((pad, D), BF16)
            with _scope("wait_x0"):
                x_copy(0).wait()
            queue.pop(0).start()
            never = _never(xb)
            with _scope("tile0"):
                _run(normalizing(0, 1))
                c = [None] * 4
                for q, ready in arrival:
                    w1_copy(*q).wait()
                    queue.pop(0).start()
                    _run(_rhs_jobs(w1c, lambda r, k: r12[0, r, k], HD, HD, ready))
                    for i in ready:
                        _fold(c, i, _dot(lhs1(1)(i), _load7(w1c, i)))
                keep(c1, c)
                x_copy(1).wait()
                w2_copy.start()
                _run(normalizing(1, 0))
            with _scope("tile1"):
                x_copy(3).start()
                x_copy(2).wait()
                stage1(0, _mix(activating(0), normalizing(2, 1)))
                x_copy(4).start()
                mem_copy.start()
                w2_copy.wait()
                x_copy(3).wait()
                stage1(1, _mix(activating(1), _rhs_jobs(w2c, lambda r, k: r12[1, r, k], HD, HD)))
                stage2(0, normalizing(3, 0))

            def slot(u, carry):
                @pl.when(u + 1 < NT)
                def _():
                    x_copy(u + 1).wait()

                @pl.when(u + 2 < NT)
                def _():
                    x_copy(u + 2).start()

                @pl.when(u < 5)
                def _():
                    w3_copy(u - 3).start()

                @pl.when(u == 5)
                def _():
                    w4_copy(0).start()
                    wo_copy(0).start()

                @pl.when(u == 6)
                def _():
                    for cp in qkv_copies(0):
                        cp.start()

                with _scope("slot"):
                    again = renormalizing(u - 3)
                    stage1(0, _mix(activating(u - 1), again[:SPLIT[0]]) + again[SPLIT[0]:SPLIT[1]])
                    stage2(u - 2, _mix(normalizing(jnp.minimum(u + 1, NT - 1), 0), again[SPLIT[1]:]))
                return carry

            lax.fori_loop(3, NT, slot, 0)
            w3_copy(0).wait()
            with _scope("tile7"):
                last = activating(NT - 1)
                halo = [c for c in range(NCB) if shifts[c * 4 // NCB] > 0]
                _run([last[c] for c in halo])
                late = w3_jobs(0)
                stage2(NT - 2, _mix(renormalizing(NT - 3), [job for c, job in enumerate(last) if c not in halo], _share(late, 0, 3)))
                stage2(NT - 1, _mix(renormalizing(NT - 2), _share(late, 1, 3) + _share(late, 2, 3)))
                _run(renormalizing(NT - 1))

        def ffn(w4c, g, mid):
            N3 = S // 2 // R3
            never = _never(xb)

            def chunk(f, carry):
                @pl.when(f + 2 < NF)
                def _():
                    w3_copy(f + 2).start()

                @pl.when(f + 1 < NF)
                def _():
                    w4_copy(f + 1).start()
                    for cp in qkv_copies(f + 1):
                        cp.start()
                    w3_copy(f + 1).wait()

                wo_copy(f + 1).start()
                for cp in qkv_copies(f) + [w4_copy(f)]:
                    cp.wait()
                pre, post = {}, {}

                def join(parts):
                    return [
                        jnp.concatenate([jnp.concatenate(p[k][2 * a:2 * a + 2], axis=1) for p in parts for a in range(2)], axis=0)
                        for k in range(4)
                    ]

                pacer = _Pacer(never)

                def up(t, *side):
                    if LU == 1:
                        pre[t] = [None] * 4
                        for i in _ORDER:
                            _fold(pre[t], i, pacer.dot(_load7(yc, i, pl.ds(t * R3 // 2, R3 // 2)), _load7(w3c.at[f % 2], i)))
                    else:
                        pre[t] = join([
                            _strassen2(
                                lambda i, a, b: yc[i, pl.ds(t * R3 + (2 * s + a) * RU, RU), pl.ds(b * HD // 2, HD // 2)],
                                w3c.at[f % 2], pacer)
                            for s in range(R3 // (2 * RU))])
                    pacer.run(*side)

                def activate(t, lo, gate):
                    for k, v in enumerate(pre[t]):
                        g[t % 2, k // 2, pl.ds(lo, NORM3), pl.ds(k % 2 * FC // 2, FC // 2)] = _gelu2(gate(v[lo:lo + NORM3]))

                def down(t, *side):
                    if LD == 1:
                        for s in range(R3 // RD):
                            lhs = functools.cache(_lhs_from(lambda a, b: g[t % 2, a, pl.ds(s * RD, RD), pl.ds(b * FC // 2, FC // 2)]))
                            for i in _ORDER:
                                macc[i, pl.ds(t * R3 + s * RD, RD), :] += pacer.dot(lhs(i), _load7(w4c, i))
                    else:
                        for s in range(R3 // (2 * RD)):
                            for i in _ORDER:
                                outer = functools.cache(lambda a, b: _operand(_LHS[i], lambda u, v: g[
                                    t % 2, u, pl.ds((2 * s + a) * RD, RD), pl.ds((2 * v + b) * FC // 4, FC // 4)]))
                                lhs = functools.cache(_lhs_from(outer))
                                for c in range(2 // CW):
                                    def idx(q):
                                        return (i, pl.ds(t * R3 + (2 * s + q // 2) * RD, RD), pl.ds(q % 2 * HD // 2 + c * LANES, CW * LANES))

                                    acc = [macc[idx(q)] for q in range(4)]
                                    for j in _ORDER:
                                        w = _get(w4c, (7 * i + j, c)) if CW == 1 else _load7(w4c, 7 * i + j)
                                        _fold(acc, j, pacer.dot(lhs(j), w))
                                    for q in range(4):
                                        macc[idx(q)] = acc[q]
                    pacer.run(*side)

                def rows_of(fn, t):
                    return _jobs(fn, [t], range(0, R3, NORM3))

                side = [qkv_jobs(f, mid)]
                w3j = w3_jobs(f + 1)
                total = WU * (N3 - 2) + WD * (N3 - 1) + WE + W1
                at = 0

                def take(n):
                    nonlocal at
                    at += n
                    return [l[len(l) * (at - n) // total:len(l) * at // total] for l in side]

                with _scope("chunk"):
                    up(0, (_rhs_jobs, _rhs2_jobs)[LD - 1](w4c, lambda r, k: r4[f % 2, r, k], FC // 2 // LD, HD // LD))
                    up(1, rows_of(activate, 0), *take(W1))
                    for t in range(N3 - 2):
                        down(t, rows_of(activate, t + 1), *take(WD), _share(w3j, t, N3))
                        up(t + 2, *take(WU))
                    down(N3 - 2, rows_of(activate, N3 - 1), *take(WD), _share(w3j, N3 - 2, N3))
                    down(N3 - 1, *take(WE), _share(w3j, N3 - 1, N3))
                return carry

            lax.fori_loop(0, NF, chunk, 0)

        if "1" in PARTS:
            pl.run_scoped(
                token_mixing,
                pltpu.VMEM((2, D, D), BF16),
                pltpu.VMEM((2, 2, R1, D), F32),
                pltpu.VMEM((2, R1, D), F32),
                pltpu.VMEM((2, R1, D), F32),
                pltpu.VMEM((NCB, S + 2 * SUB, LANES), F32),
                pltpu.SemaphoreType.DMA((NT,)),
                pltpu.SemaphoreType.DMA((5,)),
            )
        if "3" in PARTS:
            pl.run_scoped(
                ffn,
                _words(49, HD // 2 // LANES, FC // 8),
                pltpu.VMEM((2, 2, R3, FC), F32),
                _words(6, NP * (DP + 1)),
            )
        else:
            k = xb[0:8, 0:128].astype(jnp.int32)[0, 0]
            xb[0:16, 0:128] = yc[k, 0:16, 0:128].astype(BF16) + w3c[k, k, k, 0:16].astype(F32).astype(BF16)

    def recurrence(wo, base, xc, gq, fq, ob, oc, go, sem_out):
        NG = NP // PG
        L = M + SEG
        PR = PERIOD * SEG
        HR = PR // 2
        QR = PR // 4
        NPER = (S // SEG - 1) // PERIOD
        assert NPER * PR + SEG == S
        scale = DH ** -0.5
        row = lax.broadcasted_iota(jnp.int32, (L, L), 0)
        col = lax.broadcasted_iota(jnp.int32, (L, L), 1)
        mask = (row < M) | (row >= col)

        def w_in(i, p, which=(0, 1, 2)):
            return jnp.concatenate([_get(wqkv, (i, j, p)) for j in which], axis=1)

        def w_out(i, g):
            return _load7(wo, i, pl.ds(g * PG * DH // 2, PG * DH // 2))

        def token_lhs(r0):
            blocks = [xn[pl.ds(r0 + a * HR, HR), pl.ds(b * HD, HD)].astype(F32) for a in range(2) for b in range(2)]
            for i, v in enumerate(_operands(_LHS, blocks)):
                xc[i] = v

        def out_copy(r0, n):
            return pltpu.make_async_copy(xb.at[pl.ds(r0, n)], out_hbm.at[pl.ds(r0, n)], sem_out)

        def emit(r0):
            xb[pl.ds(r0, PR), :] = (base[pl.ds(r0, PR), :] + go[...]).astype(BF16)

        def quarter(a, half):
            return pl.ds(a * HR + half * QR, QR)

        pltpu.make_async_copy(wo_hbm, raw_o, sem_o).wait()
        mem_copy.wait()
        with _scope("a_pro"):
            pacer = _Pacer(_never(xb))

            def collect(lo, gate):
                c = [None] * 4
                for i in _ORDER:
                    v = macc[i, pl.ds(lo, NORM), :]
                    _fold(c, i, gate(v) if i < 3 else v)
                t, r = divmod(lo, R1)
                for k, v in enumerate(c):
                    base[pl.ds(t * T1 + k // 2 * R1 + r, NORM), pl.ds(k % 2 * HD, HD)] = 0.5 * v

            token_lhs(0)
            for p in range(NP):
                c = [None] * 4
                for i in _ORDER:
                    _fold(c, i, pacer.dot(xc[i], w_in(i, p)))
                for j in range(3):
                    for k, v in enumerate(c):
                        gq[j, 2 * p + k % 2, pl.ds(k // 2 * HR, HR), :] = _lanes(v, j)
            pacer.run(wo_jobs(wo), _jobs(collect, range(0, S // 2, NORM)))
            ob[...] = jnp.zeros(ob.shape, F32)
            go[...] = jnp.zeros(go.shape, F32)

        def period(it, mem):
            done = pl.multiple_of(jnp.maximum(it - 2, 0) * PR, PR)
            token_lhs(pl.multiple_of((it + 1) * PR, HR))
            emit(done)
            for step, products in enumerate(_STEP_PRODUCTS):
                mem = segment(step, products, mem)

            @pl.when(it >= 2)
            def _():
                out_copy(done, PR).start()

            return mem

        def segment(step, products, mem):
            rows = pl.ds(step * SEG, SEG)
            ml = _mem_lhs(mem[:, :HD], mem[:, HD:])
            lhs = {
                i: jnp.concatenate([ml[i], xc[i, pl.ds(s * QR, n * QR), :]], axis=0)
                for i, (s, n) in products
            }
            qkv_mem, prob, att_mem, acc = {}, {}, {}, {}

            def project(p):
                if step == 0:
                    for j in range(3):
                        for b in range(2):
                            fq[j, 2 * p + b] = gq[j, 2 * p + b]
                    blocks = [ob[2 * p + b, pl.ds(a * HR, HR), :] for a in range(2) for b in range(2)]
                    for i, v in enumerate(_operands(_LHS, blocks)):
                        oc[i, p, pl.ds(0, HR), :] = v
                r = {i: _dot(lhs[i], w_in(i, p)) for i, _ in products}
                qkv_mem[2 * p], qkv_mem[2 * p + 1] = _mem_out(step, {i: v[:M] for i, v in r.items()})
                for j in range(3):
                    def ld(a, b, half):
                        return gq[j, 2 * p + b, quarter(a, half), :]

                    def st(a, b, half, v):
                        gq[j, 2 * p + b, quarter(a, half), :] = v

                    _token_out(step, {i: _lanes(v[M:], j) for i, v in r.items()}, ld, st)

            def part(j, h):
                return jnp.concatenate([_lanes(qkv_mem[h], j), fq[j, h, rows, :]], axis=0)

            def scores(h):
                prob[h] = _softmax_rows(part(0, h), part(1, h), mask, scale)

            def attend(h):
                o = _dot(prob[h], part(2, h))
                att_mem[h] = o[:M]
                ob[h, rows, :] = o[M:]

            def outproj(g, k):
                i, (s, n) = products[k]
                a = jnp.concatenate([
                    jnp.concatenate(
                        [_mem_lhs(att_mem[2 * p], att_mem[2 * p + 1])[i], oc[i, p, pl.ds(s * QR, n * QR), :]],
                        axis=0)
                    for p in range(g * PG, (g + 1) * PG)], axis=1)
                r = _dot(a, w_out(i, g))
                acc[i] = acc[i] + r if i in acc else r

            todo = [(g, k) for g in range(NG) for k in range(4)]
            for t in range(NP + 2):
                if t < NP:
                    project(t)
                else:
                    for _ in range(TAIL[t - NP]):
                        outproj(*todo.pop(0))
                if 0 <= t - 1 < NP:
                    scores(2 * (t - 1))
                    scores(2 * (t - 1) + 1)
                if 0 <= t - 2:
                    attend(2 * (t - 2))
                    attend(2 * (t - 2) + 1)
                for _ in range(2):
                    if t < NP and len(todo) > sum(TAIL) + 4 and (todo[0][0] + 1) * PG <= t - 2:
                        outproj(*todo.pop(0))
            for job in todo:
                outproj(*job)

            def ld(a, b, half):
                return go[quarter(a, half), pl.ds(b * HD, HD)]

            def st(a, b, half, v):
                go[quarter(a, half), pl.ds(b * HD, HD)] = v

            _token_out(step, {i: v[M:] for i, v in acc.items()}, ld, st)
            return jnp.concatenate(_mem_out(step, {i: v[:M] for i, v in acc.items()}), axis=1)

        with _scope("a_loop"):
            mem = lax.fori_loop(0, NPER, period, mem0[...].astype(F32))

        with _scope("a_epi"):
            emit((NPER - 2) * PR)
            out_copy((NPER - 2) * PR, PR).start()
            ml = _mem_lhs(mem[:, :HD], mem[:, HD:])
            rows = pl.ds(0, SEG)
            ER = (PR + SEG) // 2
            kv_mem, prob, acc = {}, {}, {}

            def part(j, h):
                return jnp.concatenate([_lanes(kv_mem[h], j - 1), gq[j, h, rows, :]], axis=0)

            def outproj(g, i):
                a = jnp.concatenate([oc[i, p] for p in range(g * PG, (g + 1) * PG)], axis=1)
                r = _dot(a, w_out(i, g))
                acc[i] = acc[i] + r if i in acc else r

            todo = [(g, i) for g in range(NG) for i in _ORDER]
            for t in range(NP + 4):
                if t < NP:
                    kv_mem[2 * t], kv_mem[2 * t + 1] = _mem_out(
                        1, {i: _dot(ml[i], w_in(i, t, (1, 2))) for i, _ in _STEP_PRODUCTS[1]})
                if 0 <= t - 2 < NP:
                    for h in (2 * (t - 2), 2 * (t - 2) + 1):
                        prob[h] = _softmax_rows(gq[0, h, rows, :], part(1, h), mask[M:], scale)
                if 0 <= t - 4:
                    p = t - 4
                    new = [_dot(prob[h], part(2, h)) for h in (2 * p, 2 * p + 1)]
                    top = [ob[2 * p + b, pl.ds(0, ER), :] for b in range(2)]
                    bot = [jnp.concatenate([ob[2 * p + b, pl.ds(ER, PR - ER), :], new[b]], axis=0) for b in range(2)]
                    for i, v in enumerate(_operands(_LHS, top + bot)):
                        oc[i, p] = v
                if t >= NP - 1:
                    for _ in range(3):
                        outproj(*todo.pop(0))
            for job in todo:
                outproj(*job)
            c = [None] * 4
            for i in _ORDER:
                _fold(c, i, acc[i])
            r0 = (NPER - 1) * PR
            for k, v in enumerate(c):
                idx = (pl.ds(r0 + k // 2 * ER, ER), pl.ds(k % 2 * HD, HD))
                xb[idx] = (base[idx] + v).astype(BF16)
            out_copy(r0, 2 * ER).start()
        with _scope("tail"):
            out_copy(0, S).wait()

    if "1" in PARTS or "3" in PARTS:
        pl.run_scoped(
            mixer,
            pltpu.VMEM((7, S // 2, HD), F32),
            _words(2, 49, FC // 4 // LANES, HD // 4),
            pltpu.VMEM((2, D, FC), BF16),
            pltpu.VMEM((2, FC, D), BF16),
            pltpu.VMEM((2, 6, DP * H, LANES), BF16),
            pltpu.SemaphoreType.DMA((2, 2)),
            pltpu.SemaphoreType.DMA((2, 6)),
        )

    def rest():
        PR = PERIOD * SEG
        if "A" not in PARTS:
            k = xb[0:8, 0:128].astype(jnp.int32)[0, 0]
            k16 = pl.ds(pl.multiple_of(k * 16, 16), 16)
            xb[0:16, 0:128] = (_get(wqkv, (k, k, k, pl.ds(0, 8))) + xn[k16, 0:128] + macc[k, k16, 0:128].astype(BF16))
            pltpu.sync_copy(xb, out_hbm)
            return
        pl.run_scoped(
            recurrence,
            _words(7, HD // LANES, H * DH // 4),
            pltpu.VMEM((S, D), F32),
            pltpu.VMEM((7, PR // 2, HD), F32),
            pltpu.VMEM((3, H, PR, DH), F32),
            pltpu.VMEM((3, H, PR, DH), F32),
            pltpu.VMEM((H, PR, DH), F32),
            pltpu.VMEM((7, NP, (PR + SEG) // 2, DH), F32),
            pltpu.VMEM((PR, D), F32),
            pltpu.SemaphoreType.DMA(()),
        )

    rest()


@functools.partial(jax.jit, static_argnames=("A_seg_len",))
def pallas_parallel_sum__memory_aug_recurrent_mem_tr__mixer_s_mlp__prompt_kernel(
    A_x: jax.Array,
    A_mem0: jax.Array,
    A_Wq: jax.Array,
    A_Wk: jax.Array,
    A_Wv: jax.Array,
    A_Wo: jax.Array,
    A_seg_len: int,
    B_x: jax.Array,
    B_w1: jax.Array,
    B_w2: jax.Array,
    B_w3: jax.Array,
    B_w4: jax.Array,
):
    del B_x
    B, S, D = A_x.shape
    _, H, DH = A_Wq.shape
    M = A_mem0.shape[1]
    F = B_w3.shape[1]
    SEG = int(A_seg_len)
    assert B == 1 and DH == LANES
    HD = D // 2
    parts = F // FC + 1

    hbm = pl.BlockSpec(memory_space=pl.ANY)
    out = pl.pallas_call(
        functools.partial(_kernel, S=S, D=D, H=H, DH=DH, M=M, SEG=SEG, F=F),
        out_shape=jax.ShapeDtypeStruct((S, D), A_x.dtype),
        in_specs=[hbm] * 10,
        out_specs=hbm,
        scratch_shapes=[
            pltpu.VMEM((S, D), BF16),
            pltpu.VMEM((S + (PERIOD - 1) * SEG, D), BF16),
            pltpu.VMEM((7, S // 2, HD), F32),
            _words(7, 3, H // 2, HD // 2, f32=WQF),
            pltpu.VMEM((H * DH, D), BF16),
            pltpu.VMEM((M, D), BF16),
            pltpu.SemaphoreType.DMA(()),
            pltpu.SemaphoreType.DMA(()),
        ],
        compiler_params=pltpu.CompilerParams(vmem_limit_bytes=127 * 1024 * 1024, flags=FLAGS),
    )(
        A_x.reshape(S, D),
        A_mem0.reshape(M, D),
        A_Wq.reshape(D * H, DH),
        A_Wk.reshape(D * H, DH),
        A_Wv.reshape(D * H, DH),
        A_Wo.reshape(H * DH, D),
        B_w1, B_w2, B_w3, B_w4,
    )
    return out.reshape(B, S, D)
```

```python
import contextlib
import functools
import itertools
import math

import jax
import jax.numpy as jnp
import numpy as np
from jax import lax
from jax.experimental import pallas as pl
from jax.experimental.pallas import tpu as pltpu

F32 = jnp.float32
BF16 = jnp.bfloat16
U32 = jnp.uint32
LANES = 128
SUB = 8
PACK = 16
EPS = 1e-5
R1 = 128
RU = 64
RD = 32
R3 = 256
FC = 512
PERIOD = 3
SPLIT = (5, 6)
WU, WD, WE, W1 = 3, 1, 3, 1
TAIL = (64, 64)
YPRE = True
SCOPES = False
PARTS = "13A"
FLAGS = None


def _scope(name):
    return jax.named_scope(name) if SCOPES else contextlib.nullcontext()


def _layernorm(x):
    m = jnp.mean(x, axis=-1, keepdims=True)
    d = x - m
    v = jnp.mean(d * d, axis=-1, keepdims=True)
    r = lax.rsqrt(v + EPS)
    return d * r, v * r * r


def _gelu2(x):
    c = math.sqrt(2 / math.pi)
    return x + x * jnp.tanh(x * (c + (c * 0.044715) * (x * x)))


def _softmax_rows(q, k, mask, scale):
    z = lax.dot_general(q, k, (((1,), (1,)), ((), ())), preferred_element_type=F32)
    z = jnp.where(mask, z * scale, -1e9)
    e = jnp.exp(z - jnp.max(z, axis=-1, keepdims=True))
    s = jnp.sum(e, axis=-1, keepdims=True)
    r = pl.reciprocal(s, approx=True)
    return e * (r * (2.0 - s * r))


def _dot(a, b):
    return jnp.dot(a, b, preferred_element_type=F32)


def _put(ref, idx, v):
    ref[idx] = pltpu.bitcast(v.astype(BF16), U32)


def _get(ref, idx):
    return pltpu.bitcast(ref[idx], BF16)


def _get_wide(ref, i, rows=slice(None)):
    return jnp.concatenate([_get(ref, (i, c, rows)) for c in range(ref.shape[1])], axis=1)


def _words(*shape):
    return pltpu.VMEM(shape + (LANES,), U32)


def _lanes(v, c):
    return v[:, c * LANES:(c + 1) * LANES]


def _combine(coef, get):
    terms = sorted(((int(c), k) for k, c in np.ndenumerate(coef) if c), key=lambda t: -t[0])
    out = get(*terms[0][1]) if terms[0][0] > 0 else -get(*terms[0][1])
    for c, k in terms[1:]:
        out = out + get(*k) if c > 0 else out - get(*k)
    return out


def _scatter(acc, coef, v, tag=(), start=None):
    for k, c in np.ndenumerate(coef):
        if not c:
            continue
        k = k + tag
        if k not in acc and start is not None and (old := start(*k)) is not None:
            acc[k] = old
        if k in acc:
            acc[k] = acc[k] + v if c > 0 else acc[k] - v
        else:
            acc[k] = v if c > 0 else -v


_LHS = np.array([[1, 0, 0, 1], [0, 0, 1, 1], [1, 0, 0, 0], [0, 0, 0, 1],
                 [1, 1, 0, 0], [-1, 0, 1, 0], [0, 1, 0, -1]]).reshape(7, 2, 2)
_RHS = np.array([[1, 0, 0, 1], [1, 0, 0, 0], [0, 1, 0, -1], [-1, 0, 1, 0],
                 [0, 0, 0, 1], [1, 1, 0, 0], [0, 0, 1, 1]]).reshape(7, 2, 2)
_OUT = np.array([[1, 0, 0, 1], [0, 0, 1, -1], [0, 1, 0, 1], [1, 0, 1, 0],
                 [-1, 1, 0, 0], [0, 0, 0, 1], [1, 0, 0, 0]]).reshape(7, 2, 2)
_ORDER = (0, 3, 1, 2, 4, 5, 6)


def _hopcroft_kerr():
    n = 8
    method = (0, 1, 2, 0, 1, 2, 0, 1)
    stand_in = {(0, 3): (0, 2), (0, 6): (6, 2), (3, 6): (3, 2), (1, 4): (1, 5),
                (1, 7): (7, 5), (4, 7): (4, 5), (2, 5): (2, 7)}
    left_out = ("000010010001000022020010002002000200",
                "101101101210121210212121211211211011",
                "111111112122212101101202120120122122")
    forms = np.array([[[[1, 0], [1, 1]], [[-1, 1], [0, 1]]],
                      [[[0, 1], [1, 1]], [[1, -1], [1, 0]]],
                      [[[1, 0], [1, 0]], [[0, 1], [0, 1]]]])
    turn_a, turn_c = np.array([[0, -1], [1, 1]]), np.array([[1, -1], [1, 0]])
    eye = np.eye(n, dtype=int)
    lhs, out, groups, node, inner = [], [], [], {}, {}

    def product(a, c):
        lhs.append(a)
        out.append(c)
        groups[-1].append(len(lhs) - 1)
        return np.eye(100, dtype=int)[len(lhs) - 1]

    def add_node(key, a, c, m):
        groups.append([])
        node[key] = (a, c, m, [product(np.outer(f, a), np.outer(g, c)) for f, g in forms[m]])

    def pair(p, q):
        swap = (node[q][2] - node[p][2]) % 3 != 1
        (ai, ci, mi, di), (aj, cj, _, dj) = (node[q], node[p]) if swap else (node[p], node[q])
        sa, sc = (np.linalg.matrix_power(t, -mi % 3) for t in (turn_a, turn_c))
        add_node((p, q), ai + aj, ci - cj, (mi + 2) % 3)
        cross = product(np.outer(sa[:, 0], ai) + np.outer(sa[:, 1], aj),
                        np.outer(sc[:, 0], cj) + np.outer(sc[:, 1], ci))

        def turned(m, t, products):
            want = np.outer(sa @ forms[m, t, 0], sc @ forms[m, t, 1])
            return next(v for v, (f, g) in zip(products, forms[(m + mi) % 3]) if (np.outer(f, g) == want).all())

        dv = node[p, q][3]
        ij = cross - turned(2, 1, dv) - turned(1, 0, dj) + turned(0, 1, di)
        ji = cross + turned(2, 0, dv) - turned(0, 0, di) + turned(1, 1, dj)
        return (ji, ij) if swap else (ij, ji)

    for i in range(n):
        add_node(i, eye[i], eye[i], method[i])
        inner[i, i] = sum(node[i][3])
    for i, j in itertools.combinations(range(n), 2):
        if method[i] != method[j]:
            inner[i, j], inner[j, i] = pair(i, j)
    for (i, j), (u, k) in sorted(stand_in.items()):
        v, w = (min(u, k), max(u, k)), i + j - u
        vw, wv = pair(v, w)
        inner[u, w] = vw - inner[k, w]
        inner[w, u] = node[v][1][u] * wv + inner[w, k]
    lhs, out = np.array(lhs), np.array(out)
    rhs = np.array([[inner[i, j] for j in range(n)] for i in range(n)]).transpose(2, 0, 1)
    assert (np.einsum("pri,pjk,psl->rijksl", lhs, rhs, out)
            == np.einsum("rs,ij,kl->rijksl", np.eye(2, dtype=int), eye, eye)).all()

    used = [sorted(p for g, d in zip(groups, text) for p in g if p != g[int(d)]) for text in left_out]
    steps = []
    for s, products in enumerate(used):
        basis = rhs[products].reshape(n * n, n * n)
        dual = np.rint(np.linalg.inv(basis).T).astype(int)
        assert (basis.T @ dual == np.eye(n * n)).all()
        entries = []
        for p, u in zip(products, dual.reshape(-1, n, n)):
            i, j = np.argwhere(u)[0]
            mem_lhs, mem_out = u[:, j] * u[i, j], u[i]
            assert (np.outer(mem_lhs, mem_out) == u).all()
            when = [t for t in range(PERIOD) if p in used[t]]
            halves = (0, 1) if len(when) == 1 else (when.index(s),)
            entries.append((p, halves, mem_lhs, mem_out))
        steps.append(entries)

    def locality(p):
        idx = np.nonzero(np.abs(out[p]).sum(0))[0]
        a, b = idx.min() // 2, idx.max() // 2
        return (a, -b if a % 2 else b, tuple(idx))

    steps = [sorted(e, key=lambda t: (t[1] == (1,), locality(t[0]))) for e in steps]
    return lhs, rhs, out, steps, sorted(range(len(lhs)), key=locality)


_HK_LHS, _HK_RHS, _HK_OUT, _HK_STEPS, _HK_ORDER = _hopcroft_kerr()
NB, NPROD = _HK_RHS.shape[1], _HK_RHS.shape[0]


def _share(jobs, k, n):
    return jobs[len(jobs) * k // n:len(jobs) * (k + 1) // n]


def _mix(*lists):
    keyed = [((n + 0.5) / len(l), k, n) for k, l in enumerate(lists) for n in range(len(l))]
    return [lists[k][n] for _, k, n in sorted(keyed)]


def _jobs(fn, *ranges):
    return [functools.partial(fn, *k) for k in itertools.product(*ranges)]


def _run(jobs):
    for job in jobs:
        job(lambda v: v)


def _never(ref):
    return jnp.abs(ref[0:SUB, 0:LANES].astype(F32)) < 0.0


class _Pacer:
    def __init__(self, never):
        self.never = never
        self.tokens = []

    def dot(self, a, b):
        m = _dot(a, b)
        rounds = min(max(a.shape[1] * m.shape[1] // (4 * LANES * LANES), 1), m.shape[1] // LANES)
        self.tokens += [
            m[r:r + SUB, c:c + LANES]
            for c in range(0, m.shape[1], m.shape[1] // rounds) for r in range(0, m.shape[0], SUB)
        ]
        return m

    def run(self, *job_lists):
        tokens, self.tokens = self.tokens, []

        def gate(k, count, v):
            n = v.shape[0] // SUB
            rows = []
            for r in range(n):
                t = lax.bitcast_convert_type(tokens[len(tokens) * (k * n + r) // (count * n)], v.dtype)
                rows.append(jnp.concatenate([
                    jnp.where(self.never, t, v[r * SUB:(r + 1) * SUB, c:c + LANES])
                    for c in range(0, v.shape[1], LANES)], axis=1))
            return jnp.concatenate(rows, axis=0)

        due = []
        for job in _mix(*[
            [functools.partial(job, functools.partial(gate, k, len(jobs))) for k, job in enumerate(jobs)]
            for jobs in job_lists
        ]):
            due += job() or []
        return due

    def before(self, a, due):
        rows = [a[r:r + SUB] for r in range(0, a.shape[0], SUB)]
        for n, v in enumerate(due):
            r = len(rows) // 2 + n * len(rows) // 2 // len(due)
            rows[r] = jnp.concatenate([jnp.where(self.never, v, rows[r][:, :LANES]), rows[r][:, LANES:]], axis=1)
        return jnp.concatenate(rows, axis=0)


def _rhs(w, i):
    n = w.shape[0] // 7
    return jnp.concatenate([_get_wide(w, n * i + k) for k in range(n)], axis=0)


def _strassen(block, w, pacer, side, spread):
    c, due = {}, [[], []]
    for n, i in enumerate(_ORDER):
        m = pacer.dot(pacer.before(_combine(_LHS[i], block), due.pop(0)).astype(BF16), _rhs(w, i))
        due.append(pacer.run(_share(side, n, spread) if n < spread else []))
        _scatter(c, _OUT[i], m)
    return c


def _rhs_jobs(dst, src, which=range(7)):
    kh, nh, rows = src.shape[0] // 2, src.shape[1] // 2, 64

    def job(c, k0, gate):
        @functools.cache
        def block(a, b):
            return gate(src[pl.ds(a * kh + k0, rows), pl.ds(b * nh + c * LANES, LANES)].astype(F32))

        for i in which:
            k, r = divmod((i * kh + k0) // 2, dst.shape[2])
            _put(dst, (k, c, pl.ds(r, rows // 2)), _combine(_RHS[i], block))

    return _jobs(job, range(nh // LANES), range(0, kh, rows))


def _rhs2_jobs(dst, src):
    kq, nq = src.shape[0] // 4, src.shape[1] // 4

    @functools.cache
    def block(c, k0, a, b):
        return src[pl.ds(a * kq + k0, PACK), pl.ds(b * nq + c * LANES, LANES)].astype(F32)

    def job(c, k0, i, gate):
        outer = functools.cache(lambda a, b: gate(_combine(_RHS[i], lambda u, v: block(c, k0, 2 * u + a, 2 * v + b))))
        for j in range(7):
            _put(dst, (7 * i + j, c, pl.ds(k0 // 2, SUB)), _combine(_RHS[j], outer))

    return _jobs(job, range(nq // LANES), range(0, kq, PACK), range(7))


def _hk_jobs(block, store):
    def job(p, gate):
        first = tuple(np.argwhere(_HK_RHS[p])[0])
        store(p, _combine(_HK_RHS[p], lambda i, j: gate(block(i, j)) if (i, j) == first else block(i, j)))

    return _jobs(job, _HK_ORDER)


def _kernel(
    x_hbm, mem_hbm, wq_hbm, wk_hbm, wv_hbm, wo_hbm, w1_hbm, w2_hbm, w3_hbm, w4_hbm,
    out_hbm,
    xb, xn, macc, wqkv, wo, raw_o, mem0, sem_m, sem_o,
    *, S, D, H, DH, M, SEG, F,
):
    HD = D // 2
    NCB = D // LANES
    NG = H // NB
    T1 = 2 * R1
    NT = S // T1
    NF = F // FC
    assert LANES // PACK == NF + 1

    mem_copy = pltpu.make_async_copy(mem_hbm, mem0, sem_m)

    def wo_copy(part):
        rows = pl.ds(pl.multiple_of(part * PACK, PACK), PACK)
        return pltpu.make_async_copy(wo_hbm.at[:, rows], raw_o.at[part % 2], sem_o.at[part % 2])

    def wo_jobs(part):
        dst = wo.at[:, :, pl.ds(pl.multiple_of(part * SUB, SUB), SUB)]
        src = raw_o.at[part % 2]

        def group(g):
            block = functools.cache(lambda i, j: src[g * NB + i, :, pl.ds(j * LANES, LANES)].astype(F32))
            return _hk_jobs(block, lambda p, v: _put(dst, (p, g), v))

        return [job for g in range(NG) for job in group(g)]

    def mixer(yc, w3c, r3, r4, raw, mid, sem_f, sem_a):
        def w3_copy(f):
            cols = pl.ds(pl.multiple_of(f * FC, FC), FC)
            return pltpu.make_async_copy(w3_hbm.at[:, cols], r3.at[f % 2], sem_f.at[0, f % 2])

        def w4_copy(f):
            rows = pl.ds(pl.multiple_of(f * FC, FC), FC)
            return pltpu.make_async_copy(w4_hbm.at[rows], r4.at[f % 2], sem_f.at[1, f % 2])

        def qkv_copy(part, w):
            rows = pl.ds(pl.multiple_of(part * PACK * H, PACK * H), PACK * H)
            return pltpu.make_async_copy(
                (wq_hbm, wk_hbm, wv_hbm)[w].at[:, rows], raw.at[part % 2, w], sem_a.at[part % 2, w])

        def qkv_jobs(part):
            dst = wqkv.at[:, :, :, pl.ds(pl.multiple_of(part * SUB, SUB), SUB)]
            src = raw.at[part % 2]

            def transpose(w, half, i, gate):
                rows = gate(jnp.concatenate([
                    pltpu.bitcast(src[w, i, pl.ds(d * H + half * PACK, PACK), :], U32) for d in range(PACK)], axis=0))
                for d in range(PACK):
                    mid[w, i, pl.ds(half * SUB * (PACK + 1) + d, SUB, stride=PACK + 1), :] = rows[d * SUB:(d + 1) * SUB]

            def group(w, g):
                words = functools.cache(lambda i, pair: mid[w, i, pl.ds((g * NB // 2 + pair) * (PACK + 1), PACK), :])
                block = functools.cache(lambda i, j: pltpu.bitcast(
                    words(i, j // 2) & jnp.uint32(0xFFFF0000) if j % 2 else words(i, j // 2) << 16, F32))
                return _hk_jobs(block, lambda p, v: _put(dst, (p, w, g), v))

            units = list(itertools.product(range(3), range(H // PACK)))
            moves = [_jobs(transpose, [w], [half], range(NB)) for w, half in units] + [[]]
            sums = [[]] + [group(w, 2 * half) + group(w, 2 * half + 1) for w, half in units]
            return [job for a, b in zip(moves, sums) for job in _mix(a, b)]

        def w3_jobs(f):
            return _rhs2_jobs(w3c.at[f % 2], r3.at[f % 2])

        def token_mixing(r12, y0, c1, c2, hb, sem_x, sem_w):
            w1c, w2c = (wo.at[pl.ds(n * 7 * HD // LANES, 7 * HD // LANES)] for n in range(2))
            shifts = (-1, 1, -2, 2)

            def x_copy(t):
                rows = pl.ds(pl.multiple_of(t * T1, T1), T1)
                return pltpu.make_async_copy(x_hbm.at[rows], xb.at[rows], sem_x.at[t])

            def w1_copy(a, b):
                idx = (pl.ds(a * HD, HD), pl.ds(b * HD, HD))
                return pltpu.make_async_copy(w1_hbm.at[idx], r12.at[(0,) + idx], sem_w.at[2 * a + b])

            w2_copy = pltpu.make_async_copy(w2_hbm, r12.at[1], sem_w.at[4])

            def tile(ref, t):
                return ref.at[pl.ds(pl.multiple_of(t * T1, T1), T1)]

            def normalizing(t, slot):
                xb_t, xn_t = tile(xb, t), tile(xn, t)

                def job(lo, a, gate):
                    rows = pl.ds(a * R1 + lo, 2 * PACK)
                    n, var = _layernorm(gate(xb_t[rows, :].astype(F32)))
                    xn_t[rows, :] = n.astype(BF16)
                    y = n * lax.rsqrt(var + EPS)
                    y0[slot, a, pl.ds(lo, 2 * PACK), :] = y
                    return [y[r:r + SUB, :LANES] for r in range(0, 2 * PACK, SUB)]

                return _jobs(job, range(0, R1, 2 * PACK), range(2))

            def keep(dst, c):
                for (a, b), v in c.items():
                    dst[a, :, pl.ds(b * HD, HD)] = v

            def block1(slot):
                return lambda a, b: y0[slot, a, :, pl.ds(b * HD, HD)]

            def stage1(slot, side):
                keep(c1, _strassen(block1(slot), w1c, pacer, side, 6))

            def activating(t):
                hb_t = hb.at[:, pl.ds(pl.multiple_of(SUB + t * T1, SUB), T1)]

                def job(a, c, gate):
                    hb_t[c, pl.ds(a * R1, R1), :] = 0.5 * _gelu2(gate(c1[a, :, pl.ds(c * LANES, LANES)]))

                return _jobs(job, range(2), range(NCB))

            def stage2(t, side):
                hb_t = hb.at[:, pl.ds(pl.multiple_of(t * T1, SUB), T1 + 2 * SUB)]
                keep(c2, _strassen(lambda a, b: jnp.concatenate([
                    hb_t[c, pl.ds(SUB + a * R1 + shifts[c * 4 // NCB], R1), :]
                    for c in range(b * NCB // 2, (b + 1) * NCB // 2)], axis=1), w2c, pacer, side, 5))

            def renormalizing(t):
                xb_t, xn_t = tile(xb, t), tile(xn, t)
                acc_t = macc.at[:, pl.ds(pl.multiple_of(t * R1, R1), R1)]
                if YPRE:
                    yc_t = yc.at[:, :, pl.ds(pl.multiple_of(t * (R1 // 4), R1 // 4), R1 // 4)]
                else:
                    yc_t = yc.at[:, pl.ds(pl.multiple_of(t * R1, R1), R1)]
                first = {}

                def job(lo, k, gate):
                    x1, z = [], []
                    for a in range(2):
                        rows = pl.ds(a * R1 + k * RU + lo, PACK)
                        x1.append(xn_t[rows, :].astype(F32) + gate(c2[a, pl.ds(k * RU + lo, PACK), :]))
                        z.append(2.0 * (x1[a] + xb_t[rows, :].astype(F32)))
                    z11, z12, z21, z22 = z[0][:, :HD], z[0][:, HD:], z[1][:, :HD], z[1][:, HD:]
                    for i, v in ((6, z11), (2, z12), (1, z21), (5, z22 - z12 + z21)):
                        acc_t[i, pl.ds(k * RU + lo, PACK), :] = v
                    y, _ = _layernorm(jnp.concatenate(x1, axis=0))
                    for i in range(7):
                        v = _combine(_LHS[i], lambda a, b: y[a * PACK:(a + 1) * PACK, b * HD:(b + 1) * HD])
                        if not YPRE:
                            yc_t[i, pl.ds(k * RU + lo, PACK), :] = v
                            continue
                        first[i, k] = v
                        for j in range(7):
                            if k == int(_LHS[j, 1].any()):
                                u = _combine(_LHS[j], lambda a, b: first[i, a][:, b * HD // 2:(b + 1) * HD // 2])
                                for c in range(NCB // 4):
                                    _put(yc_t, (7 * i + j, c, pl.ds(lo // 2, SUB)), _lanes(u, c))
                    return [y[r:r + SUB, :LANES] for r in range(0, 2 * PACK, SUB)]

                return _jobs(job, range(0, RU, PACK), range(2))

            arrival = (((0, 0), (1,)), ((1, 1), (4, 0)), ((0, 1), (2, 5)), ((1, 0), (3, 6)))
            queue = [w1_copy(*q) for q, _ in arrival] + [x_copy(1), x_copy(2)]
            x_copy(0).start()
            queue.pop(0).start()
            for c in range(NCB):
                hb[c, pl.ds(0, SUB), :] = jnp.zeros((SUB, LANES), F32)
                hb[c, pl.ds(SUB + S, SUB), :] = jnp.zeros((SUB, LANES), F32)
            for i in (0, 3, 4):
                macc[i] = jnp.zeros(macc.shape[1:], F32)
            pad = xn.shape[0] - S
            xn[pl.ds(S, pad), :] = jnp.zeros((pad, D), BF16)
            with _scope("wait_x0"):
                x_copy(0).wait()
            queue.pop(0).start()
            pacer = _Pacer(_never(xb))
            with _scope("tile0"):
                _run(normalizing(0, 1))
                c = {}
                for q, ready in arrival:
                    w1_copy(*q).wait()
                    queue.pop(0).start()
                    _run(_rhs_jobs(w1c, r12.at[0], ready))
                    for i in ready:
                        _scatter(c, _OUT[i], _dot(_combine(_LHS[i], block1(1)).astype(BF16), _rhs(w1c, i)))
                keep(c1, c)
                x_copy(1).wait()
                w2_copy.start()
                _run(normalizing(1, 0))
            with _scope("tile1"):
                x_copy(3).start()
                x_copy(2).wait()
                stage1(0, _mix(activating(0), normalizing(2, 1)))
                x_copy(4).start()
                mem_copy.start()
                w2_copy.wait()
                x_copy(3).wait()
                stage1(1, _mix(activating(1), _rhs_jobs(w2c, r12.at[1])))
                stage2(0, normalizing(3, 0))

            def slot(u, carry):
                @pl.when(u + 1 < NT)
                def _():
                    x_copy(u + 1).wait()

                @pl.when(u + 2 < NT)
                def _():
                    x_copy(u + 2).start()

                @pl.when(u < 5)
                def _():
                    w3_copy(u - 3).start()

                @pl.when(u == 5)
                def _():
                    w4_copy(0).start()
                    wo_copy(0).start()

                @pl.when(u >= NT - 2)
                def _():
                    for w in range(3):
                        qkv_copy(u - (NT - 2), w).start()

                with _scope("slot"):
                    again = renormalizing(u - 3)
                    stage1(0, _mix(activating(u - 1), again[:SPLIT[0]]) + again[SPLIT[0]:SPLIT[1]])
                    stage2(u - 2, _mix(normalizing(jnp.minimum(u + 1, NT - 1), 0), again[SPLIT[1]:]))
                return carry

            lax.fori_loop(3, NT, slot, 0)
            w3_copy(0).wait()
            for w in range(3):
                qkv_copy(0, w).wait()
            with _scope("tile7"):
                last = activating(NT - 1)
                halo = [c for c in range(NCB) if shifts[c * 4 // NCB] > 0]
                _run([last[c] for c in halo])
                late = _mix(w3_jobs(0), qkv_jobs(0))
                stage2(NT - 2, _mix(
                    renormalizing(NT - 3), [job for c, job in enumerate(last) if c not in halo], _share(late, 0, 3)))
                stage2(NT - 1, _mix(renormalizing(NT - 2), _share(late, 1, 3) + _share(late, 2, 3)))
                _run(renormalizing(NT - 1))

        def ffn(w4c, g):
            N3 = S // 2 // R3
            never = _never(xb)

            def chunk(f, carry):
                @pl.when(f + 2 < NF)
                def _():
                    w3_copy(f + 2).start()

                @pl.when(f + 1 < NF)
                def _():
                    w4_copy(f + 1).start()
                    for w in range(3):
                        qkv_copy(f + 2, w).start()
                    w3_copy(f + 1).wait()

                wo_copy(f + 1).start()
                for w in range(3):
                    qkv_copy(f + 1, w).wait()
                w4_copy(f).wait()
                wo_copy(f).wait()
                pacer = _Pacer(never)
                w3f = w3c.at[f % 2]
                pre = {}

                def up(t, *side):
                    for s in range(t * R3 // (2 * RU), (t + 1) * R3 // (2 * RU)):
                        c = pre[s] = {}
                        for i in _ORDER:
                            block = functools.cache(
                                lambda a, b: yc[i, pl.ds((2 * s + a) * RU, RU), pl.ds(b * HD // 2, HD // 2)])
                            inner = {}
                            for j in _ORDER:
                                if YPRE:
                                    a = _get_wide(yc, 7 * i + j, pl.ds(s * RU // 2, RU // 2))
                                else:
                                    a = _combine(_LHS[j], block).astype(BF16)
                                _scatter(inner, _OUT[j], pacer.dot(a, _get_wide(w3f, 7 * i + j)))
                            for q, v in inner.items():
                                _scatter(c, _OUT[i], v, q)
                    pacer.run(*side)

                def activating(t):
                    def job(k, a, lo, gate):
                        for u, v, b in itertools.product(range(2), repeat=3):
                            g[t % 2, u, pl.ds((2 * k + a) * RU + lo, RD), pl.ds((2 * v + b) * FC // 4, FC // 4)] = (
                                _gelu2(gate(pre[t * R3 // (2 * RU) + k][u, v, a, b][lo:lo + RD])))

                    return _jobs(job, range(R3 // (2 * RU)), range(2), range(0, RU, RD))

                def down(t, *side):
                    for s in range(R3 // (2 * RD)):
                        for i in _ORDER:
                            outer = functools.cache(lambda a, b: _combine(_LHS[i], lambda u, v: g[
                                t % 2, u, pl.ds((2 * s + a) * RD, RD), pl.ds((2 * v + b) * FC // 4, FC // 4)]))
                            where = {
                                (a, b): (i, pl.ds(t * R3 + (2 * s + a) * RD, RD), pl.ds(b * HD // 2, HD // 2))
                                for a in range(2) for b in range(2)
                            }
                            acc = {k: macc[idx] for k, idx in where.items()}
                            for j in _ORDER:
                                a = _combine(_LHS[j], outer).astype(BF16)
                                _scatter(acc, _OUT[j], pacer.dot(a, _get_wide(w4c, 7 * i + j)))
                            for k, idx in where.items():
                                macc[idx] = acc[k]
                    pacer.run(*side)

                side = [qkv_jobs(f + 1), wo_jobs(f)]
                w3j = w3_jobs(f + 1)
                total = WU * (N3 - 2) + WD * (N3 - 1) + WE + W1
                at = 0

                def take(n):
                    nonlocal at
                    at += n
                    return [l[len(l) * (at - n) // total:len(l) * at // total] for l in side]

                with _scope("chunk"):
                    up(0, _rhs2_jobs(w4c, r4.at[f % 2]))
                    up(1, activating(0), *take(W1))
                    for t in range(N3 - 2):
                        down(t, activating(t + 1), *take(WD), _share(w3j, t, N3))
                        up(t + 2, *take(WU))
                    down(N3 - 2, activating(N3 - 1), *take(WD), _share(w3j, N3 - 2, N3))
                    down(N3 - 1, *take(WE), _share(w3j, N3 - 1, N3))
                return carry

            lax.fori_loop(0, NF, chunk, 0)

        if "1" in PARTS:
            pl.run_scoped(
                token_mixing,
                pltpu.VMEM((2, D, D), BF16),
                pltpu.VMEM((2, 2, R1, D), F32),
                pltpu.VMEM((2, R1, D), F32),
                pltpu.VMEM((2, R1, D), F32),
                pltpu.VMEM((NCB, S + 2 * SUB, LANES), F32),
                pltpu.SemaphoreType.DMA((NT,)),
                pltpu.SemaphoreType.DMA((5,)),
            )
        if "3" in PARTS:
            pl.run_scoped(
                ffn,
                _words(49, NCB // 4, FC // 8),
                pltpu.VMEM((2, 2, R3, FC), F32),
            )
        else:
            k = xb[0:8, 0:128].astype(jnp.int32)[0, 0]
            xb[0:16, 0:128] = (yc[k, k, 0:16] if YPRE else yc[k, 0:16, 0:128]).astype(F32).astype(BF16) + w3c[k, k, k, 0:16].astype(F32).astype(BF16)

    def recurrence(base, gq, fq, ob, oc, go, sem_out):
        L = M + SEG
        PR = PERIOD * SEG
        HR = PR // 2
        QR = PR // 4
        NPER = (S // SEG - 1) // PERIOD
        assert NPER * PR + SEG == S
        scale = DH ** -0.5
        row = lax.broadcasted_iota(jnp.int32, (L, L), 0)
        col = lax.broadcasted_iota(jnp.int32, (L, L), 1)
        mask = (row < M) | (row >= col)

        def out_copy(r0, n):
            return pltpu.make_async_copy(xb.at[pl.ds(r0, n)], out_hbm.at[pl.ds(r0, n)], sem_out)

        def emit(r0):
            xb[pl.ds(r0, PR), :] = (base[pl.ds(r0, PR), :] + go[...]).astype(BF16)

        def quarter(a, halves):
            return pl.ds(a * HR + halves[0] * QR, len(halves) * QR)

        wo_copy(NF).wait()
        mem_copy.wait()
        with _scope("a_pro"):
            pacer = _Pacer(_never(xb))

            def collect(lo, gate):
                c = {}
                for i in _ORDER:
                    v = macc[i, pl.ds(lo, PACK), :]
                    _scatter(c, _OUT[i], gate(v) if i < 3 else v)
                t, r = divmod(lo, R1)
                for (a, b), v in c.items():
                    base[pl.ds(t * T1 + a * R1 + r, PACK), pl.ds(b * HD, HD)] = 0.5 * v

            tokens = xn[pl.ds(0, PR), :].astype(F32)
            lhs = {p: _combine(_HK_LHS[p], lambda a, i: _lanes(tokens, i)[a * HR:(a + 1) * HR]).astype(BF16)
                   for p in _HK_ORDER}
            for w, g in itertools.product(range(3), range(NG)):
                c = {}
                for p in _HK_ORDER:
                    _scatter(c, _HK_OUT[p], pacer.dot(lhs[p], _get(wqkv, (p, w, g))))
                for (a, j), v in c.items():
                    gq[w, g * NB + j, pl.ds(a * HR, HR), :] = v
            pacer.run(wo_jobs(NF), _jobs(collect, range(0, S // 2, PACK)))
            ob[...] = jnp.zeros(ob.shape, F32)
            go[...] = jnp.zeros(go.shape, F32)

        def period(it, mem):
            done = pl.multiple_of(jnp.maximum(it - 2, 0) * PR, PR)
            tokens = xn[pl.ds(pl.multiple_of((it + 1) * PR, PR), PR), :].astype(F32)
            emit(done)
            for step in range(PERIOD):
                mem = segment(step, tokens, mem)

            @pl.when(it >= 2)
            def _():
                out_copy(done, PR).start()

            return mem

        def segment(step, tokens, mem):
            entries = _HK_STEPS[step]
            rows = pl.ds(step * SEG, SEG)
            begun = {
                k + (half,)
                for p, halves, _, _ in itertools.chain(*_HK_STEPS[:step])
                for half in halves for k, c in np.ndenumerate(_HK_OUT[p]) if c
            }

            def operand(entry, mem_block, token_block):
                p, halves, mem_lhs, _ = entry
                a = jnp.concatenate([
                    _combine(mem_lhs, mem_block),
                    _combine(_HK_LHS[p], lambda a, i: token_block(quarter(a, halves), i))], axis=0)
                return a if a.shape[0] % PACK else a.astype(BF16)

            def fold(entry, r, mem_acc, token_acc, partial):
                p, halves, _, mem_out = entry
                _scatter(mem_acc, mem_out, r[:M])
                for n, half in enumerate(halves):
                    _scatter(token_acc, _HK_OUT[p], r[M + n * QR:M + (n + 1) * QR], (half,),
                             lambda a, j, h: partial(quarter(a, (h,)), j) if (a, j, h) in begun else None)

            lhs = [
                operand(e, lambda i: _lanes(mem, i), lambda r, i: _lanes(tokens, i)[r.start:r.start + r.size])
                for e in entries
            ]
            qkv_mem, prob, att_mem, new_mem, out_acc = {}, {}, {}, {}, {}

            def project(g, w):
                if step == 0:
                    for h in range(g * NB, (g + 1) * NB):
                        fq[w, h] = gq[w, h]
                        if w == 0:
                            oc[h] = ob[h]
                mem_acc, token_acc = {}, {}

                def one(a, e):
                    fold(e, _dot(a, _get(wqkv, (e[0], w, g))), mem_acc, token_acc, lambda r, j: gq[w, g * NB + j, r, :])

                def finish():
                    for (a, j, half), v in token_acc.items():
                        gq[w, g * NB + j, quarter(a, (half,)), :] = v
                    for (j,), v in mem_acc.items():
                        qkv_mem[w, g * NB + j] = v

                return [functools.partial(one, a, e) for a, e in zip(lhs, entries)] + [finish]

            def part(w, h):
                return jnp.concatenate([qkv_mem[w, h], fq[w, h, rows, :]], axis=0)

            def scores(h):
                prob[h] = _softmax_rows(part(0, h), part(1, h), mask, scale)

            def attend(h):
                o = _dot(prob[h], part(2, h))
                att_mem[h] = o[:M]
                ob[h, rows, :] = o[M:]

            def outproj(g, e):
                a = operand(e, lambda i: att_mem[g * NB + i], lambda r, i: oc[g * NB + i, r, :])
                fold(e, _dot(a, _get(wo, (e[0], g))), new_mem, out_acc, lambda r, j: go[r, pl.ds(j * LANES, LANES)])

            def heads(fn, g):
                return _jobs(fn, range(g * NB, (g + 1) * NB))

            def play(*lists):
                for job in _mix(*lists):
                    job()

            todo = _jobs(outproj, range(NG), entries)
            early = len(todo) - len(entries) - sum(TAIL)
            at = 0
            for g in range(NG):
                play(project(g, 0))
                play(project(g, 1), heads(attend, g - 1) if g else [])
                values = project(g, 2)
                lead = len(values) // (4 if g == NG - 1 else 2)
                play(values[:lead])
                play(values[lead:lead + len(values) // 2], heads(scores, g))
                play(values[lead + len(values) // 2:])
                play(todo[at:min(early, g * len(entries))])
                at = min(early, g * len(entries))
            play(todo[at:at + TAIL[0]])
            play(todo[at + TAIL[0]:at + sum(TAIL)], heads(attend, NG - 1))
            play(todo[at + sum(TAIL):])
            for (a, j, half), v in out_acc.items():
                go[quarter(a, (half,)), pl.ds(j * LANES, LANES)] = v
            return jnp.concatenate([new_mem[j,] for j in range(NB)], axis=1)

        with _scope("a_loop"):
            mem = lax.fori_loop(0, NPER, period, mem0[...].astype(F32))

        with _scope("a_epi"):
            emit((NPER - 2) * PR)
            out_copy((NPER - 2) * PR, PR).start()
            rows = pl.ds(0, SEG)
            ER = (PR + SEG) // 2
            lhs = [_combine(e[2], lambda i: _lanes(mem, i)) for e in _HK_STEPS[0]]
            kv_mem, prob, att, out_acc = {}, {}, {}, {}

            def project(w, g):
                acc = {}
                for a, (p, _, _, mem_out) in zip(lhs, _HK_STEPS[0]):
                    _scatter(acc, mem_out, _dot(a, _get(wqkv, (p, w, g))))
                for (j,), v in acc.items():
                    kv_mem[w, g * NB + j] = jnp.concatenate([v, gq[w, g * NB + j, rows, :]], axis=0)

            def block(a, h):
                if a == 0:
                    return ob[h, pl.ds(0, ER), :]
                return jnp.concatenate([ob[h, pl.ds(ER, PR - ER), :], att[h]], axis=0)

            for t in range(NG + 2):
                if t < NG:
                    project(1, t)
                    project(2, t)
                    for h in range(t * NB, (t + 1) * NB):
                        prob[h] = _softmax_rows(gq[0, h, rows, :], kv_mem[1, h], mask[M:], scale)
                if 0 <= t - 2:
                    for p in _HK_ORDER:
                        a = _combine(_HK_LHS[p], lambda a, i: block(a, (t - 2) * NB + i))
                        _scatter(out_acc, _HK_OUT[p], _dot(a, _get(wo, (p, t - 2))))
                if 0 <= t - 1 < NG:
                    for h in range((t - 1) * NB, t * NB):
                        att[h] = _dot(prob[h], kv_mem[2, h])
            r0 = (NPER - 1) * PR
            for a in range(2):
                done = pl.ds(r0 + a * ER, ER)
                xb[done, :] = (base[done, :] + jnp.concatenate([out_acc[a, j] for j in range(NB)], axis=1)).astype(BF16)
            out_copy(r0, 2 * ER).start()
        with _scope("tail"):
            out_copy(0, S).wait()

    if "1" in PARTS or "3" in PARTS:
        pl.run_scoped(
            mixer,
            _words(49, NCB // 4, S // 8) if YPRE else pltpu.VMEM((7, S // 2, HD), F32),
            _words(2, 49, FC // 4 // LANES, HD // 4),
            pltpu.VMEM((2, D, FC), BF16),
            pltpu.VMEM((2, FC, D), BF16),
            pltpu.VMEM((2, 3, NB, PACK * H, LANES), BF16),
            _words(3, NB, H // 2 * (PACK + 1)),
            pltpu.SemaphoreType.DMA((2, 2)),
            pltpu.SemaphoreType.DMA((2, 3)),
        )
    if "A" not in PARTS:
        k = xb[0:8, 0:128].astype(jnp.int32)[0, 0]
        k16 = pl.ds(pl.multiple_of(k * 16, 16), 16)
        xb[0:16, 0:128] = (_get(wqkv, (k, k, k, pl.ds(0, 8))) + _get(wo, (k, k, pl.ds(0, 8)))
                           + xn[k16, 0:128] + macc[k, k16, 0:128].astype(BF16))
        pltpu.sync_copy(xb, out_hbm)
        return
    pl.run_scoped(
        recurrence,
        pltpu.VMEM((S, D), F32),
        pltpu.VMEM((3, H, PERIOD * SEG, DH), F32),
        pltpu.VMEM((3, H, PERIOD * SEG, DH), F32),
        pltpu.VMEM((H, PERIOD * SEG, DH), F32),
        pltpu.VMEM((H, PERIOD * SEG, DH), F32),
        pltpu.VMEM((PERIOD * SEG, D), F32),
        pltpu.SemaphoreType.DMA(()),
    )


@functools.partial(jax.jit, static_argnames=("A_seg_len",))
def pallas_parallel_sum__memory_aug_recurrent_mem_tr__mixer_s_mlp__prompt_kernel(
    A_x: jax.Array,
    A_mem0: jax.Array,
    A_Wq: jax.Array,
    A_Wk: jax.Array,
    A_Wv: jax.Array,
    A_Wo: jax.Array,
    A_seg_len: int,
    B_x: jax.Array,
    B_w1: jax.Array,
    B_w2: jax.Array,
    B_w3: jax.Array,
    B_w4: jax.Array,
):
    del B_x
    B, S, D = A_x.shape
    _, H, DH = A_Wq.shape
    M = A_mem0.shape[1]
    F = B_w3.shape[1]
    SEG = int(A_seg_len)
    assert B == 1 and DH == LANES and D == NB * LANES

    hbm = pl.BlockSpec(memory_space=pl.ANY)
    out = pl.pallas_call(
        functools.partial(_kernel, S=S, D=D, H=H, DH=DH, M=M, SEG=SEG, F=F),
        out_shape=jax.ShapeDtypeStruct((S, D), A_x.dtype),
        in_specs=[hbm] * 10,
        out_specs=hbm,
        scratch_shapes=[
            pltpu.VMEM((S, D), BF16),
            pltpu.VMEM((S + (PERIOD - 1) * SEG, D), BF16),
            pltpu.VMEM((7, S // 2, D // 2), F32),
            _words(NPROD, 3, H // NB, LANES // 2),
            _words(NPROD, H // NB, LANES // 2),
            pltpu.VMEM((2, H, PACK, D), BF16),
            pltpu.VMEM((M, D), BF16),
            pltpu.SemaphoreType.DMA(()),
            pltpu.SemaphoreType.DMA((2,)),
        ],
        compiler_params=pltpu.CompilerParams(vmem_limit_bytes=127 * 1024 * 1024, flags=FLAGS),
    )(
        A_x.reshape(S, D),
        A_mem0.reshape(M, D),
        A_Wq.reshape(NB, LANES * H, DH),
        A_Wk.reshape(NB, LANES * H, DH),
        A_Wv.reshape(NB, LANES * H, DH),
        A_Wo,
        B_w1, B_w2, B_w3, B_w4,
    )
    return out.reshape(B, S, D)
```

```python
import contextlib
import functools
import itertools
import math

import jax
import jax.numpy as jnp
import numpy as np
from jax import lax
from jax.experimental import pallas as pl
from jax.experimental.pallas import tpu as pltpu

F32 = jnp.float32
BF16 = jnp.bfloat16
U32 = jnp.uint32
LANES = 128
SUB = 8
PACK = 16
EPS = 1e-5
R1 = 128
RU = 64
RD = 32
R3 = 256
FC = 512
PERIOD = 3
WU, WD, WE, W1 = 5, 1, 2, 3
TAIL = (32, 32)
NS = 2
RS = 1
W3S = 3
SCOPES = False
PARTS = "13A"
FLAGS = None


def _scope(name):
    return jax.named_scope(name) if SCOPES else contextlib.nullcontext()


def _layernorm_jobs(read, count, finish, slack):
    mean, var = {}, {}

    def first(k, gate):
        mean[k] = jnp.mean(read(0, k, gate), axis=-1, keepdims=True)

    def second(k, gate):
        d = read(1, k, gate) - mean[k]
        var[k] = jnp.mean(d * d, axis=-1, keepdims=True)

    def idle(gate):
        pass

    last = [finish(k, mean, var) for k in range(count)]
    n = len(last[0])
    return [
        _jobs(first, range(count)) + [idle] * (2 + slack),
        [idle] + _jobs(second, range(count)) + [idle] * (1 + slack),
        [idle] * 2 * n + list(itertools.chain(*last)) + [idle] * slack * n,
    ]


def _gate_first(gate, v):
    return jnp.concatenate([gate(v[:, :LANES]), v[:, LANES:]], axis=1)


def _gelu2(x):
    c = math.sqrt(2 / math.pi)
    return x + x * jnp.tanh(x * (c + (c * 0.044715) * (x * x)))


def _softmax_rows(q, k, mask, scale):
    z = lax.dot_general(q, k, (((1,), (1,)), ((), ())), preferred_element_type=F32)
    z = jnp.where(mask, z * scale, -1e9)
    e = jnp.exp(z - jnp.max(z, axis=-1, keepdims=True))
    s = jnp.sum(e, axis=-1, keepdims=True)
    r = pl.reciprocal(s, approx=True)
    return e * (r * (2.0 - s * r))


def _dot(a, b):
    return jnp.dot(a, b, preferred_element_type=F32)


def _put(ref, idx, v):
    ref[idx] = pltpu.bitcast(v.astype(BF16), U32)


def _get(ref, idx):
    return pltpu.bitcast(ref[idx], BF16)


def _get_wide(ref, i, rows=slice(None)):
    return jnp.concatenate([_get(ref, (i, c, rows)) for c in range(ref.shape[1])], axis=1)


def _words(*shape):
    return pltpu.VMEM(shape + (LANES,), U32)


def _lanes(v, c):
    return v[:, c * LANES:(c + 1) * LANES]


def _combine(coef, get):
    terms = sorted(((int(c), k) for k, c in np.ndenumerate(coef) if c), key=lambda t: -t[0])
    out = get(*terms[0][1]) if terms[0][0] > 0 else -get(*terms[0][1])
    for c, k in terms[1:]:
        out = out + get(*k) if c > 0 else out - get(*k)
    return out


def _scatter(acc, coef, v, tag=(), start=None):
    for k, c in np.ndenumerate(coef):
        if not c:
            continue
        k = k + tag
        if k not in acc and start is not None and (old := start(*k)) is not None:
            acc[k] = old
        if k in acc:
            acc[k] = acc[k] + v if c > 0 else acc[k] - v
        else:
            acc[k] = v if c > 0 else -v


_LHS = np.array([[1, 0, 0, 1], [0, 0, 1, 1], [1, 0, 0, 0], [0, 0, 0, 1],
                 [1, 1, 0, 0], [-1, 0, 1, 0], [0, 1, 0, -1]]).reshape(7, 2, 2)
_RHS = np.array([[1, 0, 0, 1], [1, 0, 0, 0], [0, 1, 0, -1], [-1, 0, 1, 0],
                 [0, 0, 0, 1], [1, 1, 0, 0], [0, 0, 1, 1]]).reshape(7, 2, 2)
_OUT = np.array([[1, 0, 0, 1], [0, 0, 1, -1], [0, 1, 0, 1], [1, 0, 1, 0],
                 [-1, 1, 0, 0], [0, 0, 0, 1], [1, 0, 0, 0]]).reshape(7, 2, 2)
_ORDER = (0, 3, 1, 2, 4, 5, 6)


def _hopcroft_kerr():
    n = 8
    method = (0, 1, 2, 0, 1, 2, 0, 1)
    stand_in = {(0, 3): (0, 2), (0, 6): (6, 2), (3, 6): (3, 2), (1, 4): (1, 5),
                (1, 7): (7, 5), (4, 7): (4, 5), (2, 5): (2, 7)}
    left_out = ("000010010001000022020010002002000200",
                "101101101210121210212121211211211011",
                "111111112122212101101202120120122122")
    forms = np.array([[[[1, 0], [1, 1]], [[-1, 1], [0, 1]]],
                      [[[0, 1], [1, 1]], [[1, -1], [1, 0]]],
                      [[[1, 0], [1, 0]], [[0, 1], [0, 1]]]])
    turn_a, turn_c = np.array([[0, -1], [1, 1]]), np.array([[1, -1], [1, 0]])
    eye = np.eye(n, dtype=int)
    lhs, out, groups, node, inner = [], [], [], {}, {}

    def product(a, c):
        lhs.append(a)
        out.append(c)
        groups[-1].append(len(lhs) - 1)
        return np.eye(100, dtype=int)[len(lhs) - 1]

    def add_node(key, a, c, m):
        groups.append([])
        node[key] = (a, c, m, [product(np.outer(f, a), np.outer(g, c)) for f, g in forms[m]])

    def pair(p, q):
        swap = (node[q][2] - node[p][2]) % 3 != 1
        (ai, ci, mi, di), (aj, cj, _, dj) = (node[q], node[p]) if swap else (node[p], node[q])
        sa, sc = (np.linalg.matrix_power(t, -mi % 3) for t in (turn_a, turn_c))
        add_node((p, q), ai + aj, ci - cj, (mi + 2) % 3)
        cross = product(np.outer(sa[:, 0], ai) + np.outer(sa[:, 1], aj),
                        np.outer(sc[:, 0], cj) + np.outer(sc[:, 1], ci))

        def turned(m, t, products):
            want = np.outer(sa @ forms[m, t, 0], sc @ forms[m, t, 1])
            return next(v for v, (f, g) in zip(products, forms[(m + mi) % 3]) if (np.outer(f, g) == want).all())

        dv = node[p, q][3]
        ij = cross - turned(2, 1, dv) - turned(1, 0, dj) + turned(0, 1, di)
        ji = cross + turned(2, 0, dv) - turned(0, 0, di) + turned(1, 1, dj)
        return (ji, ij) if swap else (ij, ji)

    for i in range(n):
        add_node(i, eye[i], eye[i], method[i])
        inner[i, i] = sum(node[i][3])
    for i, j in itertools.combinations(range(n), 2):
        if method[i] != method[j]:
            inner[i, j], inner[j, i] = pair(i, j)
    for (i, j), (u, k) in sorted(stand_in.items()):
        v, w = (min(u, k), max(u, k)), i + j - u
        vw, wv = pair(v, w)
        inner[u, w] = vw - inner[k, w]
        inner[w, u] = node[v][1][u] * wv + inner[w, k]
    lhs, out = np.array(lhs), np.array(out)
    rhs = np.array([[inner[i, j] for j in range(n)] for i in range(n)]).transpose(2, 0, 1)
    assert (np.einsum("pri,pjk,psl->rijksl", lhs, rhs, out)
            == np.einsum("rs,ij,kl->rijksl", np.eye(2, dtype=int), eye, eye)).all()

    used = [sorted(p for g, d in zip(groups, text) for p in g if p != g[int(d)]) for text in left_out]
    steps = []
    for s, products in enumerate(used):
        basis = rhs[products].reshape(n * n, n * n)
        dual = np.rint(np.linalg.inv(basis).T).astype(int)
        assert (basis.T @ dual == np.eye(n * n)).all()
        entries = []
        for p, u in zip(products, dual.reshape(-1, n, n)):
            i, j = np.argwhere(u)[0]
            mem_lhs, mem_out = u[:, j] * u[i, j], u[i]
            assert (np.outer(mem_lhs, mem_out) == u).all()
            when = [t for t in range(PERIOD) if p in used[t]]
            halves = (0, 1) if len(when) == 1 else (when.index(s),)
            entries.append((p, halves, mem_lhs, mem_out))
        steps.append(entries)

    def locality(p):
        idx = np.nonzero(np.abs(out[p]).sum(0))[0]
        a, b = idx.min() // 2, idx.max() // 2
        return (a, -b if a % 2 else b, tuple(idx))

    steps = [sorted(e, key=lambda t: (t[1] == (1,), locality(t[0]))) for e in steps]
    return lhs, rhs, out, steps, sorted(range(len(lhs)), key=locality)


_HK_LHS, _HK_RHS, _HK_OUT, _HK_STEPS, _HK_ORDER = _hopcroft_kerr()
NB, NPROD = _HK_RHS.shape[1], _HK_RHS.shape[0]


def _share(jobs, k, n):
    return jobs[len(jobs) * k // n:len(jobs) * (k + 1) // n]


def _mix(*lists):
    keyed = [((n + 0.5) / len(l), k, n) for k, l in enumerate(lists) for n in range(len(l))]
    return [lists[k][n] for _, k, n in sorted(keyed)]


def _jobs(fn, *ranges):
    return [functools.partial(fn, *k) for k in itertools.product(*ranges)]


def _run(jobs):
    for job in jobs:
        job(lambda v: v)


def _never(ref):
    return jnp.abs(ref[0:SUB, 0:LANES].astype(F32)) < 0.0


class _Pacer:
    def __init__(self, never):
        self.never = never
        self.tokens = []

    def dot(self, a, b):
        m = _dot(a, b)
        rounds = min(max(a.shape[1] * m.shape[1] // (4 * LANES * LANES), 1), m.shape[1] // LANES)
        self.tokens += [
            m[r:r + SUB, c:c + LANES]
            for c in range(0, m.shape[1], m.shape[1] // rounds) for r in range(0, m.shape[0], SUB)
        ]
        return m

    def run(self, *job_lists):
        tokens, self.tokens = self.tokens, []

        def gate(k, count, v):
            n = v.shape[0] // SUB
            rows = []
            for r in range(n):
                t = lax.bitcast_convert_type(tokens[len(tokens) * (k * n + r) // (count * n)], v.dtype)
                rows.append(jnp.concatenate([
                    jnp.where(self.never, t, v[r * SUB:(r + 1) * SUB, c:c + LANES])
                    for c in range(0, v.shape[1], LANES)], axis=1))
            return jnp.concatenate(rows, axis=0)

        for job in _mix(*[
            [functools.partial(job, functools.partial(gate, k, len(jobs))) for k, job in enumerate(jobs)]
            for jobs in job_lists
        ]):
            job()


def _rhs(w, i):
    n = w.shape[0] // 7
    return jnp.concatenate([_get_wide(w, n * i + k) for k in range(n)], axis=0)


def _strassen(block, w, pacer, side, start=None):
    c = {}
    for i in _ORDER:
        _scatter(c, _OUT[i], pacer.dot(_combine(_LHS[i], block).astype(BF16), _rhs(w, i)), start=start)
    pacer.run(*side)
    return c


def _rhs_jobs(dst, src, which=range(7), scale=None):
    kh, nh, rows = src.shape[0] // 2, src.shape[1] // 2, 64

    def job(c, k0, gate):
        @functools.cache
        def block(a, b):
            v = gate(src[pl.ds(a * kh + k0, rows), pl.ds(b * nh + c * LANES, LANES)].astype(F32))
            return v if scale is None else scale * v

        for i in which:
            k, r = divmod((i * kh + k0) // 2, dst.shape[2])
            _put(dst, (k, c, pl.ds(r, rows // 2)), _combine(_RHS[i], block))

    return _jobs(job, range(nh // LANES), range(0, kh, rows))


def _rhs2_jobs(dst, src):
    kq, nq = src.shape[0] // 4, src.shape[1] // 4

    @functools.cache
    def block(c, k0, a, b):
        return src[pl.ds(a * kq + k0, PACK), pl.ds(b * nq + c * LANES, LANES)].astype(F32)

    def job(c, k0, i, gate):
        outer = functools.cache(lambda a, b: gate(_combine(_RHS[i], lambda u, v: block(c, k0, 2 * u + a, 2 * v + b))))
        for j in range(7):
            _put(dst, (7 * i + j, c, pl.ds(k0 // 2, SUB)), _combine(_RHS[j], outer))

    return _jobs(job, range(nq // LANES), range(0, kq, PACK), range(7))


def _hk_jobs(block, store):
    def job(p, gate):
        first = tuple(np.argwhere(_HK_RHS[p])[0])
        store(p, _combine(_HK_RHS[p], lambda i, j: gate(block(i, j)) if (i, j) == first else block(i, j)))

    return _jobs(job, _HK_ORDER)


def _kernel(
    x_hbm, mem_hbm, wq_hbm, wk_hbm, wv_hbm, wo_hbm, w1_hbm, w2_hbm, w3_hbm, w4_hbm,
    out_hbm,
    xb, xn, base, macc, wqkv, wo, raw, mid, raw_o, mem0, sem_m, sem_a, sem_o,
    *, S, D, H, DH, M, SEG, F,
):
    HD = D // 2
    NCB = D // LANES
    NG = H // NB
    T1 = 2 * R1
    NT = S // T1
    NF = F // FC
    assert LANES // PACK == NF + 1

    mem_copy = pltpu.make_async_copy(mem_hbm, mem0, sem_m)

    def wo_copy(part):
        rows = pl.ds(pl.multiple_of(part * PACK, PACK), PACK)
        return pltpu.make_async_copy(wo_hbm.at[:, rows], raw_o.at[part % 2], sem_o.at[part % 2])

    def wo_jobs(part):
        dst = wo.at[:, :, pl.ds(pl.multiple_of(part * SUB, SUB), SUB)]
        src = raw_o.at[part % 2]

        def group(g):
            block = functools.cache(lambda i, j: src[g * NB + i, :, pl.ds(j * LANES, LANES)].astype(F32))
            return _hk_jobs(block, lambda p, v: _put(dst, (p, g), v))

        return [job for g in range(NG) for job in group(g)]

    def qkv_unit(n, k):
        return divmod(3 * n + k, NF + 1)

    def qkv_fetch(n):
        for k in range(3):
            w, part = qkv_unit(n, k)
            rows = pl.ds(pl.multiple_of(part * PACK * H, PACK * H), PACK * H)
            for which, src in enumerate((wq_hbm, wk_hbm, wv_hbm)):
                @pl.when(w == which)
                def _():
                    pltpu.make_async_copy(src.at[:, rows], raw.at[n % 2, k], sem_a.at[n % 2, k]).start()

    def qkv_wait(n):
        for k in range(3):
            pltpu.make_async_copy(wq_hbm.at[:, pl.ds(0, PACK * H)], raw.at[n % 2, k], sem_a.at[n % 2, k]).wait()

    def qkv_jobs(n):
        src = raw.at[n % 2]

        def transpose(k, half, i, gate):
            rows = gate(jnp.concatenate([
                pltpu.bitcast(src[k, i, pl.ds(d * H + half * PACK, PACK), :], U32) for d in range(PACK)], axis=0))
            for d in range(PACK):
                mid[k, i, pl.ds(half * SUB * (PACK + 1) + d, SUB, stride=PACK + 1), :] = rows[d * SUB:(d + 1) * SUB]

        def group(k, g, dst):
            words = functools.cache(lambda i, pair: mid[k, i, pl.ds((g * NB // 2 + pair) * (PACK + 1), PACK), :])
            block = functools.cache(lambda i, j: pltpu.bitcast(
                words(i, j // 2) & jnp.uint32(0xFFFF0000) if j % 2 else words(i, j // 2) << 16, F32))
            return _hk_jobs(block, lambda p, v: _put(dst, pl.ds((p * NG + g) * LANES // 2, SUB), v))

        moves, sums = [], [[]]
        for k in range(3):
            w, part = qkv_unit(n, k)
            dst = wqkv.at[w, pl.ds(pl.multiple_of(part * SUB, SUB), wqkv.shape[1] - NF * SUB)]
            for half in range(H // PACK):
                moves.append(_jobs(transpose, [k], [half], range(NB)))
                sums.append(group(k, 2 * half, dst) + group(k, 2 * half + 1, dst))
        return [job for a, b in zip(moves + [[]], sums) for job in _mix(a, b)]

    def mixer(yc, w3c, r3, r4, sem_f):
        def w3_copy(f):
            cols = pl.ds(pl.multiple_of(f * FC, FC), FC)
            return pltpu.make_async_copy(w3_hbm.at[:, cols], r3.at[f % 2], sem_f.at[0, f % 2])

        def w4_copy(f):
            rows = pl.ds(pl.multiple_of(f * FC, FC), FC)
            return pltpu.make_async_copy(w4_hbm.at[rows], r4.at[f % 2], sem_f.at[1, f % 2])

        def w3_jobs(f):
            return _rhs2_jobs(w3c.at[f % 2], r3.at[f % 2])

        def token_mixing(r12, y0, c1, sem_x, sem_w):
            w1c, w2c = (wo.at[pl.ds(n * 7 * HD // LANES, 7 * HD // LANES)] for n in range(2))
            shifts = (-1, 1, -2, 2)
            HP = S + 2 * SUB

            def x_copy(t):
                rows = pl.ds(pl.multiple_of(t * T1, T1), T1)
                return pltpu.make_async_copy(x_hbm.at[rows], xb.at[rows], sem_x.at[t])

            def w1_copy(a, b):
                idx = (pl.ds(a * HD, HD), pl.ds(b * HD, HD))
                return pltpu.make_async_copy(w1_hbm.at[idx], r12.at[(0,) + idx], sem_w.at[2 * a + b])

            w2_copy = pltpu.make_async_copy(w2_hbm, r12.at[1], sem_w.at[4])

            def tile(ref, t, view=0):
                return ref.at[pl.ds(pl.multiple_of(t * T1 + view * zero, T1), T1)]

            def normalizing(t, slot):
                xs, xn_t, n = [tile(xb, t, v) for v in range(3)], tile(xn, t), 2 * PACK

                def finish(k, mean, var):
                    def job(c, gate):
                        rows, cols = pl.ds(k * n, n), pl.ds(c * HD // 2, HD // 2)
                        r = lax.rsqrt(var[k] + EPS)
                        v = (xs[2][rows, cols].astype(F32) - wide(gate, mean[k], HD // 2)) * r
                        xn_t[rows, cols] = v.astype(BF16)
                        y0[slot, rows, cols] = v * lax.rsqrt(var[k] * r * r + EPS)

                    return _jobs(job, range(4))

                return _layernorm_jobs(
                    lambda v, k, gate: _gate_first(gate, xs[v][pl.ds(k * n, n), :].astype(F32)), T1 // n, finish, NS)

            def wide(gate, column, width):
                v = gate(jnp.broadcast_to(column, (column.shape[0], LANES)))
                return jnp.concatenate([v] * (width // LANES), axis=1)

            def keep(dst, c):
                for (a, b), v in c.items():
                    dst[a, :, pl.ds(b * HD, HD)] = v

            def block1(slot):
                return lambda a, b: y0[slot, pl.ds(a * R1, R1), pl.ds(b * HD, HD)]

            def stage1(slot, *side):
                keep(c1, _strassen(block1(slot), w1c, pacer, side))

            def h_from(t):
                return wqkv.at[0, pl.ds(pl.multiple_of(t * T1, T1), (NCB - 1) * HP + T1 + 2 * SUB)]

            def activating(t):
                hb_t = h_from(t)

                def job(a, c, gate):
                    h = _gelu2(gate(c1[a, :, pl.ds(c * LANES, LANES)]))
                    hb_t[pl.ds(c * HP + SUB + a * R1, R1), :] = pltpu.bitcast(h, U32)

                return _jobs(job, range(2), range(NCB))

            def stage2(t, *side, lo=0, n=R1):
                hb_t, base_t, xn_t = h_from(t), tile(base, t), tile(xn, t)
                c = _strassen(lambda a, b: jnp.concatenate([
                    pltpu.bitcast(hb_t[pl.ds(c * HP + SUB + a * R1 + lo + shifts[c * 4 // NCB], n), :], F32)
                    for c in range(b * NCB // 2, (b + 1) * NCB // 2)], axis=1), w2c, pacer, side,
                    lambda a, b: xn_t[pl.ds(a * R1 + lo, n), pl.ds(b * HD, HD)].astype(F32))
                for (a, b), v in c.items():
                    base_t[pl.ds(a * R1 + lo, n), pl.ds(b * HD, HD)] = v

            def renormalizing(t, slack=0):
                starts = range(0, RU, PACK)
                xs = [tile(base, t, v) for v in range(3)]
                yc_t = yc.at[:, :, pl.ds(pl.multiple_of(t * (RU // 2), RU // 2), RU // 2)]

                def read(view, k, cols):
                    return jnp.concatenate([xs[view][pl.ds(q * RU + starts[k], PACK), cols] for q in range(4)], axis=0)

                def finish(k, mean, var):
                    y = {}

                    def job(c, i, gate):
                        if i == 0:
                            m, r = wide(gate, mean[k], LANES), lax.rsqrt(var[k] + EPS)
                            for q in range(4):
                                y[c, q] = (read(2, k, pl.ds(q * HD // 2 + c * LANES, LANES)) - m) * r
                        outer = functools.cache(lambda a, b: gate(_combine(
                            _LHS[i], lambda u, v: y[c, 2 * v + b][(2 * u + a) * PACK:(2 * u + a + 1) * PACK])))
                        for j in range(7):
                            _put(yc_t, (7 * i + j, c, pl.ds(starts[k] // 2, SUB)), _combine(_LHS[j], outer))

                    return _jobs(job, range(NCB // 4), range(7))

                return _layernorm_jobs(
                    lambda v, k, gate: _gate_first(gate, read(v, k, slice(None))), len(starts), finish, slack)

            arrival = (((0, 0), (1,)), ((1, 1), (4, 0)), ((0, 1), (2, 5)), ((1, 0), (3, 6)))
            quarters = [w1_copy(*q) for q, _ in arrival]
            queue = [[quarters[2], x_copy(1)], [quarters[3]], [x_copy(2)], [w2_copy]]
            x_copy(0).start()
            quarters[0].start()
            for c in range(NCB):
                wqkv[0, pl.ds(c * HP, SUB), :] = jnp.zeros((SUB, LANES), U32)
                wqkv[0, pl.ds(c * HP + SUB + S, SUB), :] = jnp.zeros((SUB, LANES), U32)


            def clearing(t):
                acc_t = macc.at[:, pl.ds(pl.multiple_of(t * R1, R1), R1)]

                def job(i, lo, gate):
                    acc_t[i, pl.ds(lo, PACK), :] = wide(gate, jnp.zeros((PACK, 1), F32), HD)

                return _jobs(job, range(7), range(0, R1, PACK))

            for t in range(3):
                _run(clearing(t))
            pad = xn.shape[0] - S
            xn[pl.ds(S, pad), :] = jnp.zeros((pad, D), BF16)
            with _scope("wait_x0"):
                x_copy(0).wait()
            quarters[1].start()
            pacer = _Pacer(_never(xb))
            zero = jnp.max(pacer.never.astype(jnp.int32))
            with _scope("tile0"):
                _run(itertools.chain(*normalizing(0, 1)))
                c = {}
                for n, (q, ready) in enumerate(arrival):
                    w1_copy(*q).wait()
                    if n == 2:
                        x_copy(1).wait()
                        *stats, ahead = normalizing(1, 0)
                        ahead = ahead[8:]
                    for cp in queue.pop(0):
                        cp.start()
                    _run(_rhs_jobs(w1c, r12.at[0], ready))
                    for i in ready:
                        _scatter(c, _OUT[i], pacer.dot(_combine(_LHS[i], block1(1)).astype(BF16), _rhs(w1c, i)))
                    pacer.run(*(stats if n == 2 else [ahead] if n == 3 else []))
                keep(c1, c)
            with _scope("tile1"):
                x_copy(3).start()
                w3_copy(0).start()
                x_copy(2).wait()
                stage1(0, activating(0), *normalizing(2, 1))
                x_copy(4).start()
                mem_copy.start()
                w2_copy.wait()
                x_copy(3).wait()
                w3_copy(0).wait()
                stage1(1, activating(1), _rhs_jobs(w2c, r12.at[1], scale=0.5))
                w3j = w3_jobs(0)
                stage2(0, w3j[:len(w3j) * W3S // 4], *normalizing(3, 0))

            def slot(u, carry):
                @pl.when(u + 1 < NT)
                def _():
                    x_copy(u + 1).wait()

                @pl.when(u + 2 < NT)
                def _():
                    x_copy(u + 2).start()

                @pl.when(u == 4)
                def _():
                    w3_copy(1).start()

                @pl.when(u == 5)
                def _():
                    w4_copy(0).start()
                    wo_copy(0).start()

                @pl.when(u == 6)
                def _():
                    qkv_fetch(0)

                with _scope("slot"):
                    idle = [lambda gate: None] * 4
                    stage1(0, activating(u - 1) + idle, *renormalizing(u - 3))
                    stage2(u - 2, clearing(u), *normalizing(jnp.minimum(u + 1, NT - 1), 0))
                return carry

            lax.fori_loop(3, NT, slot, 0)
            with _scope("tile7"):
                last = activating(NT - 1)
                halo = [c for c in range(NCB) if shifts[c * 4 // NCB] > 0]
                _run([last[c] for c in halo])
                stage2(NT - 2, [job for c, job in enumerate(last) if c not in halo], *renormalizing(NT - 3, RS))
                stage2(NT - 1, w3j[len(w3j) * W3S // 4:], *renormalizing(NT - 2, RS))
                _run(itertools.chain(*renormalizing(NT - 1)))

        def ffn(w4c, g):
            N3 = S // 2 // R3
            never = _never(xb)

            def chunk(f, carry):
                @pl.when(f + 2 < NF)
                def _():
                    w3_copy(f + 2).start()

                @pl.when(f + 1 < NF)
                def _():
                    w4_copy(f + 1).start()
                    w3_copy(f + 1).wait()

                wo_copy(f + 1).start()
                qkv_fetch(f + 1)
                qkv_wait(f)
                w4_copy(f).wait()
                wo_copy(f).wait()
                pacer = _Pacer(never)
                w3f = w3c.at[f % 2]
                pre = {}

                def up(t, *side):
                    for s in range(t * R3 // (2 * RU), (t + 1) * R3 // (2 * RU)):
                        c = pre[s] = {}
                        for i in _ORDER:
                            inner = {}
                            for j in _ORDER:
                                a = _get_wide(yc, 7 * i + j, pl.ds(s * RU // 2, RU // 2))
                                _scatter(inner, _OUT[j], pacer.dot(a, _get_wide(w3f, 7 * i + j)))
                            for q, v in inner.items():
                                _scatter(c, _OUT[i], v, q)
                    pacer.run(*side)

                def activating(t):
                    def job(k, a, lo, gate):
                        for u, v, b in itertools.product(range(2), repeat=3):
                            g[t % 2, u, pl.ds((2 * k + a) * RU + lo, RD), pl.ds((2 * v + b) * FC // 4, FC // 4)] = (
                                _gelu2(gate(pre[t * R3 // (2 * RU) + k][u, v, a, b][lo:lo + RD])))

                    return _jobs(job, range(R3 // (2 * RU)), range(2), range(0, RU, RD))

                def down(t, *side):
                    for s in range(R3 // (2 * RD)):
                        for i in _ORDER:
                            outer = functools.cache(lambda a, b: _combine(_LHS[i], lambda u, v: g[
                                t % 2, u, pl.ds((2 * s + a) * RD, RD), pl.ds((2 * v + b) * FC // 4, FC // 4)]))
                            where = {
                                (a, b): (i, pl.ds(t * R3 + (2 * s + a) * RD, RD), pl.ds(b * HD // 2, HD // 2))
                                for a in range(2) for b in range(2)
                            }
                            acc = {k: macc[idx] for k, idx in where.items()}
                            for j in _ORDER:
                                a = _combine(_LHS[j], outer).astype(BF16)
                                _scatter(acc, _OUT[j], pacer.dot(a, _get_wide(w4c, 7 * i + j)))
                            for k, idx in where.items():
                                macc[idx] = acc[k]
                    pacer.run(*side)

                side = [qkv_jobs(f), wo_jobs(f)]
                w3j = w3_jobs(f + 1)
                total = WU * (N3 - 2) + WD * (N3 - 1) + WE + W1
                at = 0

                def take(n):
                    nonlocal at
                    at += n
                    return [l[len(l) * (at - n) // total:len(l) * at // total] for l in side]

                with _scope("chunk"):
                    up(0, _rhs2_jobs(w4c, r4.at[f % 2]))
                    up(1, activating(0), *take(W1))
                    for t in range(N3 - 2):
                        down(t, activating(t + 1), *take(WD), _share(w3j, t, N3))
                        up(t + 2, *take(WU))
                    down(N3 - 2, activating(N3 - 1), *take(WD), _share(w3j, N3 - 2, N3))
                    down(N3 - 1, *take(WE), _share(w3j, N3 - 1, N3))
                return carry

            lax.fori_loop(0, NF, chunk, 0)

        if "1" in PARTS:
            pl.run_scoped(
                token_mixing,
                pltpu.VMEM((2, D, D), BF16),
                pltpu.VMEM((2, T1, D), F32),
                pltpu.VMEM((2, R1, D), F32),
                pltpu.SemaphoreType.DMA((NT,)),
                pltpu.SemaphoreType.DMA((5,)),
            )
        if "3" in PARTS:
            pl.run_scoped(
                ffn,
                _words(49, NCB // 4, FC // 8),
                pltpu.VMEM((2, 2, R3, FC), F32),
            )
        else:
            k = xb[0:8, 0:128].astype(jnp.int32)[0, 0]
            xb[0:16, 0:128] = yc[k, k, 0:16].astype(F32).astype(BF16) + w3c[k, k, k, 0:16].astype(F32).astype(BF16)

    def recurrence(res, gq, fq, ob, oc, go, sem_out):
        L = M + SEG
        PR = PERIOD * SEG
        HR = PR // 2
        QR = PR // 4
        NPER = (S // SEG - 1) // PERIOD
        assert NPER * PR + SEG == S
        scale = DH ** -0.5
        row = lax.broadcasted_iota(jnp.int32, (L, L), 0)
        col = lax.broadcasted_iota(jnp.int32, (L, L), 1)
        mask = (row < M) | (row >= col)

        def w_in(w, p, g):
            return _get(wqkv, (w, pl.ds((p * NG + g) * LANES // 2, LANES // 2)))

        def out_copy(r0, n):
            return pltpu.make_async_copy(res.at[pl.ds(r0, n)], out_hbm.at[pl.ds(r0, n)], sem_out)

        def emit(rows, attended):
            res[rows, :] = (xb[rows, :].astype(F32) + base[rows, :] + attended).astype(BF16)

        def quarter(a, halves):
            return pl.ds(a * HR + halves[0] * QR, len(halves) * QR)

        wo_copy(NF).wait()
        qkv_wait(NF)
        mem_copy.wait()
        with _scope("a_pro"):
            pacer = _Pacer(_never(xb))

            def collect(lo, gate):
                c = {}
                for i in _ORDER:
                    v = macc[i, pl.ds(lo, PACK), :]
                    _scatter(c, _OUT[i], gate(v) if i < 3 else v)
                t, r = divmod(lo, R1)
                for (a, b), v in c.items():
                    base[pl.ds(t * T1 + a * R1 + r, PACK), pl.ds(b * HD, HD)] += 0.5 * v

            tokens = xn[pl.ds(0, PR), :].astype(F32)
            lhs = {p: _combine(_HK_LHS[p], lambda a, i: _lanes(tokens, i)[a * HR:(a + 1) * HR]).astype(BF16)
                   for p in _HK_ORDER}
            for w, g in itertools.product(range(3), range(NG)):
                c = {}
                for p in _HK_ORDER:
                    _scatter(c, _HK_OUT[p], pacer.dot(lhs[p], w_in(w, p, g)))
                for (a, j), v in c.items():
                    gq[w, g * NB + j, pl.ds(a * HR, HR), :] = v
                if (w, g) == (1, NG - 2):
                    pacer.run(qkv_jobs(NF))
            pacer.run(wo_jobs(NF), _jobs(collect, range(0, S // 2, PACK)))
            ob[...] = jnp.zeros(ob.shape, F32)
            go[...] = jnp.zeros(go.shape, F32)

        def period(it, mem):
            done = pl.multiple_of(jnp.maximum(it - 2, 0) * PR, PR)
            tokens = xn[pl.ds(pl.multiple_of((it + 1) * PR, PR), PR), :].astype(F32)
            emit(pl.ds(done, PR), go[...])
            for step in range(PERIOD):
                mem = segment(step, tokens, mem)

            @pl.when(it >= 2)
            def _():
                out_copy(done, PR).start()

            return mem

        def segment(step, tokens, mem):
            entries = _HK_STEPS[step]
            rows = pl.ds(step * SEG, SEG)
            begun = {
                k + (half,)
                for p, halves, _, _ in itertools.chain(*_HK_STEPS[:step])
                for half in halves for k, c in np.ndenumerate(_HK_OUT[p]) if c
            }

            def operand(entry, mem_block, token_block):
                p, halves, mem_lhs, _ = entry
                a = jnp.concatenate([
                    _combine(mem_lhs, mem_block),
                    _combine(_HK_LHS[p], lambda a, i: token_block(quarter(a, halves), i))], axis=0)
                return a if a.shape[0] % PACK else a.astype(BF16)

            def fold(entry, r, mem_acc, token_acc, partial):
                p, halves, _, mem_out = entry
                _scatter(mem_acc, mem_out, r[:M])
                for n, half in enumerate(halves):
                    _scatter(token_acc, _HK_OUT[p], r[M + n * QR:M + (n + 1) * QR], (half,),
                             lambda a, j, h: partial(quarter(a, (h,)), j) if (a, j, h) in begun else None)

            lhs = [
                operand(e, lambda i: _lanes(mem, i), lambda r, i: _lanes(tokens, i)[r.start:r.start + r.size])
                for e in entries
            ]
            qkv_mem, prob, att_mem, new_mem, out_acc = {}, {}, {}, {}, {}

            def project(g, w):
                if step == 0:
                    for h in range(g * NB, (g + 1) * NB):
                        fq[w, h] = gq[w, h]
                        if w == 0:
                            oc[h] = ob[h]
                mem_acc, token_acc = {}, {}

                def one(a, e):
                    fold(e, _dot(a, w_in(w, e[0], g)), mem_acc, token_acc, lambda r, j: gq[w, g * NB + j, r, :])

                def finish():
                    for (a, j, half), v in token_acc.items():
                        gq[w, g * NB + j, quarter(a, (half,)), :] = v
                    for (j,), v in mem_acc.items():
                        qkv_mem[w, g * NB + j] = v

                return [functools.partial(one, a, e) for a, e in zip(lhs, entries)] + [finish]

            def part(w, h):
                return jnp.concatenate([qkv_mem[w, h], fq[w, h, rows, :]], axis=0)

            def scores(h):
                prob[h] = _softmax_rows(part(0, h), part(1, h), mask, scale)

            def attend(h):
                o = _dot(prob[h], part(2, h))
                att_mem[h] = o[:M]
                ob[h, rows, :] = o[M:]

            def outproj(g, e):
                a = operand(e, lambda i: att_mem[g * NB + i], lambda r, i: oc[g * NB + i, r, :])
                fold(e, _dot(a, _get(wo, (e[0], g))), new_mem, out_acc, lambda r, j: go[r, pl.ds(j * LANES, LANES)])

            def heads(fn, g):
                return _jobs(fn, range(g * NB, (g + 1) * NB))

            def play(*lists):
                for job in _mix(*lists):
                    job()

            todo = _jobs(outproj, range(NG), entries)
            early = len(todo) - len(entries) - sum(TAIL)
            at = 0
            for g in range(NG):
                play(project(g, 0))
                play(project(g, 1), heads(attend, g - 1) if g else [])
                values = project(g, 2)
                lead = len(values) // (4 if g == NG - 1 else 2)
                play(values[:lead])
                play(values[lead:lead + len(values) // 2], heads(scores, g))
                play(values[lead + len(values) // 2:])
                play(todo[at:min(early, g * len(entries))])
                at = min(early, g * len(entries))
            play(todo[at:at + TAIL[0]])
            play(todo[at + TAIL[0]:at + sum(TAIL)], heads(attend, NG - 1))
            play(todo[at + sum(TAIL):])
            for (a, j, half), v in out_acc.items():
                go[quarter(a, (half,)), pl.ds(j * LANES, LANES)] = v
            return jnp.concatenate([new_mem[j,] for j in range(NB)], axis=1)

        with _scope("a_loop"):
            mem = lax.fori_loop(0, NPER, period, mem0[...].astype(F32))

        with _scope("a_epi"):
            emit(pl.ds((NPER - 2) * PR, PR), go[...])
            out_copy((NPER - 2) * PR, PR).start()
            rows = pl.ds(0, SEG)
            ER = (PR + SEG) // 2
            lhs = [_combine(e[2], lambda i: _lanes(mem, i)) for e in _HK_STEPS[0]]
            kv_mem, prob, att, out_acc = {}, {}, {}, {}

            def project(w, g):
                acc = {}
                for a, (p, _, _, mem_out) in zip(lhs, _HK_STEPS[0]):
                    _scatter(acc, mem_out, _dot(a, w_in(w, p, g)))
                for (j,), v in acc.items():
                    kv_mem[w, g * NB + j] = jnp.concatenate([v, gq[w, g * NB + j, rows, :]], axis=0)

            def block(a, h):
                if a == 0:
                    return ob[h, pl.ds(0, ER), :]
                return jnp.concatenate([ob[h, pl.ds(ER, PR - ER), :], att[h]], axis=0)

            for t in range(NG + 2):
                if t < NG:
                    project(1, t)
                    project(2, t)
                    for h in range(t * NB, (t + 1) * NB):
                        prob[h] = _softmax_rows(gq[0, h, rows, :], kv_mem[1, h], mask[M:], scale)
                if 0 <= t - 2:
                    for p in _HK_ORDER:
                        a = _combine(_HK_LHS[p], lambda a, i: block(a, (t - 2) * NB + i))
                        _scatter(out_acc, _HK_OUT[p], _dot(a, _get(wo, (p, t - 2))))
                if 0 <= t - 1 < NG:
                    for h in range((t - 1) * NB, t * NB):
                        att[h] = _dot(prob[h], kv_mem[2, h])
            r0 = (NPER - 1) * PR
            for a in range(2):
                emit(pl.ds(r0 + a * ER, ER), jnp.concatenate([out_acc[a, j] for j in range(NB)], axis=1))
            out_copy(r0, 2 * ER).start()
        with _scope("tail"):
            out_copy(0, S).wait()

    if "1" in PARTS or "3" in PARTS:
        pl.run_scoped(
            mixer,
            _words(49, NCB // 4, S // 8),
            _words(2, 49, FC // 4 // LANES, HD // 4),
            pltpu.VMEM((2, D, FC), BF16),
            pltpu.VMEM((2, FC, D), BF16),
            pltpu.SemaphoreType.DMA((2, 2)),
        )
    if "A" not in PARTS:
        k = xb[0:8, 0:128].astype(jnp.int32)[0, 0]
        k16 = pl.ds(pl.multiple_of(k * 16, 16), 16)
        xb[0:16, 0:128] = (_get(wqkv, (k, pl.ds(0, 8))) + _get(wo, (k, k, pl.ds(0, 8)))
                           + xn[k16, 0:128] + macc[k, k16, 0:128].astype(BF16) + base[k16, 0:128].astype(BF16))
        pltpu.sync_copy(xb, out_hbm)
        return
    pl.run_scoped(
        recurrence,
        pltpu.VMEM((S, D), BF16),
        pltpu.VMEM((3, H, PERIOD * SEG, DH), F32),
        pltpu.VMEM((3, H, PERIOD * SEG, DH), F32),
        pltpu.VMEM((H, PERIOD * SEG, DH), F32),
        pltpu.VMEM((H, PERIOD * SEG, DH), F32),
        pltpu.VMEM((PERIOD * SEG, D), F32),
        pltpu.SemaphoreType.DMA(()),
    )


@functools.partial(jax.jit, static_argnames=("A_seg_len",))
def pallas_parallel_sum__memory_aug_recurrent_mem_tr__mixer_s_mlp__prompt_kernel(
    A_x: jax.Array,
    A_mem0: jax.Array,
    A_Wq: jax.Array,
    A_Wk: jax.Array,
    A_Wv: jax.Array,
    A_Wo: jax.Array,
    A_seg_len: int,
    B_x: jax.Array,
    B_w1: jax.Array,
    B_w2: jax.Array,
    B_w3: jax.Array,
    B_w4: jax.Array,
):
    del B_x
    B, S, D = A_x.shape
    _, H, DH = A_Wq.shape
    M = A_mem0.shape[1]
    F = B_w3.shape[1]
    SEG = int(A_seg_len)
    assert B == 1 and DH == LANES and D == NB * LANES

    hbm = pl.BlockSpec(memory_space=pl.ANY)
    out = pl.pallas_call(
        functools.partial(_kernel, S=S, D=D, H=H, DH=DH, M=M, SEG=SEG, F=F),
        out_shape=jax.ShapeDtypeStruct((S, D), A_x.dtype),
        in_specs=[hbm] * 10,
        out_specs=hbm,
        scratch_shapes=[
            pltpu.VMEM((S, D), BF16),
            pltpu.VMEM((S + (PERIOD - 1) * SEG, D), BF16),
            pltpu.VMEM((S, D), F32),
            pltpu.VMEM((7, S // 2, D // 2), F32),
            _words(3, NPROD * H // NB * LANES // 2),
            _words(NPROD, H // NB, LANES // 2),
            pltpu.VMEM((2, 3, NB, PACK * H, LANES), BF16),
            _words(3, NB, H // 2 * (PACK + 1)),
            pltpu.VMEM((2, H, PACK, D), BF16),
            pltpu.VMEM((M, D), BF16),
            pltpu.SemaphoreType.DMA(()),
            pltpu.SemaphoreType.DMA((2, 3)),
            pltpu.SemaphoreType.DMA((2,)),
        ],
        compiler_params=pltpu.CompilerParams(vmem_limit_bytes=127 * 1024 * 1024, flags=FLAGS),
    )(
        A_x.reshape(S, D),
        A_mem0.reshape(M, D),
        A_Wq.reshape(NB, LANES * H, DH),
        A_Wk.reshape(NB, LANES * H, DH),
        A_Wv.reshape(NB, LANES * H, DH),
        A_Wo,
        B_w1, B_w2, B_w3, B_w4,
    )
    return out.reshape(B, S, D)
```

```python
import contextlib
import functools
import itertools
import math

import jax
import jax.numpy as jnp
import numpy as np
from jax import lax
from jax.experimental import pallas as pl
from jax.experimental.pallas import tpu as pltpu

F32 = jnp.float32
BF16 = jnp.bfloat16
U32 = jnp.uint32
LANES = 128
SUB = 8
PACK = 16
EPS = 1e-5
R1 = 128
RU = 64
RD = 32
R3 = 256
FC = 512
PERIOD = 3
WS = (0, 4, 0, 4, 0, 4, 1, 0)
W4 = 8
TAIL = (32, 32)
NS = 2
RS = 1
W3S = 3
PLAN = "0a///b/c/1/d2/w//3v"
SCOPES = False
PARTS = "13A"
FLAGS = None


def _scope(name):
    return jax.named_scope(name) if SCOPES else contextlib.nullcontext()


def _layernorm_jobs(read, count, finish, slack):
    mean, var = {}, {}

    def first(k, gate):
        mean[k] = jnp.mean(read(0, k, gate), axis=-1, keepdims=True)

    def second(k, gate):
        d = read(1, k, gate) - mean[k]
        var[k] = jnp.mean(d * d, axis=-1, keepdims=True)

    def idle(gate):
        pass

    last = [finish(k, mean, var) for k in range(count)]
    n = len(last[0])
    return [
        _jobs(first, range(count)) + [idle] * (2 + slack),
        [idle] + _jobs(second, range(count)) + [idle] * (1 + slack),
        [idle] * 2 * n + list(itertools.chain(*last)) + [idle] * slack * n,
    ]


def _gate_first(gate, v):
    return jnp.concatenate([gate(v[:, :LANES]), v[:, LANES:]], axis=1)


def _gelu2(x):
    c = math.sqrt(2 / math.pi)
    return x + x * jnp.tanh(x * (c + (c * 0.044715) * (x * x)))


def _softmax_rows(q, k, mask, scale):
    z = lax.dot_general(q, k, (((1,), (1,)), ((), ())), preferred_element_type=F32)
    z = jnp.where(mask, z * scale, -1e9)
    e = jnp.exp(z - jnp.max(z, axis=-1, keepdims=True))
    s = jnp.sum(e, axis=-1, keepdims=True)
    r = pl.reciprocal(s, approx=True)
    return e * (r * (2.0 - s * r))


def _dot(a, b):
    return jnp.dot(a, b, preferred_element_type=F32)


def _put(ref, idx, v):
    ref[idx] = pltpu.bitcast(v.astype(BF16), U32)


def _get(ref, idx):
    return pltpu.bitcast(ref[idx], BF16)


def _get_wide(ref, i, rows=slice(None)):
    return jnp.concatenate([_get(ref, (i, c, rows)) for c in range(ref.shape[1])], axis=1)


def _words(*shape):
    return pltpu.VMEM(shape + (LANES,), U32)


def _lanes(v, c):
    return v[:, c * LANES:(c + 1) * LANES]


def _combine(coef, get):
    terms = sorted(((int(c), k) for k, c in np.ndenumerate(coef) if c), key=lambda t: -t[0])
    out = get(*terms[0][1]) if terms[0][0] > 0 else -get(*terms[0][1])
    for c, k in terms[1:]:
        out = out + get(*k) if c > 0 else out - get(*k)
    return out


def _scatter(acc, coef, v, tag=(), start=None):
    for k, c in np.ndenumerate(coef):
        if not c:
            continue
        k = k + tag
        if k not in acc and start is not None and (old := start(*k)) is not None:
            acc[k] = old
        if k in acc:
            acc[k] = acc[k] + v if c > 0 else acc[k] - v
        else:
            acc[k] = v if c > 0 else -v


_LHS = np.array([[1, 0, 0, 1], [0, 0, 1, 1], [1, 0, 0, 0], [0, 0, 0, 1],
                 [1, 1, 0, 0], [-1, 0, 1, 0], [0, 1, 0, -1]]).reshape(7, 2, 2)
_RHS = np.array([[1, 0, 0, 1], [1, 0, 0, 0], [0, 1, 0, -1], [-1, 0, 1, 0],
                 [0, 0, 0, 1], [1, 1, 0, 0], [0, 0, 1, 1]]).reshape(7, 2, 2)
_OUT = np.array([[1, 0, 0, 1], [0, 0, 1, -1], [0, 1, 0, 1], [1, 0, 1, 0],
                 [-1, 1, 0, 0], [0, 0, 0, 1], [1, 0, 0, 0]]).reshape(7, 2, 2)
_ORDER = (0, 3, 1, 2, 4, 5, 6)


def _hopcroft_kerr():
    n = 8
    method = (0, 1, 2, 0, 1, 2, 0, 1)
    stand_in = {(0, 3): (0, 2), (0, 6): (6, 2), (3, 6): (3, 2), (1, 4): (1, 5),
                (1, 7): (7, 5), (4, 7): (4, 5), (2, 5): (2, 7)}
    left_out = ("000010010001000022020010002002000200",
                "101101101210121210212121211211211011",
                "111111112122212101101202120120122122")
    forms = np.array([[[[1, 0], [1, 1]], [[-1, 1], [0, 1]]],
                      [[[0, 1], [1, 1]], [[1, -1], [1, 0]]],
                      [[[1, 0], [1, 0]], [[0, 1], [0, 1]]]])
    turn_a, turn_c = np.array([[0, -1], [1, 1]]), np.array([[1, -1], [1, 0]])
    eye = np.eye(n, dtype=int)
    lhs, out, groups, node, inner = [], [], [], {}, {}

    def product(a, c):
        lhs.append(a)
        out.append(c)
        groups[-1].append(len(lhs) - 1)
        return np.eye(100, dtype=int)[len(lhs) - 1]

    def add_node(key, a, c, m):
        groups.append([])
        node[key] = (a, c, m, [product(np.outer(f, a), np.outer(g, c)) for f, g in forms[m]])

    def pair(p, q):
        swap = (node[q][2] - node[p][2]) % 3 != 1
        (ai, ci, mi, di), (aj, cj, _, dj) = (node[q], node[p]) if swap else (node[p], node[q])
        sa, sc = (np.linalg.matrix_power(t, -mi % 3) for t in (turn_a, turn_c))
        add_node((p, q), ai + aj, ci - cj, (mi + 2) % 3)
        cross = product(np.outer(sa[:, 0], ai) + np.outer(sa[:, 1], aj),
                        np.outer(sc[:, 0], cj) + np.outer(sc[:, 1], ci))

        def turned(m, t, products):
            want = np.outer(sa @ forms[m, t, 0], sc @ forms[m, t, 1])
            return next(v for v, (f, g) in zip(products, forms[(m + mi) % 3]) if (np.outer(f, g) == want).all())

        dv = node[p, q][3]
        ij = cross - turned(2, 1, dv) - turned(1, 0, dj) + turned(0, 1, di)
        ji = cross + turned(2, 0, dv) - turned(0, 0, di) + turned(1, 1, dj)
        return (ji, ij) if swap else (ij, ji)

    for i in range(n):
        add_node(i, eye[i], eye[i], method[i])
        inner[i, i] = sum(node[i][3])
    for i, j in itertools.combinations(range(n), 2):
        if method[i] != method[j]:
            inner[i, j], inner[j, i] = pair(i, j)
    for (i, j), (u, k) in sorted(stand_in.items()):
        v, w = (min(u, k), max(u, k)), i + j - u
        vw, wv = pair(v, w)
        inner[u, w] = vw - inner[k, w]
        inner[w, u] = node[v][1][u] * wv + inner[w, k]
    lhs, out = np.array(lhs), np.array(out)
    rhs = np.array([[inner[i, j] for j in range(n)] for i in range(n)]).transpose(2, 0, 1)
    assert (np.einsum("pri,pjk,psl->rijksl", lhs, rhs, out)
            == np.einsum("rs,ij,kl->rijksl", np.eye(2, dtype=int), eye, eye)).all()

    used = [sorted(p for g, d in zip(groups, text) for p in g if p != g[int(d)]) for text in left_out]
    steps = []
    for s, products in enumerate(used):
        basis = rhs[products].reshape(n * n, n * n)
        dual = np.rint(np.linalg.inv(basis).T).astype(int)
        assert (basis.T @ dual == np.eye(n * n)).all()
        entries = []
        for p, u in zip(products, dual.reshape(-1, n, n)):
            i, j = np.argwhere(u)[0]
            mem_lhs, mem_out = u[:, j] * u[i, j], u[i]
            assert (np.outer(mem_lhs, mem_out) == u).all()
            when = [t for t in range(PERIOD) if p in used[t]]
            halves = (0, 1) if len(when) == 1 else (when.index(s),)
            entries.append((p, halves, mem_lhs, mem_out))
        steps.append(entries)

    def locality(p):
        idx = np.nonzero(np.abs(out[p]).sum(0))[0]
        a, b = idx.min() // 2, idx.max() // 2
        return (a, -b if a % 2 else b, tuple(idx))

    steps = [sorted(e, key=lambda t: (t[1] == (1,), locality(t[0]))) for e in steps]
    return lhs, rhs, out, steps, sorted(range(len(lhs)), key=locality)


_HK_LHS, _HK_RHS, _HK_OUT, _HK_STEPS, _HK_ORDER = _hopcroft_kerr()
NB, NPROD = _HK_RHS.shape[1], _HK_RHS.shape[0]


def _share(jobs, k, n):
    return jobs[len(jobs) * k // n:len(jobs) * (k + 1) // n]


def _mix(*lists):
    keyed = [((n + 0.5) / len(l), k, n) for k, l in enumerate(lists) for n in range(len(l))]
    return [lists[k][n] for _, k, n in sorted(keyed)]


def _jobs(fn, *ranges):
    return [functools.partial(fn, *k) for k in itertools.product(*ranges)]


def _run(jobs):
    for job in jobs:
        job(lambda v: v)


def _never(ref):
    return jnp.abs(ref[0:SUB, 0:LANES].astype(F32)) < 0.0


class _Pacer:
    def __init__(self, never):
        self.never = never
        self.tokens = []

    def dot(self, a, b):
        m = _dot(a, b)
        rounds = min(max(a.shape[1] * m.shape[1] // (4 * LANES * LANES), 1), m.shape[1] // LANES)
        self.tokens += [
            m[r:r + SUB, c:c + LANES]
            for c in range(0, m.shape[1], m.shape[1] // rounds) for r in range(0, m.shape[0], SUB)
        ]
        return m

    def run(self, *job_lists):
        tokens, self.tokens = self.tokens, []

        def gate(k, count, v):
            n = v.shape[0] // SUB
            rows = []
            for r in range(n):
                t = lax.bitcast_convert_type(tokens[len(tokens) * (k * n + r) // (count * n)], v.dtype)
                rows.append(jnp.concatenate([
                    jnp.where(self.never, t, v[r * SUB:(r + 1) * SUB, c:c + LANES])
                    for c in range(0, v.shape[1], LANES)], axis=1))
            return jnp.concatenate(rows, axis=0)

        for job in _mix(*[
            [functools.partial(job, functools.partial(gate, k, len(jobs))) for k, job in enumerate(jobs)]
            for jobs in job_lists
        ]):
            job()


def _rhs(w, i):
    n = w.shape[0] // 7
    return jnp.concatenate([_get_wide(w, n * i + k) for k in range(n)], axis=0)


def _strassen(block, w, pacer, side, start=None):
    c = {}
    for i in _ORDER:
        _scatter(c, _OUT[i], pacer.dot(_combine(_LHS[i], block).astype(BF16), _rhs(w, i)), start=start)
    pacer.run(*side)
    return c


def _rhs_jobs(dst, src, which=range(7), scale=None):
    kh, nh, rows = src.shape[0] // 2, src.shape[1] // 2, 64

    def job(c, k0, gate):
        @functools.cache
        def block(a, b):
            v = gate(src[pl.ds(a * kh + k0, rows), pl.ds(b * nh + c * LANES, LANES)].astype(F32))
            return v if scale is None else scale * v

        for i in which:
            k, r = divmod((i * kh + k0) // 2, dst.shape[2])
            _put(dst, (k, c, pl.ds(r, rows // 2)), _combine(_RHS[i], block))

    return _jobs(job, range(nh // LANES), range(0, kh, rows))


def _rhs2_jobs(dst, src):
    kq, nq = src.shape[0] // 4, src.shape[1] // 4

    @functools.cache
    def block(c, k0, a, b):
        return src[pl.ds(a * kq + k0, PACK), pl.ds(b * nq + c * LANES, LANES)].astype(F32)

    def job(c, k0, i, gate):
        outer = functools.cache(lambda a, b: gate(_combine(_RHS[i], lambda u, v: block(c, k0, 2 * u + a, 2 * v + b))))
        for j in range(7):
            _put(dst, (7 * i + j, c, pl.ds(k0 // 2, SUB)), _combine(_RHS[j], outer))

    return _jobs(job, range(nq // LANES), range(0, kq, PACK), range(7))


def _hk_jobs(block, store):
    def job(p, gate):
        first = tuple(np.argwhere(_HK_RHS[p])[0])
        store(p, _combine(_HK_RHS[p], lambda i, j: gate(block(i, j)) if (i, j) == first else block(i, j)))

    return _jobs(job, _HK_ORDER)


def _kernel(
    x_hbm, mem_hbm, wq_hbm, wk_hbm, wv_hbm, wo_hbm, w1_hbm, w2_hbm, w3_hbm, w4_hbm,
    out_hbm,
    xb, xn, base, macc, wqkv, wo, raw, mid, raw_o, mem0, sem_m, sem_a, sem_o,
    *, S, D, H, DH, M, SEG, F,
):
    HD = D // 2
    NCB = D // LANES
    NG = H // NB
    T1 = 2 * R1
    NT = S // T1
    NF = F // FC
    assert LANES // PACK == NF + 1

    mem_copy = pltpu.make_async_copy(mem_hbm, mem0, sem_m)

    def wo_copy(part):
        rows = pl.ds(pl.multiple_of(part * PACK, PACK), PACK)
        return pltpu.make_async_copy(wo_hbm.at[:, rows], raw_o.at[part % 2], sem_o.at[part % 2])

    def wo_jobs(part):
        dst = wo.at[:, :, pl.ds(pl.multiple_of(part * SUB, SUB), SUB)]
        src = raw_o.at[part % 2]

        def group(g):
            block = functools.cache(lambda i, j: src[g * NB + i, :, pl.ds(j * LANES, LANES)].astype(F32))
            return _hk_jobs(block, lambda p, v: _put(dst, (p, g), v))

        return [job for g in range(NG) for job in group(g)]

    def qkv_unit(n, k):
        return divmod(3 * n + k, NF + 1)

    def qkv_fetch(n):
        for k in range(3):
            w, part = qkv_unit(n, k)
            rows = pl.ds(pl.multiple_of(part * PACK * H, PACK * H), PACK * H)
            for which, src in enumerate((wq_hbm, wk_hbm, wv_hbm)):
                @pl.when(w == which)
                def _():
                    pltpu.make_async_copy(src.at[:, rows], raw.at[n % 2, k], sem_a.at[n % 2, k]).start()

    def qkv_wait(n):
        for k in range(3):
            pltpu.make_async_copy(wq_hbm.at[:, pl.ds(0, PACK * H)], raw.at[n % 2, k], sem_a.at[n % 2, k]).wait()

    def qkv_jobs(n):
        src = raw.at[n % 2]

        def transpose(k, half, i, gate):
            rows = gate(jnp.concatenate([
                pltpu.bitcast(src[k, i, pl.ds(d * H + half * PACK, PACK), :], U32) for d in range(PACK)], axis=0))
            for d in range(PACK):
                mid[k, i, pl.ds(half * SUB * (PACK + 1) + d, SUB, stride=PACK + 1), :] = rows[d * SUB:(d + 1) * SUB]

        def group(k, g, dst):
            words = functools.cache(lambda i, pair: mid[k, i, pl.ds((g * NB // 2 + pair) * (PACK + 1), PACK), :])
            block = functools.cache(lambda i, j: pltpu.bitcast(
                words(i, j // 2) & jnp.uint32(0xFFFF0000) if j % 2 else words(i, j // 2) << 16, F32))
            return _hk_jobs(block, lambda p, v: _put(dst, pl.ds((p * NG + g) * LANES // 2, SUB), v))

        moves, sums = [], [[]]
        for k in range(3):
            w, part = qkv_unit(n, k)
            dst = wqkv.at[w, pl.ds(pl.multiple_of(part * SUB, SUB), wqkv.shape[1] - NF * SUB)]
            for half in range(H // PACK):
                moves.append(_jobs(transpose, [k], [half], range(NB)))
                sums.append(group(k, 2 * half, dst) + group(k, 2 * half + 1, dst))
        return [job for a, b in zip(moves + [[]], sums) for job in _mix(a, b)]

    def mixer(yc, w3c, r3, r4, sem_f):
        def w3_copy(f):
            cols = pl.ds(pl.multiple_of(f * FC, FC), FC)
            return pltpu.make_async_copy(w3_hbm.at[:, cols], r3.at[f % 2], sem_f.at[0, f % 2])

        def w4_copy(f):
            rows = pl.ds(pl.multiple_of(f * FC, FC), FC)
            return pltpu.make_async_copy(w4_hbm.at[rows], r4.at[f % 2], sem_f.at[1, f % 2])

        def w3_jobs(f):
            return _rhs2_jobs(w3c.at[f % 2], r3.at[f % 2])

        def token_mixing(r12, y0, c1, sem_x, sem_w):
            w1c, w2c = (wo.at[pl.ds(n * 7 * HD // LANES, 7 * HD // LANES)] for n in range(2))
            shifts = (-1, 1, -2, 2)
            HP = S + 2 * SUB

            def x_copy(t):
                rows = pl.ds(pl.multiple_of(t * T1, T1), T1)
                return pltpu.make_async_copy(x_hbm.at[rows], xb.at[rows], sem_x.at[t])

            def w1_copy(a, b):
                idx = (pl.ds(a * HD, HD), pl.ds(b * HD, HD))
                return pltpu.make_async_copy(w1_hbm.at[idx], r12.at[(0,) + idx], sem_w.at[2 * a + b])

            w2_copy = pltpu.make_async_copy(w2_hbm, r12.at[1], sem_w.at[4])

            def tile(ref, t, view=0):
                return ref.at[pl.ds(pl.multiple_of(t * T1 + view * zero, T1), T1)]

            def normalizing(t, slot):
                xs, xn_t, n = [tile(xb, t, v) for v in range(3)], tile(xn, t), 2 * PACK

                def finish(k, mean, var):
                    def job(c, gate):
                        rows, cols = pl.ds(k * n, n), pl.ds(c * HD // 2, HD // 2)
                        r = lax.rsqrt(var[k] + EPS)
                        v = (xs[2][rows, cols].astype(F32) - wide(gate, mean[k], HD // 2)) * r
                        xn_t[rows, cols] = v.astype(BF16)
                        y0[slot, rows, cols] = v * lax.rsqrt(var[k] * r * r + EPS)

                    return _jobs(job, range(4))

                return _layernorm_jobs(
                    lambda v, k, gate: _gate_first(gate, xs[v][pl.ds(k * n, n), :].astype(F32)), T1 // n, finish, NS)

            def wide(gate, column, width):
                v = gate(jnp.broadcast_to(column, (column.shape[0], LANES)))
                return jnp.concatenate([v] * (width // LANES), axis=1)

            def keep(dst, c):
                for (a, b), v in c.items():
                    dst[a, :, pl.ds(b * HD, HD)] = v

            def block1(slot):
                return lambda a, b: y0[slot, pl.ds(a * R1, R1), pl.ds(b * HD, HD)]

            def stage1(slot, *side):
                keep(c1, _strassen(block1(slot), w1c, pacer, side))

            def h_from(t):
                return wqkv.at[0, pl.ds(pl.multiple_of(t * T1, T1), (NCB - 1) * HP + T1 + 2 * SUB)]

            def activating(t):
                hb_t = h_from(t)

                def job(a, c, gate):
                    h = _gelu2(gate(c1[a, :, pl.ds(c * LANES, LANES)]))
                    hb_t[pl.ds(c * HP + SUB + a * R1, R1), :] = pltpu.bitcast(h, U32)

                return _jobs(job, range(2), range(NCB))

            def stage2(t, *side, lo=0, n=R1):
                hb_t, base_t, xn_t = h_from(t), tile(base, t), tile(xn, t)
                c = _strassen(lambda a, b: jnp.concatenate([
                    pltpu.bitcast(hb_t[pl.ds(c * HP + SUB + a * R1 + lo + shifts[c * 4 // NCB], n), :], F32)
                    for c in range(b * NCB // 2, (b + 1) * NCB // 2)], axis=1), w2c, pacer, side,
                    lambda a, b: xn_t[pl.ds(a * R1 + lo, n), pl.ds(b * HD, HD)].astype(F32))
                for (a, b), v in c.items():
                    base_t[pl.ds(a * R1 + lo, n), pl.ds(b * HD, HD)] = v

            def renormalizing(t, slack=0):
                starts = range(0, RU, PACK)
                xs = [tile(base, t, v) for v in range(3)]
                yc_t = yc.at[:, :, pl.ds(pl.multiple_of(t * (RU // 2), RU // 2), RU // 2)]

                def read(view, k, cols):
                    return jnp.concatenate([
                        xs[view][pl.ds(2 * (a * RU + starts[k]) + u * PACK, PACK), cols]
                        for u in range(2) for a in range(2)], axis=0)

                def finish(k, mean, var):
                    y = {}

                    def job(c, i, gate):
                        if i == 0:
                            m, r = wide(gate, mean[k], LANES), lax.rsqrt(var[k] + EPS)
                            for q in range(4):
                                y[c, q] = (read(2, k, pl.ds(q * HD // 2 + c * LANES, LANES)) - m) * r
                        outer = functools.cache(lambda a, b: gate(_combine(
                            _LHS[i], lambda u, v: y[c, 2 * v + b][(2 * u + a) * PACK:(2 * u + a + 1) * PACK])))
                        for j in range(7):
                            _put(yc_t, (7 * i + j, c, pl.ds(starts[k] // 2, SUB)), _combine(_LHS[j], outer))

                    return _jobs(job, range(NCB // 4), range(7))

                return _layernorm_jobs(
                    lambda v, k, gate: _gate_first(gate, read(v, k, slice(None))), len(starts), finish, slack)

            arrival = (((0, 0), (1,)), ((1, 1), (4, 0)), ((0, 1), (2, 5)), ((1, 0), (3, 6)))
            quarters = [w1_copy(*q) for q, _ in arrival]
            named = dict(a=quarters[0], b=quarters[1], c=quarters[2], d=quarters[3], w=w2_copy, v=w3_copy(0))
            queue = [[x_copy(int(k)) if k.isdigit() else named[k] for k in step] for step in PLAN.split("/")]

            def launch():
                for cp in queue.pop(0):
                    cp.start()

            launch()
            for c in range(NCB):
                wqkv[0, pl.ds(c * HP, SUB), :] = jnp.zeros((SUB, LANES), U32)
                wqkv[0, pl.ds(c * HP + SUB + S, SUB), :] = jnp.zeros((SUB, LANES), U32)


            def clearing(t):
                acc_t = macc.at[:, pl.ds(pl.multiple_of(t * R1, R1), R1)]

                def job(i, lo, gate):
                    acc_t[i, pl.ds(lo, PACK), :] = wide(gate, jnp.zeros((PACK, 1), F32), HD)

                return _jobs(job, range(7), range(0, R1, PACK))

            for t in range(3):
                _run(clearing(t))
                launch()
            pad = xn.shape[0] - S
            xn[pl.ds(S, pad), :] = jnp.zeros((pad, D), BF16)
            with _scope("wait_x0"):
                x_copy(0).wait()
            launch()
            pacer = _Pacer(_never(xb))
            zero = 0
            with _scope("tile0"):
                _run(itertools.chain(*normalizing(0, 1)))
                zero = jnp.max(pacer.never.astype(jnp.int32))
                c = {}
                for n, (q, ready) in enumerate(arrival):
                    with _scope("wait_q"):
                        w1_copy(*q).wait()
                    if n == 2:
                        with _scope("wait_x1"):
                            x_copy(1).wait()
                        *stats, ahead = normalizing(1, 0)
                        ahead = ahead[8:]
                    launch()
                    _run(_rhs_jobs(w1c, r12.at[0], ready))
                    for i in ready:
                        _scatter(c, _OUT[i], pacer.dot(_combine(_LHS[i], block1(1)).astype(BF16), _rhs(w1c, i)))
                    pacer.run(*(stats if n == 2 else [ahead] if n == 3 else []))
                keep(c1, c)
            with _scope("tile1"):
                launch()
                with _scope("wait_x2"):
                    x_copy(2).wait()
                stage1(0, activating(0), *normalizing(2, 1))
                with _scope("wait_w2"):
                    w2_copy.wait()
                stage1(1, activating(1), _rhs_jobs(w2c, r12.at[1], scale=0.5))
                x_copy(4).start()
                mem_copy.start()
                with _scope("wait_w3"):
                    x_copy(3).wait()
                    w3_copy(0).wait()
                w3j = w3_jobs(0)
                stage2(0, w3j[:len(w3j) * W3S // 4], *normalizing(3, 0))

            def slot(u, carry):
                @pl.when(u + 1 < NT)
                def _():
                    x_copy(u + 1).wait()

                @pl.when(u + 2 < NT)
                def _():
                    x_copy(u + 2).start()

                @pl.when(u == 4)
                def _():
                    w3_copy(1).start()

                @pl.when(u == 5)
                def _():
                    w4_copy(0).start()
                    wo_copy(0).start()

                @pl.when(u == 6)
                def _():
                    qkv_fetch(0)

                with _scope("slot"):
                    idle = [lambda gate: None] * 4
                    stage1(0, activating(u - 1) + idle, *renormalizing(u - 3))
                    stage2(u - 2, clearing(u), *normalizing(jnp.minimum(u + 1, NT - 1), 0))
                return carry

            lax.fori_loop(3, NT, slot, 0)
            with _scope("tile7"):
                last = activating(NT - 1)
                halo = [c for c in range(NCB) if shifts[c * 4 // NCB] > 0]
                _run([last[c] for c in halo])
                stage2(NT - 2, [job for c, job in enumerate(last) if c not in halo], *renormalizing(NT - 3, RS))
                stage2(NT - 1, w3j[len(w3j) * W3S // 4:], *renormalizing(NT - 2, RS))
                _run(itertools.chain(*renormalizing(NT - 1)))

        def ffn(w4c, *g):
            N3 = S // 2 // R3
            never = _never(xb)

            def chunk(f, carry):
                @pl.when(f + 2 < NF)
                def _():
                    w3_copy(f + 2).start()

                @pl.when(f + 1 < NF)
                def _():
                    w4_copy(f + 1).start()
                    w3_copy(f + 1).wait()

                wo_copy(f + 1).start()
                qkv_fetch(f + 1)
                qkv_wait(f)
                w4_copy(f).wait()
                wo_copy(f).wait()
                pacer = _Pacer(never)
                w3f = w3c.at[f % 2]
                pre = {}

                def up(t, *side):
                    for s in range(t * R3 // (2 * RU), (t + 1) * R3 // (2 * RU)):
                        c = pre[s] = {}
                        for i in _ORDER:
                            inner = {}
                            for j in _ORDER:
                                a = _get_wide(yc, 7 * i + j, pl.ds(s * RU // 2, RU // 2))
                                _scatter(inner, _OUT[j], pacer.dot(a, _get_wide(w3f, 7 * i + j)))
                            for q, v in inner.items():
                                _scatter(c, _OUT[i], v, q)
                    pacer.run(*side)

                def activating(t):
                    def job(k, a, lo, gate):
                        for u, v, b in itertools.product(range(2), repeat=3):
                            g[t % 2][u, pl.ds((2 * k + a) * RU + lo, RD), pl.ds((2 * v + b) * FC // 4, FC // 4)] = (
                                _gelu2(gate(pre[t * R3 // (2 * RU) + k][u, v, a, b][lo:lo + RD])))

                    return _jobs(job, range(R3 // (2 * RU)), range(2), range(0, RU, RD))

                def down(t, *side):
                    for s in range(R3 // (2 * RD)):
                        for i in _ORDER:
                            outer = functools.cache(lambda a, b: _combine(_LHS[i], lambda u, v: g[t % 2][
                                u, pl.ds((2 * s + a) * RD, RD), pl.ds((2 * v + b) * FC // 4, FC // 4)]))
                            where = {
                                (a, b): (i, pl.ds(t * R3 + (2 * s + a) * RD, RD), pl.ds(b * HD // 2, HD // 2))
                                for a in range(2) for b in range(2)
                            }
                            acc = {k: macc[idx] for k, idx in where.items()}
                            for j in _ORDER:
                                a = _combine(_LHS[j], outer).astype(BF16)
                                _scatter(acc, _OUT[j], pacer.dot(a, _get_wide(w4c, 7 * i + j)))
                            for k, idx in where.items():
                                macc[idx] = acc[k]
                    pacer.run(*side)

                side = [qkv_jobs(f), wo_jobs(f)]
                w3j = w3_jobs(f + 1)
                total = sum(WS)
                at = 0

                def take(n):
                    nonlocal at
                    at += n
                    return [l[len(l) * (at - n) // total:len(l) * at // total] for l in side]

                with _scope("chunk"):
                    w4j = _rhs2_jobs(w4c, r4.at[f % 2])
                    cut = len(w4j) * W4 // 8
                    up(0, w4j[:cut], *take(WS[0]))
                    up(1, activating(0), w4j[cut:], *take(WS[1]))
                    down(0, _share(w3j, 0, 3), *take(WS[2]))
                    up(2, activating(1), *take(WS[3]))
                    down(1, _share(w3j, 1, 3), *take(WS[4]))
                    up(3, activating(2), *take(WS[5]))
                    down(2, activating(3), *take(WS[6]))
                    down(3, _share(w3j, 2, 3), *take(WS[7]))
                return carry

            lax.fori_loop(0, NF, chunk, 0)

        if "1" in PARTS:
            pl.run_scoped(
                token_mixing,
                pltpu.VMEM((2, D, D), BF16),
                pltpu.VMEM((2, T1, D), F32),
                pltpu.VMEM((2, R1, D), F32),
                pltpu.SemaphoreType.DMA((NT,)),
                pltpu.SemaphoreType.DMA((5,)),
            )
        if "3" in PARTS:
            pl.run_scoped(
                ffn,
                _words(49, NCB // 4, FC // 8),
                pltpu.VMEM((2, R3, FC), F32),
                pltpu.VMEM((2, R3, FC), F32),
            )
        else:
            for cp in (w3_copy(1), w4_copy(0), wo_copy(0), mem_copy):
                cp.wait()
            qkv_wait(0)
            k = xb[0:8, 0:128].astype(jnp.int32)[0, 0]
            xb[0:16, 0:128] = yc[k, k, 0:16].astype(F32).astype(BF16) + w3c[k, k, k, 0:16].astype(F32).astype(BF16)

    def recurrence(res, gq, fq, ob, oc, go, sem_out):
        L = M + SEG
        PR = PERIOD * SEG
        HR = PR // 2
        QR = PR // 4
        NPER = (S // SEG - 1) // PERIOD
        assert NPER * PR + SEG == S
        scale = DH ** -0.5
        row = lax.broadcasted_iota(jnp.int32, (L, L), 0)
        col = lax.broadcasted_iota(jnp.int32, (L, L), 1)
        mask = (row < M) | (row >= col)

        def w_in(w, p, g):
            return _get(wqkv, (w, pl.ds((p * NG + g) * LANES // 2, LANES // 2)))

        def out_copy(r0, n):
            return pltpu.make_async_copy(res.at[pl.ds(r0, n)], out_hbm.at[pl.ds(r0, n)], sem_out)

        def emit(r0, attended):
            n = attended.shape[0]
            c = {}
            for i in _ORDER:
                _scatter(c, _OUT[i], macc[i, pl.ds(pl.multiple_of(r0 // 2, PACK), n // 2), :])
            ffn = jnp.concatenate([
                jnp.concatenate([c[u, 0][r:r + PACK], c[u, 1][r:r + PACK]], axis=1)
                for r in range(0, n // 2, PACK) for u in range(2)], axis=0)
            rows = pl.ds(r0, n)
            res[rows, :] = (xb[rows, :].astype(F32) + base[rows, :] + 0.5 * ffn + attended).astype(BF16)

        def quarter(a, halves):
            return pl.ds(a * HR + halves[0] * QR, len(halves) * QR)

        wo_copy(NF).wait()
        qkv_wait(NF)
        mem_copy.wait()
        with _scope("a_pro"):
            pacer = _Pacer(_never(xb))

            def clear(h, gate):
                ob[h] = z = gate(jnp.zeros((PR, DH), F32))
                if h < NCB:
                    go[:, pl.ds(h * LANES, LANES)] = z

            tokens = xn[pl.ds(0, PR), :].astype(F32)
            lhs = {p: _combine(_HK_LHS[p], lambda a, i: _lanes(tokens, i)[a * HR:(a + 1) * HR]).astype(BF16)
                   for p in _HK_ORDER}
            for w, g in itertools.product(range(3), range(NG)):
                c = {}
                for p in _HK_ORDER:
                    _scatter(c, _HK_OUT[p], pacer.dot(lhs[p], w_in(w, p, g)))
                for (a, j), v in c.items():
                    gq[w, g * NB + j, pl.ds(a * HR, HR), :] = v
                if (w, g) == (1, NG - 1):
                    pacer.run(qkv_jobs(NF))
            pacer.run(wo_jobs(NF), _jobs(clear, range(H)))

        def period(it, mem):
            done = pl.multiple_of(jnp.maximum(it - 2, 0) * PR, PR)
            tokens = xn[pl.ds(pl.multiple_of((it + 1) * PR, PR), PR), :].astype(F32)
            emit(done, go[...])
            for step in range(PERIOD):
                mem = segment(step, tokens, mem)

            @pl.when(it >= 2)
            def _():
                out_copy(done, PR).start()

            return mem

        def segment(step, tokens, mem):
            entries = _HK_STEPS[step]
            rows = pl.ds(step * SEG, SEG)
            begun = {
                k + (half,)
                for p, halves, _, _ in itertools.chain(*_HK_STEPS[:step])
                for half in halves for k, c in np.ndenumerate(_HK_OUT[p]) if c
            }

            def operand(entry, mem_block, token_block):
                p, halves, mem_lhs, _ = entry
                a = jnp.concatenate([
                    _combine(mem_lhs, mem_block),
                    _combine(_HK_LHS[p], lambda a, i: token_block(quarter(a, halves), i))], axis=0)
                return a if a.shape[0] % PACK else a.astype(BF16)

            def fold(entry, r, mem_acc, token_acc, partial):
                p, halves, _, mem_out = entry
                _scatter(mem_acc, mem_out, r[:M])
                for n, half in enumerate(halves):
                    _scatter(token_acc, _HK_OUT[p], r[M + n * QR:M + (n + 1) * QR], (half,),
                             lambda a, j, h: partial(quarter(a, (h,)), j) if (a, j, h) in begun else None)

            lhs = [
                operand(e, lambda i: _lanes(mem, i), lambda r, i: _lanes(tokens, i)[r.start:r.start + r.size])
                for e in entries
            ]
            qkv_mem, prob, att_mem, new_mem, out_acc = {}, {}, {}, {}, {}

            def project(g, w):
                if step == 0:
                    for h in range(g * NB, (g + 1) * NB):
                        fq[w, h] = gq[w, h]
                        if w == 0:
                            oc[h] = ob[h]
                mem_acc, token_acc = {}, {}

                def one(a, e):
                    fold(e, _dot(a, w_in(w, e[0], g)), mem_acc, token_acc, lambda r, j: gq[w, g * NB + j, r, :])

                def finish():
                    for (a, j, half), v in token_acc.items():
                        gq[w, g * NB + j, quarter(a, (half,)), :] = v
                    for (j,), v in mem_acc.items():
                        qkv_mem[w, g * NB + j] = v

                return [functools.partial(one, a, e) for a, e in zip(lhs, entries)] + [finish]

            def part(w, h):
                return jnp.concatenate([qkv_mem[w, h], fq[w, h, rows, :]], axis=0)

            def scores(h):
                prob[h] = _softmax_rows(part(0, h), part(1, h), mask, scale)

            def attend(h):
                o = _dot(prob[h], part(2, h))
                att_mem[h] = o[:M]
                ob[h, rows, :] = o[M:]

            def outproj(g, e):
                a = operand(e, lambda i: att_mem[g * NB + i], lambda r, i: oc[g * NB + i, r, :])
                fold(e, _dot(a, _get(wo, (e[0], g))), new_mem, out_acc, lambda r, j: go[r, pl.ds(j * LANES, LANES)])

            def heads(fn, g):
                return _jobs(fn, range(g * NB, (g + 1) * NB))

            def play(*lists):
                for job in _mix(*lists):
                    job()

            todo = _jobs(outproj, range(NG), entries)
            early = len(todo) - len(entries) - sum(TAIL)
            at = 0
            for g in range(NG):
                play(project(g, 0))
                play(project(g, 1), heads(attend, g - 1) if g else [])
                values = project(g, 2)
                lead = len(values) // (4 if g == NG - 1 else 2)
                play(values[:lead])
                play(values[lead:lead + len(values) // 2], heads(scores, g))
                play(values[lead + len(values) // 2:])
                play(todo[at:min(early, g * len(entries))])
                at = min(early, g * len(entries))
            play(todo[at:at + TAIL[0]])
            play(todo[at + TAIL[0]:at + sum(TAIL)], heads(attend, NG - 1))
            play(todo[at + sum(TAIL):])
            for (a, j, half), v in out_acc.items():
                go[quarter(a, (half,)), pl.ds(j * LANES, LANES)] = v
            return jnp.concatenate([new_mem[j,] for j in range(NB)], axis=1)

        with _scope("a_loop"):
            mem = lax.fori_loop(0, NPER, period, mem0[...].astype(F32))

        with _scope("a_epi"):
            emit((NPER - 2) * PR, go[...])
            out_copy((NPER - 2) * PR, PR).start()
            rows = pl.ds(0, SEG)
            ER = (PR + SEG) // 2
            lhs = [_combine(e[2], lambda i: _lanes(mem, i)) for e in _HK_STEPS[0]]
            kv_mem, prob, att, out_acc = {}, {}, {}, {}

            def project(w, g):
                acc = {}
                for a, (p, _, _, mem_out) in zip(lhs, _HK_STEPS[0]):
                    _scatter(acc, mem_out, _dot(a, w_in(w, p, g)))
                for (j,), v in acc.items():
                    kv_mem[w, g * NB + j] = jnp.concatenate([v, gq[w, g * NB + j, rows, :]], axis=0)

            def block(a, h):
                if a == 0:
                    return ob[h, pl.ds(0, ER), :]
                return jnp.concatenate([ob[h, pl.ds(ER, PR - ER), :], att[h]], axis=0)

            for t in range(NG + 2):
                if t < NG:
                    project(1, t)
                    project(2, t)
                    for h in range(t * NB, (t + 1) * NB):
                        prob[h] = _softmax_rows(gq[0, h, rows, :], kv_mem[1, h], mask[M:], scale)
                if 0 <= t - 2:
                    for p in _HK_ORDER:
                        a = _combine(_HK_LHS[p], lambda a, i: block(a, (t - 2) * NB + i))
                        _scatter(out_acc, _HK_OUT[p], _dot(a, _get(wo, (p, t - 2))))
                if 0 <= t - 1 < NG:
                    for h in range((t - 1) * NB, t * NB):
                        att[h] = _dot(prob[h], kv_mem[2, h])
            r0 = (NPER - 1) * PR
            for a in range(2):
                emit(r0 + a * ER, jnp.concatenate([out_acc[a, j] for j in range(NB)], axis=1))
            out_copy(r0, 2 * ER).start()
        with _scope("tail"):
            out_copy(0, S).wait()

    if "1" in PARTS or "3" in PARTS:
        pl.run_scoped(
            mixer,
            _words(49, NCB // 4, S // 8),
            _words(2, 49, FC // 4 // LANES, HD // 4),
            pltpu.VMEM((2, D, FC), BF16),
            pltpu.VMEM((2, FC, D), BF16),
            pltpu.SemaphoreType.DMA((2, 2)),
        )
    if "A" not in PARTS:
        k = xb[0:8, 0:128].astype(jnp.int32)[0, 0]
        k16 = pl.ds(pl.multiple_of(k * 16, 16), 16)
        xb[0:16, 0:128] = (_get(wqkv, (k, pl.ds(0, 8))) + _get(wo, (k, k, pl.ds(0, 8)))
                           + xn[k16, 0:128] + macc[k, k16, 0:128].astype(BF16) + base[k16, 0:128].astype(BF16))
        pltpu.sync_copy(xb, out_hbm)
        return
    pl.run_scoped(
        recurrence,
        pltpu.VMEM((S, D), BF16),
        pltpu.VMEM((3, H, PERIOD * SEG, DH), F32),
        pltpu.VMEM((3, H, PERIOD * SEG, DH), F32),
        pltpu.VMEM((H, PERIOD * SEG, DH), F32),
        pltpu.VMEM((H, PERIOD * SEG, DH), F32),
        pltpu.VMEM((PERIOD * SEG, D), F32),
        pltpu.SemaphoreType.DMA(()),
    )


@functools.partial(jax.jit, static_argnames=("A_seg_len",))
def pallas_parallel_sum__memory_aug_recurrent_mem_tr__mixer_s_mlp__prompt_kernel(
    A_x: jax.Array,
    A_mem0: jax.Array,
    A_Wq: jax.Array,
    A_Wk: jax.Array,
    A_Wv: jax.Array,
    A_Wo: jax.Array,
    A_seg_len: int,
    B_x: jax.Array,
    B_w1: jax.Array,
    B_w2: jax.Array,
    B_w3: jax.Array,
    B_w4: jax.Array,
):
    del B_x
    B, S, D = A_x.shape
    _, H, DH = A_Wq.shape
    M = A_mem0.shape[1]
    F = B_w3.shape[1]
    SEG = int(A_seg_len)
    assert B == 1 and DH == LANES and D == NB * LANES

    hbm = pl.BlockSpec(memory_space=pl.ANY)
    out = pl.pallas_call(
        functools.partial(_kernel, S=S, D=D, H=H, DH=DH, M=M, SEG=SEG, F=F),
        out_shape=jax.ShapeDtypeStruct((S, D), A_x.dtype),
        in_specs=[hbm] * 10,
        out_specs=hbm,
        scratch_shapes=[
            pltpu.VMEM((S, D), BF16),
            pltpu.VMEM((S + (PERIOD - 1) * SEG, D), BF16),
            pltpu.VMEM((S, D), F32),
            pltpu.VMEM((7, S // 2, D // 2), F32),
            _words(3, NPROD * H // NB * LANES // 2),
            _words(NPROD, H // NB, LANES // 2),
            pltpu.VMEM((2, 3, NB, PACK * H, LANES), BF16),
            _words(3, NB, H // 2 * (PACK + 1)),
            pltpu.VMEM((2, H, PACK, D), BF16),
            pltpu.VMEM((M, D), BF16),
            pltpu.SemaphoreType.DMA(()),
            pltpu.SemaphoreType.DMA((2, 3)),
            pltpu.SemaphoreType.DMA((2,)),
        ],
        compiler_params=pltpu.CompilerParams(vmem_limit_bytes=127 * 1024 * 1024, flags=FLAGS, disable_bounds_checks=True),
    )(
        A_x.reshape(S, D),
        A_mem0.reshape(M, D),
        A_Wq.reshape(NB, LANES * H, DH),
        A_Wk.reshape(NB, LANES * H, DH),
        A_Wv.reshape(NB, LANES * H, DH),
        A_Wo,
        B_w1, B_w2, B_w3, B_w4,
    )
    return out.reshape(B, S, D)
```

```python
import contextlib
import functools
import itertools
import math

import jax
import jax.numpy as jnp
import numpy as np
from jax import lax
from jax.experimental import pallas as pl
from jax.experimental.pallas import tpu as pltpu

F32 = jnp.float32
BF16 = jnp.bfloat16
U32 = jnp.uint32
LANES = 128
SUB = 8
PACK = 16
EPS = 1e-5
R1 = 128
RU = 64
RD = 32
R3 = 256
FC = 512
PERIOD = 3
WS = (0, 4, 0, 4, 0, 4, 1, 0)
W4 = 8
TAIL = (40, 24)
NS = 2
RS = 1
W3S = 3
PLAN = "0a///b/c/1/d2/w//3v"
SCOPES = False
PARTS = "13A"
FLAGS = {'XLA_TPU_EVENLY_DISTRIBUTE_CRITICAL_NODES': True}


def _scope(name):
    return jax.named_scope(name) if SCOPES else contextlib.nullcontext()


def _layernorm_jobs(read, count, finish, slack):
    mean, var = {}, {}

    def first(k, gate):
        mean[k] = jnp.mean(read(0, k, gate), axis=-1, keepdims=True)

    def second(k, gate):
        d = read(1, k, gate) - mean[k]
        var[k] = jnp.mean(d * d, axis=-1, keepdims=True)

    def idle(gate):
        pass

    last = [finish(k, mean, var) for k in range(count)]
    n = len(last[0])
    return [
        _jobs(first, range(count)) + [idle] * (2 + slack),
        [idle] + _jobs(second, range(count)) + [idle] * (1 + slack),
        [idle] * 2 * n + list(itertools.chain(*last)) + [idle] * slack * n,
    ]


def _gate_first(gate, v):
    return jnp.concatenate([gate(v[:, :LANES]), v[:, LANES:]], axis=1)


def _gelu2(x):
    c = math.sqrt(2 / math.pi)
    return x + x * jnp.tanh(x * (c + (c * 0.044715) * (x * x)))


def _softmax_rows(q, k, mask, scale):
    z = lax.dot_general(q, k, (((1,), (1,)), ((), ())), preferred_element_type=F32)
    z = jnp.where(mask, z * scale, -1e9)
    e = jnp.exp(z - jnp.max(z, axis=-1, keepdims=True))
    s = jnp.sum(e, axis=-1, keepdims=True)
    r = pl.reciprocal(s, approx=True)
    return e * (r * (2.0 - s * r))


def _dot(a, b):
    return jnp.dot(a, b, preferred_element_type=F32)


def _put(ref, idx, v):
    ref[idx] = pltpu.bitcast(v.astype(BF16), U32)


def _get(ref, idx):
    return pltpu.bitcast(ref[idx], BF16)


def _get_wide(ref, i, rows=slice(None)):
    return jnp.concatenate([_get(ref, (i, c, rows)) for c in range(ref.shape[1])], axis=1)


def _words(*shape):
    return pltpu.VMEM(shape + (LANES,), U32)


def _lanes(v, c):
    return v[:, c * LANES:(c + 1) * LANES]


def _combine(coef, get):
    terms = sorted(((int(c), k) for k, c in np.ndenumerate(coef) if c), key=lambda t: -t[0])
    out = get(*terms[0][1]) if terms[0][0] > 0 else -get(*terms[0][1])
    for c, k in terms[1:]:
        out = out + get(*k) if c > 0 else out - get(*k)
    return out


def _scatter(acc, coef, v, tag=(), start=None):
    for k, c in np.ndenumerate(coef):
        if not c:
            continue
        k = k + tag
        if k not in acc and start is not None and (old := start(*k)) is not None:
            acc[k] = old
        if k in acc:
            acc[k] = acc[k] + v if c > 0 else acc[k] - v
        else:
            acc[k] = v if c > 0 else -v


_LHS = np.array([[1, 0, 0, 1], [0, 0, 1, 1], [1, 0, 0, 0], [0, 0, 0, 1],
                 [1, 1, 0, 0], [-1, 0, 1, 0], [0, 1, 0, -1]]).reshape(7, 2, 2)
_RHS = np.array([[1, 0, 0, 1], [1, 0, 0, 0], [0, 1, 0, -1], [-1, 0, 1, 0],
                 [0, 0, 0, 1], [1, 1, 0, 0], [0, 0, 1, 1]]).reshape(7, 2, 2)
_OUT = np.array([[1, 0, 0, 1], [0, 0, 1, -1], [0, 1, 0, 1], [1, 0, 1, 0],
                 [-1, 1, 0, 0], [0, 0, 0, 1], [1, 0, 0, 0]]).reshape(7, 2, 2)
_ORDER = (0, 3, 1, 2, 4, 5, 6)


def _hopcroft_kerr():
    n = 8
    method = (0, 1, 2, 0, 1, 2, 0, 1)
    stand_in = {(0, 3): (0, 2), (0, 6): (6, 2), (3, 6): (3, 2), (1, 4): (1, 5),
                (1, 7): (7, 5), (4, 7): (4, 5), (2, 5): (2, 7)}
    left_out = ("000010010001000022020010002002000200",
                "101101101210121210212121211211211011",
                "111111112122212101101202120120122122")
    forms = np.array([[[[1, 0], [1, 1]], [[-1, 1], [0, 1]]],
                      [[[0, 1], [1, 1]], [[1, -1], [1, 0]]],
                      [[[1, 0], [1, 0]], [[0, 1], [0, 1]]]])
    turn_a, turn_c = np.array([[0, -1], [1, 1]]), np.array([[1, -1], [1, 0]])
    eye = np.eye(n, dtype=int)
    lhs, out, groups, node, inner = [], [], [], {}, {}

    def product(a, c):
        lhs.append(a)
        out.append(c)
        groups[-1].append(len(lhs) - 1)
        return np.eye(100, dtype=int)[len(lhs) - 1]

    def add_node(key, a, c, m):
        groups.append([])
        node[key] = (a, c, m, [product(np.outer(f, a), np.outer(g, c)) for f, g in forms[m]])

    def pair(p, q):
        swap = (node[q][2] - node[p][2]) % 3 != 1
        (ai, ci, mi, di), (aj, cj, _, dj) = (node[q], node[p]) if swap else (node[p], node[q])
        sa, sc = (np.linalg.matrix_power(t, -mi % 3) for t in (turn_a, turn_c))
        add_node((p, q), ai + aj, ci - cj, (mi + 2) % 3)
        cross = product(np.outer(sa[:, 0], ai) + np.outer(sa[:, 1], aj),
                        np.outer(sc[:, 0], cj) + np.outer(sc[:, 1], ci))

        def turned(m, t, products):
            want = np.outer(sa @ forms[m, t, 0], sc @ forms[m, t, 1])
            return next(v for v, (f, g) in zip(products, forms[(m + mi) % 3]) if (np.outer(f, g) == want).all())

        dv = node[p, q][3]
        ij = cross - turned(2, 1, dv) - turned(1, 0, dj) + turned(0, 1, di)
        ji = cross + turned(2, 0, dv) - turned(0, 0, di) + turned(1, 1, dj)
        return (ji, ij) if swap else (ij, ji)

    for i in range(n):
        add_node(i, eye[i], eye[i], method[i])
        inner[i, i] = sum(node[i][3])
    for i, j in itertools.combinations(range(n), 2):
        if method[i] != method[j]:
            inner[i, j], inner[j, i] = pair(i, j)
    for (i, j), (u, k) in sorted(stand_in.items()):
        v, w = (min(u, k), max(u, k)), i + j - u
        vw, wv = pair(v, w)
        inner[u, w] = vw - inner[k, w]
        inner[w, u] = node[v][1][u] * wv + inner[w, k]
    lhs, out = np.array(lhs), np.array(out)
    rhs = np.array([[inner[i, j] for j in range(n)] for i in range(n)]).transpose(2, 0, 1)
    assert (np.einsum("pri,pjk,psl->rijksl", lhs, rhs, out)
            == np.einsum("rs,ij,kl->rijksl", np.eye(2, dtype=int), eye, eye)).all()

    used = [sorted(p for g, d in zip(groups, text) for p in g if p != g[int(d)]) for text in left_out]
    steps = []
    for s, products in enumerate(used):
        basis = rhs[products].reshape(n * n, n * n)
        dual = np.rint(np.linalg.inv(basis).T).astype(int)
        assert (basis.T @ dual == np.eye(n * n)).all()
        entries = []
        for p, u in zip(products, dual.reshape(-1, n, n)):
            i, j = np.argwhere(u)[0]
            mem_lhs, mem_out = u[:, j] * u[i, j], u[i]
            assert (np.outer(mem_lhs, mem_out) == u).all()
            when = [t for t in range(PERIOD) if p in used[t]]
            halves = (0, 1) if len(when) == 1 else (when.index(s),)
            entries.append((p, halves, mem_lhs, mem_out))
        steps.append(entries)

    def locality(p):
        idx = np.nonzero(np.abs(out[p]).sum(0))[0]
        a, b = idx.min() // 2, idx.max() // 2
        return (a, -b if a % 2 else b, tuple(idx))

    steps = [sorted(e, key=lambda t: (t[1] == (1,), locality(t[0]))) for e in steps]
    return lhs, rhs, out, steps, sorted(range(len(lhs)), key=locality)


_HK_LHS, _HK_RHS, _HK_OUT, _HK_STEPS, _HK_ORDER = _hopcroft_kerr()
NB, NPROD = _HK_RHS.shape[1], _HK_RHS.shape[0]


def _share(jobs, k, n):
    return jobs[len(jobs) * k // n:len(jobs) * (k + 1) // n]


def _mix(*lists):
    keyed = [((n + 0.5) / len(l), k, n) for k, l in enumerate(lists) for n in range(len(l))]
    return [lists[k][n] for _, k, n in sorted(keyed)]


def _jobs(fn, *ranges):
    return [functools.partial(fn, *k) for k in itertools.product(*ranges)]


def _run(jobs):
    for job in jobs:
        job(lambda v: v)


def _never(ref):
    return jnp.abs(ref[0:SUB, 0:LANES].astype(F32)) < 0.0


class _Pacer:
    def __init__(self, never):
        self.never = never
        self.tokens = []

    def dot(self, a, b):
        m = _dot(a, b)
        rounds = min(max(a.shape[1] * m.shape[1] // (4 * LANES * LANES), 1), m.shape[1] // LANES)
        self.tokens += [
            m[r:r + SUB, c:c + LANES]
            for c in range(0, m.shape[1], m.shape[1] // rounds) for r in range(0, m.shape[0], SUB)
        ]
        return m

    def run(self, *job_lists):
        tokens, self.tokens = self.tokens, []

        def gate(k, count, v):
            n = v.shape[0] // SUB
            rows = []
            for r in range(n):
                t = lax.bitcast_convert_type(tokens[len(tokens) * (k * n + r) // (count * n)], v.dtype)
                rows.append(jnp.concatenate([
                    jnp.where(self.never, t, v[r * SUB:(r + 1) * SUB, c:c + LANES])
                    for c in range(0, v.shape[1], LANES)], axis=1))
            return jnp.concatenate(rows, axis=0)

        for job in _mix(*[
            [functools.partial(job, functools.partial(gate, k, len(jobs))) for k, job in enumerate(jobs)]
            for jobs in job_lists
        ]):
            job()


def _rhs(w, i):
    n = w.shape[0] // 7
    return jnp.concatenate([_get_wide(w, n * i + k) for k in range(n)], axis=0)


def _strassen(block, w, pacer, side, start=None):
    c = {}
    for i in _ORDER:
        _scatter(c, _OUT[i], pacer.dot(_combine(_LHS[i], block).astype(BF16), _rhs(w, i)), start=start)
    pacer.run(*side)
    return c


def _rhs_jobs(dst, src, which=range(7), scale=None):
    kh, nh, rows = src.shape[0] // 2, src.shape[1] // 2, 64

    def job(c, k0, gate):
        @functools.cache
        def block(a, b):
            v = gate(src[pl.ds(a * kh + k0, rows), pl.ds(b * nh + c * LANES, LANES)].astype(F32))
            return v if scale is None else scale * v

        for i in which:
            k, r = divmod((i * kh + k0) // 2, dst.shape[2])
            _put(dst, (k, c, pl.ds(r, rows // 2)), _combine(_RHS[i], block))

    return _jobs(job, range(nh // LANES), range(0, kh, rows))


def _rhs2_jobs(dst, src):
    kq, nq = src.shape[0] // 4, src.shape[1] // 4

    @functools.cache
    def block(c, k0, a, b):
        return src[pl.ds(a * kq + k0, PACK), pl.ds(b * nq + c * LANES, LANES)].astype(F32)

    def job(c, k0, i, gate):
        outer = functools.cache(lambda a, b: gate(_combine(_RHS[i], lambda u, v: block(c, k0, 2 * u + a, 2 * v + b))))
        for j in range(7):
            _put(dst, (7 * i + j, c, pl.ds(k0 // 2, SUB)), _combine(_RHS[j], outer))

    return _jobs(job, range(nq // LANES), range(0, kq, PACK), range(7))


def _hk_jobs(block, store):
    def job(p, gate):
        first = tuple(np.argwhere(_HK_RHS[p])[0])
        store(p, _combine(_HK_RHS[p], lambda i, j: gate(block(i, j)) if (i, j) == first else block(i, j)))

    return _jobs(job, _HK_ORDER)


def _kernel(
    x_hbm, mem_hbm, wq_hbm, wk_hbm, wv_hbm, wo_hbm, w1_hbm, w2_hbm, w3_hbm, w4_hbm,
    out_hbm,
    xb, xn, base, macc, wqkv, wo, raw, mid, raw_o, mem0, sem_m, sem_a, sem_o,
    *, S, D, H, DH, M, SEG, F,
):
    HD = D // 2
    NCB = D // LANES
    NG = H // NB
    T1 = 2 * R1
    NT = S // T1
    NF = F // FC
    assert LANES // PACK == NF + 1

    mem_copy = pltpu.make_async_copy(mem_hbm, mem0, sem_m)

    def wo_copy(part):
        rows = pl.ds(pl.multiple_of(part * PACK, PACK), PACK)
        return pltpu.make_async_copy(wo_hbm.at[:, rows], raw_o.at[part % 2], sem_o.at[part % 2])

    def wo_jobs(part):
        dst = wo.at[:, :, pl.ds(pl.multiple_of(part * SUB, SUB), SUB)]
        src = raw_o.at[part % 2]

        def group(g):
            block = functools.cache(lambda i, j: src[g * NB + i, :, pl.ds(j * LANES, LANES)].astype(F32))
            return _hk_jobs(block, lambda p, v: _put(dst, (p, g), v))

        return [job for g in range(NG) for job in group(g)]

    def qkv_unit(n, k):
        return divmod(3 * n + k, NF + 1)

    def qkv_fetch(n):
        for k in range(3):
            w, part = qkv_unit(n, k)
            rows = pl.ds(pl.multiple_of(part * PACK * H, PACK * H), PACK * H)
            for which, src in enumerate((wq_hbm, wk_hbm, wv_hbm)):
                @pl.when(w == which)
                def _():
                    pltpu.make_async_copy(src.at[:, rows], raw.at[n % 2, k], sem_a.at[n % 2, k]).start()

    def qkv_wait(n):
        for k in range(3):
            pltpu.make_async_copy(wq_hbm.at[:, pl.ds(0, PACK * H)], raw.at[n % 2, k], sem_a.at[n % 2, k]).wait()

    def qkv_jobs(n):
        src = raw.at[n % 2]

        def transpose(k, half, i, gate):
            rows = gate(jnp.concatenate([
                pltpu.bitcast(src[k, i, pl.ds(d * H + half * PACK, PACK), :], U32) for d in range(PACK)], axis=0))
            for d in range(PACK):
                mid[k, i, pl.ds(half * SUB * (PACK + 1) + d, SUB, stride=PACK + 1), :] = rows[d * SUB:(d + 1) * SUB]

        def group(k, g, dst):
            words = functools.cache(lambda i, pair: mid[k, i, pl.ds((g * NB // 2 + pair) * (PACK + 1), PACK), :])
            block = functools.cache(lambda i, j: pltpu.bitcast(
                words(i, j // 2) & jnp.uint32(0xFFFF0000) if j % 2 else words(i, j // 2) << 16, F32))
            return _hk_jobs(block, lambda p, v: _put(dst, pl.ds((p * NG + g) * LANES // 2, SUB), v))

        moves, sums = [], [[]]
        for k in range(3):
            w, part = qkv_unit(n, k)
            dst = wqkv.at[w, pl.ds(pl.multiple_of(part * SUB, SUB), wqkv.shape[1] - NF * SUB)]
            for half in range(H // PACK):
                moves.append(_jobs(transpose, [k], [half], range(NB)))
                sums.append(group(k, 2 * half, dst) + group(k, 2 * half + 1, dst))
        return [job for a, b in zip(moves + [[]], sums) for job in _mix(a, b)]

    def mixer(yc, w3c, r3, r4, sem_f):
        def w3_copy(f):
            cols = pl.ds(pl.multiple_of(f * FC, FC), FC)
            return pltpu.make_async_copy(w3_hbm.at[:, cols], r3.at[f % 2], sem_f.at[0, f % 2])

        def w4_copy(f):
            rows = pl.ds(pl.multiple_of(f * FC, FC), FC)
            return pltpu.make_async_copy(w4_hbm.at[rows], r4.at[f % 2], sem_f.at[1, f % 2])

        def w3_jobs(f):
            return _rhs2_jobs(w3c.at[f % 2], r3.at[f % 2])

        def token_mixing(r12, y0, c1, sem_x, sem_w):
            w1c, w2c = (wo.at[pl.ds(n * 7 * HD // LANES, 7 * HD // LANES)] for n in range(2))
            shifts = (-1, 1, -2, 2)
            HP = S + 2 * SUB

            def x_copy(t):
                rows = pl.ds(pl.multiple_of(t * T1, T1), T1)
                return pltpu.make_async_copy(x_hbm.at[rows], xb.at[rows], sem_x.at[t])

            def w1_copy(a, b):
                idx = (pl.ds(a * HD, HD), pl.ds(b * HD, HD))
                return pltpu.make_async_copy(w1_hbm.at[idx], r12.at[(0,) + idx], sem_w.at[2 * a + b])

            w2_copy = pltpu.make_async_copy(w2_hbm, r12.at[1], sem_w.at[4])

            def tile(ref, t, view=0):
                return ref.at[pl.ds(pl.multiple_of(t * T1 + view * zero, T1), T1)]

            def normalizing(t, slot):
                xs, xn_t, n = [tile(xb, t, v) for v in range(3)], tile(xn, t), 2 * PACK

                def finish(k, mean, var):
                    def job(c, gate):
                        rows, cols = pl.ds(k * n, n), pl.ds(c * HD // 2, HD // 2)
                        r = lax.rsqrt(var[k] + EPS)
                        v = (xs[2][rows, cols].astype(F32) - wide(gate, mean[k], HD // 2)) * r
                        xn_t[rows, cols] = v.astype(BF16)
                        y0[slot, rows, cols] = v * lax.rsqrt(var[k] * r * r + EPS)

                    return _jobs(job, range(4))

                return _layernorm_jobs(
                    lambda v, k, gate: _gate_first(gate, xs[v][pl.ds(k * n, n), :].astype(F32)), T1 // n, finish, NS)

            def wide(gate, column, width):
                v = gate(jnp.broadcast_to(column, (column.shape[0], LANES)))
                return jnp.concatenate([v] * (width // LANES), axis=1)

            def keep(dst, c):
                for (a, b), v in c.items():
                    dst[a, :, pl.ds(b * HD, HD)] = v

            def block1(slot):
                return lambda a, b: y0[slot, pl.ds(a * R1, R1), pl.ds(b * HD, HD)]

            def stage1(slot, *side):
                keep(c1, _strassen(block1(slot), w1c, pacer, side))

            def h_from(t):
                return wqkv.at[0, pl.ds(pl.multiple_of(t * T1, T1), (NCB - 1) * HP + T1 + 2 * SUB)]

            def activating(t):
                hb_t = h_from(t)

                def job(a, c, gate):
                    h = _gelu2(gate(c1[a, :, pl.ds(c * LANES, LANES)]))
                    hb_t[pl.ds(c * HP + SUB + a * R1, R1), :] = pltpu.bitcast(h, U32)

                return _jobs(job, range(2), range(NCB))

            def stage2(t, *side, lo=0, n=R1):
                hb_t, base_t, xn_t = h_from(t), tile(base, t), tile(xn, t)
                c = _strassen(lambda a, b: jnp.concatenate([
                    pltpu.bitcast(hb_t[pl.ds(c * HP + SUB + a * R1 + lo + shifts[c * 4 // NCB], n), :], F32)
                    for c in range(b * NCB // 2, (b + 1) * NCB // 2)], axis=1), w2c, pacer, side,
                    lambda a, b: xn_t[pl.ds(a * R1 + lo, n), pl.ds(b * HD, HD)].astype(F32))
                for (a, b), v in c.items():
                    base_t[pl.ds(a * R1 + lo, n), pl.ds(b * HD, HD)] = v

            def renormalizing(t, slack=0, starts=range(0, RU, PACK)):
                xs = [tile(base, t, v) for v in range(3)]
                yc_t = yc.at[:, :, pl.ds(pl.multiple_of(t * (RU // 2), RU // 2), RU // 2)]

                def read(view, k, cols):
                    return jnp.concatenate([
                        xs[view][pl.ds(2 * (a * RU + starts[k]) + u * PACK, PACK), cols]
                        for u in range(2) for a in range(2)], axis=0)

                def finish(k, mean, var):
                    y = {}

                    def job(c, i, gate):
                        if i == 0:
                            m, r = wide(gate, mean[k], LANES), lax.rsqrt(var[k] + EPS)
                            for q in range(4):
                                y[c, q] = (read(2, k, pl.ds(q * HD // 2 + c * LANES, LANES)) - m) * r
                        outer = functools.cache(lambda a, b: gate(_combine(
                            _LHS[i], lambda u, v: y[c, 2 * v + b][(2 * u + a) * PACK:(2 * u + a + 1) * PACK])))
                        for j in range(7):
                            _put(yc_t, (7 * i + j, c, pl.ds(starts[k] // 2, SUB)), _combine(_LHS[j], outer))

                    return _jobs(job, range(NCB // 4), range(7))

                return _layernorm_jobs(
                    lambda v, k, gate: _gate_first(gate, read(v, k, slice(None))), len(starts), finish, slack)

            arrival = (((0, 0), (1,)), ((1, 1), (4, 0)), ((0, 1), (2, 5)), ((1, 0), (3, 6)))
            quarters = [w1_copy(*q) for q, _ in arrival]
            named = dict(a=quarters[0], b=quarters[1], c=quarters[2], d=quarters[3], w=w2_copy, v=w3_copy(0))
            queue = [[x_copy(int(k)) if k.isdigit() else named[k] for k in step] for step in PLAN.split("/")]

            def launch():
                for cp in queue.pop(0):
                    cp.start()

            launch()
            for c in range(NCB):
                wqkv[0, pl.ds(c * HP, SUB), :] = jnp.zeros((SUB, LANES), U32)
                wqkv[0, pl.ds(c * HP + SUB + S, SUB), :] = jnp.zeros((SUB, LANES), U32)


            def clearing(t):
                acc_t = macc.at[:, pl.ds(pl.multiple_of(t * R1, R1), R1)]

                def job(i, lo, gate):
                    acc_t[i, pl.ds(lo, PACK), :] = wide(gate, jnp.zeros((PACK, 1), F32), HD)

                return _jobs(job, range(7), range(0, R1, PACK))

            for t in range(3):
                _run(clearing(t))
                launch()
            pad = xn.shape[0] - S
            xn[pl.ds(S, pad), :] = jnp.zeros((pad, D), BF16)
            with _scope("wait_x0"):
                x_copy(0).wait()
            launch()
            pacer = _Pacer(_never(xb))
            zero = 0
            with _scope("tile0"):
                _run(itertools.chain(*normalizing(0, 1)))
                zero = jnp.max(pacer.never.astype(jnp.int32))
                c = {}
                for n, (q, ready) in enumerate(arrival):
                    with _scope("wait_q"):
                        w1_copy(*q).wait()
                    if n == 2:
                        with _scope("wait_x1"):
                            x_copy(1).wait()
                        *stats, ahead = normalizing(1, 0)
                        ahead = ahead[8:]
                    launch()
                    _run(_rhs_jobs(w1c, r12.at[0], ready))
                    for i in ready:
                        _scatter(c, _OUT[i], pacer.dot(_combine(_LHS[i], block1(1)).astype(BF16), _rhs(w1c, i)))
                    pacer.run(*(stats if n == 2 else [ahead] if n == 3 else []))
                keep(c1, c)
            with _scope("tile1"):
                launch()
                with _scope("wait_x2"):
                    x_copy(2).wait()
                stage1(0, activating(0), *normalizing(2, 1))
                with _scope("wait_w2"):
                    w2_copy.wait()
                stage1(1, activating(1), _rhs_jobs(w2c, r12.at[1], scale=0.5))
                x_copy(4).start()
                mem_copy.start()
                with _scope("wait_w3"):
                    x_copy(3).wait()
                    w3_copy(0).wait()
                w3j = w3_jobs(0)
                stage2(0, w3j[:len(w3j) * W3S // 4], *normalizing(3, 0))

            def slot(u, carry):
                @pl.when(u + 1 < NT)
                def _():
                    x_copy(u + 1).wait()

                @pl.when(u + 2 < NT)
                def _():
                    x_copy(u + 2).start()

                @pl.when(u == 4)
                def _():
                    w3_copy(1).start()

                @pl.when(u == 5)
                def _():
                    w4_copy(0).start()
                    wo_copy(0).start()

                @pl.when(u == 6)
                def _():
                    qkv_fetch(0)

                with _scope("slot"):
                    stage1(0, activating(u - 1) + [lambda gate: None] * 4, *renormalizing(u - 3))
                    stage2(u - 2, clearing(u), *normalizing(jnp.minimum(u + 1, NT - 1), 0))
                return carry

            lax.fori_loop(3, NT, slot, 0)
            with _scope("tile7"):
                last = activating(NT - 1)
                halo = [c for c in range(NCB) if shifts[c * 4 // NCB] > 0]
                _run([last[c] for c in halo])
                stage2(NT - 2, [job for c, job in enumerate(last) if c not in halo], *renormalizing(NT - 3, RS))
                stage2(NT - 1, w3j[len(w3j) * W3S // 4:], *renormalizing(NT - 2, RS))
                _run(itertools.chain(*renormalizing(NT - 1)))

        def ffn(w4c, *g):
            N3 = S // 2 // R3
            never = _never(xb)

            def chunk(f, carry):
                @pl.when(f + 2 < NF)
                def _():
                    w3_copy(f + 2).start()

                @pl.when(f + 1 < NF)
                def _():
                    w4_copy(f + 1).start()
                    w3_copy(f + 1).wait()

                wo_copy(f + 1).start()
                qkv_fetch(f + 1)
                qkv_wait(f)
                w4_copy(f).wait()
                wo_copy(f).wait()
                pacer = _Pacer(never)
                w3f = w3c.at[f % 2]
                pre = {}

                def up(t, *side):
                    for s in range(t * R3 // (2 * RU), (t + 1) * R3 // (2 * RU)):
                        c = pre[s] = {}
                        for i in _ORDER:
                            inner = {}
                            for j in _ORDER:
                                a = _get_wide(yc, 7 * i + j, pl.ds(s * RU // 2, RU // 2))
                                _scatter(inner, _OUT[j], pacer.dot(a, _get_wide(w3f, 7 * i + j)))
                            for q, v in inner.items():
                                _scatter(c, _OUT[i], v, q)
                    pacer.run(*side)

                def activating(t):
                    def job(k, a, lo, gate):
                        for u, v, b in itertools.product(range(2), repeat=3):
                            g[t % 2][u, pl.ds((2 * k + a) * RU + lo, RD), pl.ds((2 * v + b) * FC // 4, FC // 4)] = (
                                _gelu2(gate(pre[t * R3 // (2 * RU) + k][u, v, a, b][lo:lo + RD])))

                    return _jobs(job, range(R3 // (2 * RU)), range(2), range(0, RU, RD))

                def down(t, *side):
                    for s in range(R3 // (2 * RD)):
                        for i in _ORDER:
                            outer = functools.cache(lambda a, b: _combine(_LHS[i], lambda u, v: g[t % 2][
                                u, pl.ds((2 * s + a) * RD, RD), pl.ds((2 * v + b) * FC // 4, FC // 4)]))
                            where = {
                                (a, b): (i, pl.ds(t * R3 + (2 * s + a) * RD, RD), pl.ds(b * HD // 2, HD // 2))
                                for a in range(2) for b in range(2)
                            }
                            acc = {k: macc[idx] for k, idx in where.items()}
                            for j in _ORDER:
                                a = _combine(_LHS[j], outer).astype(BF16)
                                _scatter(acc, _OUT[j], pacer.dot(a, _get_wide(w4c, 7 * i + j)))
                            for k, idx in where.items():
                                macc[idx] = acc[k]
                    pacer.run(*side)

                side = [qkv_jobs(f), wo_jobs(f)]
                w3j = w3_jobs(f + 1)
                total = sum(WS)
                at = 0

                def take(n):
                    nonlocal at
                    at += n
                    return [l[len(l) * (at - n) // total:len(l) * at // total] for l in side]

                with _scope("chunk"):
                    w4j = _rhs2_jobs(w4c, r4.at[f % 2])
                    cut = len(w4j) * W4 // 8
                    up(0, w4j[:cut], *take(WS[0]))
                    up(1, activating(0), w4j[cut:], *take(WS[1]))
                    down(0, _share(w3j, 0, 3), *take(WS[2]))
                    up(2, activating(1), *take(WS[3]))
                    down(1, _share(w3j, 1, 3), *take(WS[4]))
                    up(3, activating(2), *take(WS[5]))
                    down(2, activating(3), *take(WS[6]))
                    down(3, _share(w3j, 2, 3), *take(WS[7]))
                return carry

            lax.fori_loop(0, NF, chunk, 0)

        if "1" in PARTS:
            pl.run_scoped(
                token_mixing,
                pltpu.VMEM((2, D, D), BF16),
                pltpu.VMEM((2, T1, D), F32),
                pltpu.VMEM((2, R1, D), F32),
                pltpu.SemaphoreType.DMA((NT,)),
                pltpu.SemaphoreType.DMA((5,)),
            )
        if "3" in PARTS:
            pl.run_scoped(
                ffn,
                _words(49, NCB // 4, FC // 8),
                pltpu.VMEM((2, R3, FC), F32),
                pltpu.VMEM((2, R3, FC), F32),
            )
        else:
            for cp in (w3_copy(1), w4_copy(0), wo_copy(0), mem_copy):
                cp.wait()
            qkv_wait(0)
            k = xb[0:8, 0:128].astype(jnp.int32)[0, 0]
            xb[0:16, 0:128] = yc[k, k, 0:16].astype(F32).astype(BF16) + w3c[k, k, k, 0:16].astype(F32).astype(BF16)

    def recurrence(res, gq, fq, ob, oc, go, sem_out):
        L = M + SEG
        PR = PERIOD * SEG
        HR = PR // 2
        QR = PR // 4
        NPER = (S // SEG - 1) // PERIOD
        assert NPER * PR + SEG == S
        scale = DH ** -0.5
        row = lax.broadcasted_iota(jnp.int32, (L, L), 0)
        col = lax.broadcasted_iota(jnp.int32, (L, L), 1)
        mask = (row < M) | (row >= col)

        def w_in(w, p, g):
            return _get(wqkv, (w, pl.ds((p * NG + g) * LANES // 2, LANES // 2)))

        def out_copy(r0, n):
            return pltpu.make_async_copy(res.at[pl.ds(r0, n)], out_hbm.at[pl.ds(r0, n)], sem_out)

        def emit(r0, attended):
            n = attended.shape[0]
            c = {}
            for i in _ORDER:
                _scatter(c, _OUT[i], macc[i, pl.ds(pl.multiple_of(r0 // 2, PACK), n // 2), :])
            ffn = jnp.concatenate([
                jnp.concatenate([c[u, 0][r:r + PACK], c[u, 1][r:r + PACK]], axis=1)
                for r in range(0, n // 2, PACK) for u in range(2)], axis=0)
            rows = pl.ds(pl.multiple_of(r0, 2 * PACK), n)
            res[rows, :] = (xb[rows, :].astype(F32) + base[rows, :] + 0.5 * ffn + attended).astype(BF16)

        def emitting(r0):
            return _jobs(lambda r, gate: emit(r0 + r, gate(go[pl.ds(r, 2 * PACK), :])), range(0, PR, 2 * PACK))

        def quarter(a, halves):
            return pl.ds(a * HR + halves[0] * QR, len(halves) * QR)

        wo_copy(NF).wait()
        qkv_wait(NF)
        mem_copy.wait()
        with _scope("a_pro"):
            pacer = _Pacer(_never(xb))

            def clear(h, gate):
                ob[h] = z = gate(jnp.zeros((PR, DH), F32))
                if h < NCB:
                    go[:, pl.ds(h * LANES, LANES)] = z

            tokens = xn[pl.ds(0, PR), :].astype(F32)
            lhs = {p: _combine(_HK_LHS[p], lambda a, i: _lanes(tokens, i)[a * HR:(a + 1) * HR]).astype(BF16)
                   for p in _HK_ORDER}
            for w, g in itertools.product(range(3), range(NG)):
                c = {}
                for p in _HK_ORDER:
                    _scatter(c, _HK_OUT[p], pacer.dot(lhs[p], w_in(w, p, g)))
                for (a, j), v in c.items():
                    gq[w, g * NB + j, pl.ds(a * HR, HR), :] = v
                if (w, g) == (1, NG - 1):
                    pacer.run(qkv_jobs(NF))
            pacer.run(wo_jobs(NF), _jobs(clear, range(H)))

        def period(it, mem):
            done = pl.multiple_of(jnp.maximum(it - 2, 0) * PR, PR)
            tokens = xn[pl.ds(pl.multiple_of((it + 1) * PR, PR), PR), :].astype(F32)

            for step in range(PERIOD):
                mem = segment(step, tokens, mem, emitting(done) if step == 0 else [])

            @pl.when(it >= 2)
            def _():
                out_copy(done, PR).start()

            return mem

        def segment(step, tokens, mem, side):
            entries = _HK_STEPS[step]
            rows = pl.ds(step * SEG, SEG)
            begun = {
                k + (half,)
                for p, halves, _, _ in itertools.chain(*_HK_STEPS[:step])
                for half in halves for k, c in np.ndenumerate(_HK_OUT[p]) if c
            }

            def operand(entry, mem_block, token_block):
                p, halves, mem_lhs, _ = entry
                a = jnp.concatenate([
                    _combine(mem_lhs, mem_block),
                    _combine(_HK_LHS[p], lambda a, i: token_block(quarter(a, halves), i))], axis=0)
                return a if a.shape[0] % PACK else a.astype(BF16)

            def fold(entry, r, mem_acc, token_acc, partial):
                p, halves, _, mem_out = entry
                _scatter(mem_acc, mem_out, r[:M])
                for n, half in enumerate(halves):
                    _scatter(token_acc, _HK_OUT[p], r[M + n * QR:M + (n + 1) * QR], (half,),
                             lambda a, j, h: partial(quarter(a, (h,)), j) if (a, j, h) in begun else None)

            lhs = [
                operand(e, lambda i: _lanes(mem, i), lambda r, i: _lanes(tokens, i)[r.start:r.start + r.size])
                for e in entries
            ]
            qkv_mem, prob, att_mem, new_mem, out_acc = {}, {}, {}, {}, {}

            def project(g, w):
                mem_acc, token_acc = {}, {}

                if step == 0:
                    for h in range(g * NB, (g + 1) * NB):
                        fq[w, h] = gq[w, h]
                        if w == 0:
                            oc[h] = ob[h]

                def one(a, e):
                    fold(e, pacer.dot(a, w_in(w, e[0], g)), mem_acc, token_acc, lambda r, j: gq[w, g * NB + j, r, :])

                def finish():
                    pacer.run(_share(side, 3 * g + w, 3 * NG - 3) if g < NG - 1 else [])
                    for (a, j, half), v in token_acc.items():
                        gq[w, g * NB + j, quarter(a, (half,)), :] = v
                    for (j,), v in mem_acc.items():
                        qkv_mem[w, g * NB + j] = v

                return [functools.partial(one, a, e) for a, e in zip(lhs, entries)] + [finish]

            def part(w, h):
                return jnp.concatenate([qkv_mem[w, h], fq[w, h, rows, :]], axis=0)

            def scores(h):
                prob[h] = _softmax_rows(part(0, h), part(1, h), mask, scale)

            def attend(h):
                o = _dot(prob[h], part(2, h))
                att_mem[h] = o[:M]
                ob[h, rows, :] = o[M:]

            def outproj(g, e):
                a = operand(e, lambda i: att_mem[g * NB + i], lambda r, i: oc[g * NB + i, r, :])
                fold(e, _dot(a, _get(wo, (e[0], g))), new_mem, out_acc, lambda r, j: go[r, pl.ds(j * LANES, LANES)])

            def heads(fn, g):
                return _jobs(fn, range(g * NB, (g + 1) * NB))

            def play(*lists):
                for job in _mix(*lists):
                    job()

            todo = _jobs(outproj, range(NG), entries)
            early = len(todo) - len(entries) - sum(TAIL)
            at = 0
            for g in range(NG):
                play(project(g, 0))
                play(project(g, 1), heads(attend, g - 1) if g else [])
                values = project(g, 2)
                lead = len(values) // (4 if g == NG - 1 else 2)
                play(values[:lead])
                play(values[lead:lead + len(values) // 2], heads(scores, g))
                play(values[lead + len(values) // 2:])
                play(todo[at:min(early, g * len(entries))])
                at = min(early, g * len(entries))
            play(todo[at:at + TAIL[0]])
            play(todo[at + TAIL[0]:at + sum(TAIL)], heads(attend, NG - 1))
            play(todo[at + sum(TAIL):])
            for (a, j, half), v in out_acc.items():
                go[quarter(a, (half,)), pl.ds(j * LANES, LANES)] = v
            return jnp.concatenate([new_mem[j,] for j in range(NB)], axis=1)

        with _scope("a_loop"):
            mem = lax.fori_loop(0, NPER, period, mem0[...].astype(F32))

        with _scope("a_epi"):
            rows = pl.ds(0, SEG)
            ER = (PR + SEG) // 2
            lhs = [_combine(e[2], lambda i: _lanes(mem, i)) for e in _HK_STEPS[0]]
            kv_mem, prob, att, out_acc = {}, {}, {}, {}

            def project(w, g):
                acc = {}
                for a, (p, _, _, mem_out) in zip(lhs, _HK_STEPS[0]):
                    _scatter(acc, mem_out, pacer.dot(a, w_in(w, p, g)))
                for (j,), v in acc.items():
                    kv_mem[w, g * NB + j] = jnp.concatenate([v, gq[w, g * NB + j, rows, :]], axis=0)

            def block(a, h):
                if a == 0:
                    return ob[h, pl.ds(0, ER), :]
                return jnp.concatenate([ob[h, pl.ds(ER, PR - ER), :], att[h]], axis=0)

            for t in range(NG + 2):
                if t < NG:
                    project(1, t)
                    project(2, t)
                    for h in range(t * NB, (t + 1) * NB):
                        prob[h] = _softmax_rows(gq[0, h, rows, :], kv_mem[1, h], mask[M:], scale)
                if 0 <= t - 2:
                    for p in _HK_ORDER:
                        a = _combine(_HK_LHS[p], lambda a, i: block(a, (t - 2) * NB + i))
                        _scatter(out_acc, _HK_OUT[p], _dot(a, _get(wo, (p, t - 2))))
                if 0 <= t - 1 < NG:
                    for h in range((t - 1) * NB, t * NB):
                        att[h] = _dot(prob[h], kv_mem[2, h])
            pacer.run(emitting((NPER - 2) * PR))
            r0 = (NPER - 1) * PR
            for a in range(2):
                emit(r0 + a * ER, jnp.concatenate([out_acc[a, j] for j in range(NB)], axis=1))
            out_copy(r0 - PR, PR + 2 * ER).start()
        with _scope("tail"):
            out_copy(0, S).wait()

    if "1" in PARTS or "3" in PARTS:
        pl.run_scoped(
            mixer,
            _words(49, NCB // 4, S // 8),
            _words(2, 49, FC // 4 // LANES, HD // 4),
            pltpu.VMEM((2, D, FC), BF16),
            pltpu.VMEM((2, FC, D), BF16),
            pltpu.SemaphoreType.DMA((2, 2)),
        )
    if "A" not in PARTS:
        k = xb[0:8, 0:128].astype(jnp.int32)[0, 0]
        k16 = pl.ds(pl.multiple_of(k * 16, 16), 16)
        xb[0:16, 0:128] = (_get(wqkv, (k, pl.ds(0, 8))) + _get(wo, (k, k, pl.ds(0, 8)))
                           + xn[k16, 0:128] + macc[k, k16, 0:128].astype(BF16) + base[k16, 0:128].astype(BF16))
        pltpu.sync_copy(xb, out_hbm)
        return
    pl.run_scoped(
        recurrence,
        pltpu.VMEM((S, D), BF16),
        pltpu.VMEM((3, H, PERIOD * SEG, DH), F32),
        pltpu.VMEM((3, H, PERIOD * SEG, DH), F32),
        pltpu.VMEM((H, PERIOD * SEG, DH), F32),
        pltpu.VMEM((H, PERIOD * SEG, DH), F32),
        pltpu.VMEM((PERIOD * SEG, D), F32),
        pltpu.SemaphoreType.DMA(()),
    )


@functools.partial(jax.jit, static_argnames=("A_seg_len",))
def pallas_parallel_sum__memory_aug_recurrent_mem_tr__mixer_s_mlp__prompt_kernel(
    A_x: jax.Array,
    A_mem0: jax.Array,
    A_Wq: jax.Array,
    A_Wk: jax.Array,
    A_Wv: jax.Array,
    A_Wo: jax.Array,
    A_seg_len: int,
    B_x: jax.Array,
    B_w1: jax.Array,
    B_w2: jax.Array,
    B_w3: jax.Array,
    B_w4: jax.Array,
):
    del B_x
    B, S, D = A_x.shape
    _, H, DH = A_Wq.shape
    M = A_mem0.shape[1]
    F = B_w3.shape[1]
    SEG = int(A_seg_len)
    assert B == 1 and DH == LANES and D == NB * LANES

    hbm = pl.BlockSpec(memory_space=pl.ANY)
    out = pl.pallas_call(
        functools.partial(_kernel, S=S, D=D, H=H, DH=DH, M=M, SEG=SEG, F=F),
        out_shape=jax.ShapeDtypeStruct((S, D), A_x.dtype),
        in_specs=[hbm] * 10,
        out_specs=hbm,
        scratch_shapes=[
            pltpu.VMEM((S, D), BF16),
            pltpu.VMEM((S + (PERIOD - 1) * SEG, D), BF16),
            pltpu.VMEM((S, D), F32),
            pltpu.VMEM((7, S // 2, D // 2), F32),
            _words(3, NPROD * H // NB * LANES // 2),
            _words(NPROD, H // NB, LANES // 2),
            pltpu.VMEM((2, 3, NB, PACK * H, LANES), BF16),
            _words(3, NB, H // 2 * (PACK + 1)),
            pltpu.VMEM((2, H, PACK, D), BF16),
            pltpu.VMEM((M, D), BF16),
            pltpu.SemaphoreType.DMA(()),
            pltpu.SemaphoreType.DMA((2, 3)),
            pltpu.SemaphoreType.DMA((2,)),
        ],
        compiler_params=pltpu.CompilerParams(vmem_limit_bytes=127 * 1024 * 1024, flags=FLAGS, disable_bounds_checks=True),
    )(
        A_x.reshape(S, D),
        A_mem0.reshape(M, D),
        A_Wq.reshape(NB, LANES * H, DH),
        A_Wk.reshape(NB, LANES * H, DH),
        A_Wv.reshape(NB, LANES * H, DH),
        A_Wo,
        B_w1, B_w2, B_w3, B_w4,
    )
    return out.reshape(B, S, D)
```

```python
import functools
import itertools
import math

import jax
import jax.numpy as jnp
import numpy as np
from jax import lax
from jax.experimental import pallas as pl
from jax.experimental.pallas import tpu as pltpu

F32 = jnp.float32
BF16 = jnp.bfloat16
U32 = jnp.uint32
LANES = 128
SUB = 8
PACK = 16
EPS = 1e-5
R1 = 128
RU = 64
RD = 32
R3 = 256
FC = 512
PERIOD = 3
PREP_SHARE = (1, 5, 6, 6, 2)
TAIL = (44, 24)
LEAD = (2, 4)


def _layernorm_jobs(read, count, finish, slack):
    mean, var = {}, {}

    def first(k, gate):
        mean[k] = jnp.mean(read(0, k, gate), axis=-1, keepdims=True)

    def second(k, gate):
        d = read(1, k, gate) - mean[k]
        var[k] = jnp.mean(d * d, axis=-1, keepdims=True)

    def idle(gate):
        pass

    last = [finish(k, mean, var) for k in range(count)]
    n = len(last[0])
    return [
        _jobs(first, range(count)) + [idle] * (2 + slack),
        [idle] + _jobs(second, range(count)) + [idle] * (1 + slack),
        [idle] * 2 * n + list(itertools.chain(*last)) + [idle] * slack * n,
    ]


def _gate_first(gate, v):
    return jnp.concatenate([gate(v[:, :LANES]), v[:, LANES:]], axis=1)


def _gelu2(x):
    c = math.sqrt(2 / math.pi)
    return x + x * jnp.tanh(x * (c + (c * 0.044715) * (x * x)))


def _softmax_rows(q, k, mask, scale):
    z = lax.dot_general(q, k, (((1,), (1,)), ((), ())), preferred_element_type=F32)
    z = jnp.where(mask, z * scale, -1e9)
    e = jnp.exp(z - jnp.max(z, axis=-1, keepdims=True))
    s = jnp.sum(e, axis=-1, keepdims=True)
    r = pl.reciprocal(s, approx=True)
    return e * (r * (2.0 - s * r))


def _dot(a, b):
    return jnp.dot(a, b, preferred_element_type=F32)


def _put(ref, idx, v):
    ref[idx] = pltpu.bitcast(v.astype(BF16), U32)


def _get(ref, idx):
    return pltpu.bitcast(ref[idx], BF16)


def _get_wide(ref, i, rows=slice(None)):
    return jnp.concatenate([_get(ref, (i, c, rows)) for c in range(ref.shape[1])], axis=1)


def _words(*shape):
    return pltpu.VMEM(shape + (LANES,), U32)


def _lanes(v, c):
    return v[:, c * LANES:(c + 1) * LANES]


def _combine(coef, get):
    terms = sorted(((int(c), k) for k, c in np.ndenumerate(coef) if c), key=lambda t: -t[0])
    out = get(*terms[0][1]) if terms[0][0] > 0 else -get(*terms[0][1])
    for c, k in terms[1:]:
        out = out + get(*k) if c > 0 else out - get(*k)
    return out


def _scatter(acc, coef, v, tag=(), start=None):
    for k, c in np.ndenumerate(coef):
        if not c:
            continue
        k = k + tag
        if k not in acc and start is not None and (old := start(*k)) is not None:
            acc[k] = old
        if k in acc:
            acc[k] = acc[k] + v if c > 0 else acc[k] - v
        else:
            acc[k] = v if c > 0 else -v


_LHS = np.array([[1, 0, 0, 1], [0, 0, 1, 1], [1, 0, 0, 0], [0, 0, 0, 1],
                 [1, 1, 0, 0], [-1, 0, 1, 0], [0, 1, 0, -1]]).reshape(7, 2, 2)
_RHS = np.array([[1, 0, 0, 1], [1, 0, 0, 0], [0, 1, 0, -1], [-1, 0, 1, 0],
                 [0, 0, 0, 1], [1, 1, 0, 0], [0, 0, 1, 1]]).reshape(7, 2, 2)
_OUT = np.array([[1, 0, 0, 1], [0, 0, 1, -1], [0, 1, 0, 1], [1, 0, 1, 0],
                 [-1, 1, 0, 0], [0, 0, 0, 1], [1, 0, 0, 0]]).reshape(7, 2, 2)
_ORDER = (0, 3, 1, 2, 4, 5, 6)


def _hopcroft_kerr():
    n = 8
    method = (0, 1, 2, 0, 1, 2, 0, 1)
    stand_in = {(0, 3): (0, 2), (0, 6): (6, 2), (3, 6): (3, 2), (1, 4): (1, 5),
                (1, 7): (7, 5), (4, 7): (4, 5), (2, 5): (2, 7)}
    left_out = ("000010010001000022020010002002000200",
                "101101101210121210212121211211211011",
                "111111112122212101101202120120122122")
    forms = np.array([[[[1, 0], [1, 1]], [[-1, 1], [0, 1]]],
                      [[[0, 1], [1, 1]], [[1, -1], [1, 0]]],
                      [[[1, 0], [1, 0]], [[0, 1], [0, 1]]]])
    turn_a, turn_c = np.array([[0, -1], [1, 1]]), np.array([[1, -1], [1, 0]])
    eye = np.eye(n, dtype=int)
    lhs, out, groups, node, inner = [], [], [], {}, {}

    def product(a, c):
        lhs.append(a)
        out.append(c)
        groups[-1].append(len(lhs) - 1)
        return np.eye(100, dtype=int)[len(lhs) - 1]

    def add_node(key, a, c, m):
        groups.append([])
        node[key] = (a, c, m, [product(np.outer(f, a), np.outer(g, c)) for f, g in forms[m]])

    def pair(p, q):
        swap = (node[q][2] - node[p][2]) % 3 != 1
        (ai, ci, mi, di), (aj, cj, _, dj) = (node[q], node[p]) if swap else (node[p], node[q])
        sa, sc = (np.linalg.matrix_power(t, -mi % 3) for t in (turn_a, turn_c))
        add_node((p, q), ai + aj, ci - cj, (mi + 2) % 3)
        cross = product(np.outer(sa[:, 0], ai) + np.outer(sa[:, 1], aj),
                        np.outer(sc[:, 0], cj) + np.outer(sc[:, 1], ci))

        def turned(m, t, products):
            want = np.outer(sa @ forms[m, t, 0], sc @ forms[m, t, 1])
            return next(v for v, (f, g) in zip(products, forms[(m + mi) % 3]) if (np.outer(f, g) == want).all())

        dv = node[p, q][3]
        ij = cross - turned(2, 1, dv) - turned(1, 0, dj) + turned(0, 1, di)
        ji = cross + turned(2, 0, dv) - turned(0, 0, di) + turned(1, 1, dj)
        return (ji, ij) if swap else (ij, ji)

    for i in range(n):
        add_node(i, eye[i], eye[i], method[i])
        inner[i, i] = sum(node[i][3])
    for i, j in itertools.combinations(range(n), 2):
        if method[i] != method[j]:
            inner[i, j], inner[j, i] = pair(i, j)
    for (i, j), (u, k) in sorted(stand_in.items()):
        v, w = (min(u, k), max(u, k)), i + j - u
        vw, wv = pair(v, w)
        inner[u, w] = vw - inner[k, w]
        inner[w, u] = node[v][1][u] * wv + inner[w, k]
    lhs, out = np.array(lhs), np.array(out)
    rhs = np.array([[inner[i, j] for j in range(n)] for i in range(n)]).transpose(2, 0, 1)
    sign = np.where(rhs.max((1, 2)) > 0, 1, -1)[:, None, None]
    rhs, out = sign * rhs, sign * out
    assert (np.einsum("pri,pjk,psl->rijksl", lhs, rhs, out)
            == np.einsum("rs,ij,kl->rijksl", np.eye(2, dtype=int), eye, eye)).all()

    used = [sorted(p for g, d in zip(groups, text) for p in g if p != g[int(d)]) for text in left_out]
    steps = []
    for products in used:
        basis = rhs[products].reshape(n * n, n * n)
        dual = np.rint(np.linalg.inv(basis).T).astype(int)
        assert (basis.T @ dual == np.eye(n * n)).all()
        entries = []
        for p, u in zip(products, dual.reshape(-1, n, n)):
            i, j = np.argwhere(u)[0]
            mem_lhs, mem_out = u[:, j] * u[i, j], u[i]
            assert (np.outer(mem_lhs, mem_out) == u).all()
            entries.append((p, tuple(t for t in range(PERIOD) if p in used[t]), mem_lhs, mem_out))
        steps.append(entries)

    def locality(p):
        idx = np.nonzero(np.abs(out[p]).sum(0))[0]
        a, b = idx.min() // 2, idx.max() // 2
        return (a, -b if a % 2 else b, tuple(idx))

    steps = [sorted(e, key=lambda t: locality(t[0])) for e in steps]
    return lhs, rhs, out, steps, sorted(range(len(lhs)), key=locality)


_HK_LHS, _HK_RHS, _HK_OUT, _HK_STEPS, _HK_ORDER = _hopcroft_kerr()
NB, NPROD = _HK_RHS.shape[1], _HK_RHS.shape[0]


def _plan(takes, by_half=()):
    return [
        sorted(((p, (0, 1) if len(when) == 1 else (int(step != takes[when]),), a, c) for p, when, a, c in entries),
               key=lambda e: e[1] if step in by_half else ())
        for step, entries in enumerate(_HK_STEPS)
    ]


_DUE = (0, 1)
_PLAN_IN = _plan({(0, 1): 0, (0, 2): 2, (1, 2): 2})
_PLAN_OUT = _plan({(0, 1): 1, (0, 2): 2, (1, 2): 1}, by_half=(2,))


def _begun(plan, step):
    return {
        k + (h,)
        for h in range(2) for back in range(1, (step - _DUE[h] - 1) % PERIOD + 1)
        for p, halves, _, _ in plan[(step - back) % PERIOD] if h in halves
        for k, c in np.ndenumerate(_HK_OUT[p]) if c
    }


def _share(jobs, k, n):
    return jobs[len(jobs) * k // n:len(jobs) * (k + 1) // n]


def _mix(*lists):
    keyed = [((n + 0.5) / len(l), k, n) for k, l in enumerate(lists) for n in range(len(l))]
    return [lists[k][n] for _, k, n in sorted(keyed)]


def _jobs(fn, *ranges):
    return [functools.partial(fn, *k) for k in itertools.product(*ranges)]


def _run(jobs):
    for job in jobs:
        job(lambda v: v)


def _never(ref):
    return jnp.abs(ref[0:SUB, 0:LANES].astype(F32)) < 0.0


class _Pacer:
    def __init__(self, never):
        self.never = never
        self.tokens = []

    def dot(self, a, b):
        m = _dot(a, b)
        rounds = min(max(a.shape[1] * m.shape[1] // (4 * LANES * LANES), 1), m.shape[1] // LANES)
        self.tokens += [
            m[r:r + SUB, c:c + LANES]
            for c in range(0, m.shape[1], m.shape[1] // rounds) for r in range(0, m.shape[0], SUB)
        ]
        return m

    def run(self, *job_lists):
        tokens, self.tokens = self.tokens, []

        def gate(k, count, v):
            n = v.shape[0] // SUB
            rows = []
            for r in range(n):
                t = lax.bitcast_convert_type(tokens[len(tokens) * (k * n + r) // (count * n)], v.dtype)
                rows.append(jnp.concatenate([
                    jnp.where(self.never, t, v[r * SUB:(r + 1) * SUB, c:c + LANES])
                    for c in range(0, v.shape[1], LANES)], axis=1))
            return jnp.concatenate(rows, axis=0)

        for job in _mix(*[
            [functools.partial(job, functools.partial(gate, k, len(jobs))) for k, job in enumerate(jobs)]
            for jobs in job_lists
        ]):
            job()


def _rhs(w, i):
    n = w.shape[0] // 7
    return jnp.concatenate([_get_wide(w, n * i + k) for k in range(n)], axis=0)


def _strassen(block, w, pacer, side, start=None):
    c = {}
    for i in _ORDER:
        _scatter(c, _OUT[i], pacer.dot(_combine(_LHS[i], block).astype(BF16), _rhs(w, i)), start=start)
    pacer.run(*side)
    return c


def _rhs_jobs(dst, src, which=range(7), scale=None):
    kh, nh, rows = src.shape[0] // 2, src.shape[1] // 2, 64

    def job(c, k0, gate):
        @functools.cache
        def block(a, b):
            v = gate(src[pl.ds(a * kh + k0, rows), pl.ds(b * nh + c * LANES, LANES)].astype(F32))
            return v if scale is None else scale * v

        for i in which:
            k, r = divmod((i * kh + k0) // 2, dst.shape[2])
            _put(dst, (k, c, pl.ds(r, rows // 2)), _combine(_RHS[i], block))

    return _jobs(job, range(nh // LANES), range(0, kh, rows))


def _rhs2_jobs(dst, src):
    kq, nq = src.shape[0] // 4, src.shape[1] // 4

    @functools.cache
    def block(c, k0, a, b):
        return src[pl.ds(a * kq + k0, PACK), pl.ds(b * nq + c * LANES, LANES)].astype(F32)

    def job(c, k0, i, gate):
        outer = functools.cache(lambda a, b: gate(_combine(_RHS[i], lambda u, v: block(c, k0, 2 * u + a, 2 * v + b))))
        for j in range(7):
            _put(dst, (7 * i + j, c, pl.ds(k0 // 2, SUB)), _combine(_RHS[j], outer))

    return _jobs(job, range(nq // LANES), range(0, kq, PACK), range(7))


def _hk_jobs(block, store):
    def job(p, gate):
        first = tuple(np.argwhere(_HK_RHS[p])[0].tolist())
        store(p, _combine(_HK_RHS[p], lambda i, j: gate(block(i, j)) if (i, j) == first else block(i, j)))

    return _jobs(job, _HK_ORDER)


def _kernel(
    x_hbm, mem_hbm, wq_hbm, wk_hbm, wv_hbm, wo_hbm, w1_hbm, w2_hbm, w3_hbm, w4_hbm,
    out_hbm,
    xb, xn, base, macc, wqkv, wo, raw, mid, raw_o, mem0, sem_m, sem_a, sem_o,
    *, S, D, H, DH, M, SEG, F,
):
    HD = D // 2
    NCB = D // LANES
    NG = H // NB
    T1 = 2 * R1
    NT = S // T1
    NF = F // FC
    assert LANES // PACK == NF + 1

    mem_copy = pltpu.make_async_copy(mem_hbm, mem0, sem_m)

    def wo_copy(part):
        rows = pl.ds(pl.multiple_of(part * PACK, PACK), PACK)
        return pltpu.make_async_copy(wo_hbm.at[:, rows], raw_o.at[part % 2], sem_o.at[part % 2])

    def wo_jobs(part, g):
        dst = wo.at[:, g, pl.ds(pl.multiple_of(part * SUB, SUB), SUB)]
        src = raw_o.at[part % 2, pl.ds(g * NB, NB)]
        block = functools.cache(lambda i, j: src[i, :, pl.ds(j * LANES, LANES)].astype(F32))
        return _hk_jobs(block, lambda p, v: _put(dst, p, v))

    def qkv_unit(n, k):
        return divmod(3 * n + k, NF + 1)

    def qkv_fetch(n):
        for k in range(3):
            w, part = qkv_unit(n, k)
            rows = pl.ds(pl.multiple_of(part * PACK * H, PACK * H), PACK * H)
            for which, src in enumerate((wq_hbm, wk_hbm, wv_hbm)):
                @pl.when(w == which)
                def _():
                    pltpu.make_async_copy(src.at[:, rows], raw.at[n % 2, k], sem_a.at[n % 2, k]).start()

    def qkv_wait(n):
        for k in range(3):
            pltpu.make_async_copy(wq_hbm.at[:, pl.ds(0, PACK * H)], raw.at[n % 2, k], sem_a.at[n % 2, k]).wait()

    def regroup_jobs(n, k, half):
        src = raw.at[n % 2, k, :, pl.ds(pl.multiple_of(half * PACK, PACK), PACK * H - PACK)]

        def job(i, gate):
            rows = gate(jnp.concatenate(
                [pltpu.bitcast(src[i, pl.ds(d * H, PACK), :], U32) for d in range(PACK)], axis=0))
            for d in range(PACK):
                mid[k, half, i, pl.ds(d, SUB, stride=PACK + 1), :] = rows[d * SUB:(d + 1) * SUB]

        return _jobs(job, range(NB))

    def combine_jobs(n, k, g):
        w, part = qkv_unit(n, k)
        step = NG * LANES // 2
        dst = wqkv.at[w, pl.ds(pl.multiple_of(part * SUB + g * (LANES // 2), SUB), (NPROD - 1) * step + SUB)]
        src = mid.at[k, g // 2, :, pl.ds(g % 2 * (NB // 2 * (PACK + 1)), NB // 2 * (PACK + 1))]
        words = functools.cache(lambda i, pair: src[i, pl.ds(pair * (PACK + 1), PACK), :])
        block = functools.cache(lambda i, j: pltpu.bitcast(
            words(i, j // 2) & jnp.uint32(0xFFFF0000) if j % 2 else words(i, j // 2) << 16, F32))
        return _hk_jobs(block, lambda p, v: _put(dst, pl.ds(p * step, SUB), v))

    def qkv_jobs(n):
        units = list(itertools.product(range(3), range(NG // 2)))
        moves = [regroup_jobs(n, k, half) for k, half in units] + [[]]
        sums = [[]] + [combine_jobs(n, k, 2 * half) + combine_jobs(n, k, 2 * half + 1) for k, half in units]
        return [job for a, b in zip(moves, sums) for job in _mix(a, b)]

    def mixer(yc, w3c, r3, r4, sem_f):
        def w3_copy(f):
            cols = pl.ds(pl.multiple_of(f * FC, FC), FC)
            return pltpu.make_async_copy(w3_hbm.at[:, cols], r3.at[f % 2], sem_f.at[0, f % 2])

        def w4_copy(f):
            rows = pl.ds(pl.multiple_of(f * FC, FC), FC)
            return pltpu.make_async_copy(w4_hbm.at[rows], r4.at[f % 2], sem_f.at[1, f % 2])

        def w3_jobs(f):
            return _rhs2_jobs(w3c.at[f % 2], r3.at[f % 2])

        def token_mixing(r12, y0, c1, sem_x, sem_w):
            w1c, w2c = (wo.at[pl.ds(n * 7 * HD // LANES, 7 * HD // LANES)] for n in range(2))
            shifts = (-1, 1, -2, 2)
            HP = S + 2 * SUB

            def x_copy(t):
                rows = pl.ds(pl.multiple_of(t * T1, T1), T1)
                return pltpu.make_async_copy(x_hbm.at[rows], xb.at[rows], sem_x.at[t])

            def w1_copy(a, b):
                idx = (pl.ds(a * HD, HD), pl.ds(b * HD, HD))
                return pltpu.make_async_copy(w1_hbm.at[idx], r12.at[(0,) + idx], sem_w.at[2 * a + b])

            w2_copy = pltpu.make_async_copy(w2_hbm, r12.at[1], sem_w.at[4])

            def tile(ref, t, view=0):
                return ref.at[pl.ds(pl.multiple_of(t * T1 + view * zero, T1), T1)]

            def normalizing(t, slot):
                xs, xn_t, n = [tile(xb, t, v) for v in range(3)], tile(xn, t), 2 * PACK

                def finish(k, mean, var):
                    def job(c, gate):
                        rows, cols = pl.ds(k * n, n), pl.ds(c * HD // 2, HD // 2)
                        r = lax.rsqrt(var[k] + EPS)
                        v = (xs[2][rows, cols].astype(F32) - wide(gate, mean[k], HD // 2)) * r
                        xn_t[rows, cols] = v.astype(BF16)
                        y0[slot, rows, cols] = v * lax.rsqrt(var[k] * r * r + EPS)

                    return _jobs(job, range(4))

                return _layernorm_jobs(
                    lambda v, k, gate: _gate_first(gate, xs[v][pl.ds(k * n, n), :].astype(F32)), T1 // n, finish, 2)

            def wide(gate, column, width):
                v = gate(jnp.broadcast_to(column, (column.shape[0], LANES)))
                return jnp.concatenate([v] * (width // LANES), axis=1)

            def keep(dst, c):
                for (a, b), v in c.items():
                    dst[a, :, pl.ds(b * HD, HD)] = v

            def block1(slot):
                return lambda a, b: y0[slot, pl.ds(a * R1, R1), pl.ds(b * HD, HD)]

            def stage1(slot, *side):
                keep(c1, _strassen(block1(slot), w1c, pacer, side))

            def h_from(t):
                return wqkv.at[0, pl.ds(pl.multiple_of(t * T1, T1), (NCB - 1) * HP + T1 + 2 * SUB)]

            def activating(t):
                hb_t = h_from(t)

                def job(a, c, gate):
                    h = _gelu2(gate(c1[a, :, pl.ds(c * LANES, LANES)]))
                    hb_t[pl.ds(c * HP + SUB + a * R1, R1), :] = pltpu.bitcast(h, U32)

                return _jobs(job, range(2), range(NCB))

            def stage2(t, *side):
                hb_t, base_t, xn_t = h_from(t), tile(base, t), tile(xn, t)
                c = _strassen(lambda a, b: jnp.concatenate([
                    pltpu.bitcast(hb_t[pl.ds(c * HP + SUB + a * R1 + shifts[c * 4 // NCB], R1), :], F32)
                    for c in range(b * NCB // 2, (b + 1) * NCB // 2)], axis=1), w2c, pacer, side,
                    lambda a, b: xn_t[pl.ds(a * R1, R1), pl.ds(b * HD, HD)].astype(F32))
                for (a, b), v in c.items():
                    base_t[pl.ds(a * R1, R1), pl.ds(b * HD, HD)] = v

            def renormalizing(t, slack=0):
                starts = range(0, RU, PACK)
                xs = [tile(base, t, v) for v in range(3)]
                yc_t = yc.at[:, :, pl.ds(pl.multiple_of(t * (RU // 2), RU // 2), RU // 2)]

                def read(view, k, cols):
                    return jnp.concatenate([
                        xs[view][pl.ds(2 * (a * RU + starts[k]) + u * PACK, PACK), cols]
                        for u in range(2) for a in range(2)], axis=0)

                def finish(k, mean, var):
                    y = {}

                    def job(c, i, gate):
                        if i == 0:
                            m, r = wide(gate, mean[k], LANES), lax.rsqrt(var[k] + EPS)
                            for q in range(4):
                                y[c, q] = (read(2, k, pl.ds(q * HD // 2 + c * LANES, LANES)) - m) * r
                        outer = functools.cache(lambda a, b: gate(_combine(
                            _LHS[i], lambda u, v: y[c, 2 * v + b][(2 * u + a) * PACK:(2 * u + a + 1) * PACK])))
                        for j in range(7):
                            _put(yc_t, (7 * i + j, c, pl.ds(starts[k] // 2, SUB)), _combine(_LHS[j], outer))

                    return _jobs(job, range(NCB // 4), range(7))

                return _layernorm_jobs(
                    lambda v, k, gate: _gate_first(gate, read(v, k, slice(None))), len(starts), finish, slack)

            arrival = (((0, 0), (1,)), ((1, 1), (4, 0)), ((0, 1), (2, 5)), ((1, 0), (3, 6)))
            quarters = [w1_copy(*q) for q, _ in arrival]
            queue = [
                [x_copy(0), quarters[0]], [], [], [quarters[1]], [quarters[2]], [x_copy(1)],
                [quarters[3], x_copy(2)], [w2_copy], [], [x_copy(3), w3_copy(0)],
            ]

            def launch():
                for cp in queue.pop(0):
                    cp.start()

            launch()
            for c in range(NCB):
                wqkv[0, pl.ds(c * HP, SUB), :] = jnp.zeros((SUB, LANES), U32)
                wqkv[0, pl.ds(c * HP + SUB + S, SUB), :] = jnp.zeros((SUB, LANES), U32)

            def clearing(t):
                acc_t = macc.at[:, pl.ds(pl.multiple_of(t * R1, R1), R1)]

                def job(i, lo, gate):
                    acc_t[i, pl.ds(lo, PACK), :] = wide(gate, jnp.zeros((PACK, 1), F32), HD)

                return _jobs(job, range(7), range(0, R1, PACK))

            for t in range(3):
                _run(clearing(t))
                launch()
            pad = xn.shape[0] - S
            xn[pl.ds(S, pad), :] = jnp.zeros((pad, D), BF16)
            x_copy(0).wait()
            launch()
            pacer = _Pacer(_never(xb))
            zero = 0
            _run(itertools.chain(*normalizing(0, 1)))
            zero = jnp.max(pacer.never.astype(jnp.int32))
            c = {}
            for n, (q, ready) in enumerate(arrival):
                w1_copy(*q).wait()
                if n == 2:
                    x_copy(1).wait()
                    *stats, ahead = normalizing(1, 0)
                    ahead = ahead[8:]
                launch()
                _run(_rhs_jobs(w1c, r12.at[0], ready))
                for i in ready:
                    _scatter(c, _OUT[i], pacer.dot(_combine(_LHS[i], block1(1)).astype(BF16), _rhs(w1c, i)))
                pacer.run(*(stats if n == 2 else [ahead] if n == 3 else []))
            keep(c1, c)
            launch()
            x_copy(2).wait()
            stage1(0, activating(0), *normalizing(2, 1))
            w2_copy.wait()
            stage1(1, activating(1), _rhs_jobs(w2c, r12.at[1], scale=0.5))
            x_copy(4).start()
            mem_copy.start()
            x_copy(3).wait()
            w3_copy(0).wait()
            w3j = w3_jobs(0)
            stage2(0, w3j[:len(w3j) * 3 // 4], *normalizing(3, 0))

            def slot(u, carry):
                @pl.when(u + 1 < NT)
                def _():
                    x_copy(u + 1).wait()

                @pl.when(u + 2 < NT)
                def _():
                    x_copy(u + 2).start()

                @pl.when(u == 4)
                def _():
                    w3_copy(1).start()

                @pl.when(u == 5)
                def _():
                    w4_copy(0).start()
                    wo_copy(0).start()

                @pl.when(u == 6)
                def _():
                    qkv_fetch(0)

                stage1(0, activating(u - 1) + [lambda gate: None] * 4, *renormalizing(u - 3))
                stage2(u - 2, clearing(u), *normalizing(jnp.minimum(u + 1, NT - 1), 0))
                return carry

            lax.fori_loop(3, NT, slot, 0)
            last = activating(NT - 1)
            halo = [c for c in range(NCB) if shifts[c * 4 // NCB] > 0]
            _run([last[c] for c in halo])
            stage2(NT - 2, [job for c, job in enumerate(last) if c not in halo], *renormalizing(NT - 3, 1))
            stage2(NT - 1, w3j[len(w3j) * 3 // 4:], *renormalizing(NT - 2, 1))
            _run(itertools.chain(*renormalizing(NT - 1)))

        def ffn(w4c, *g):
            assert S // 2 == 4 * R3
            never = _never(xb)

            def chunk(f, carry):
                @pl.when(f + 2 < NF)
                def _():
                    w3_copy(f + 2).start()

                @pl.when(f + 1 < NF)
                def _():
                    w4_copy(f + 1).start()
                    w3_copy(f + 1).wait()

                wo_copy(f + 1).start()
                qkv_fetch(f + 1)
                qkv_wait(f)
                w4_copy(f).wait()
                wo_copy(f).wait()
                pacer = _Pacer(never)
                w3f = w3c.at[f % 2]
                pre = {}

                def up(t, *side):
                    for s in range(t * R3 // (2 * RU), (t + 1) * R3 // (2 * RU)):
                        c = pre[s] = {}
                        for i in _ORDER:
                            inner = {}
                            for j in _ORDER:
                                a = _get_wide(yc, 7 * i + j, pl.ds(s * RU // 2, RU // 2))
                                _scatter(inner, _OUT[j], pacer.dot(a, _get_wide(w3f, 7 * i + j)))
                            for q, v in inner.items():
                                _scatter(c, _OUT[i], v, q)
                    pacer.run(*side)

                def activating(t):
                    def job(k, a, lo, gate):
                        for u, v, b in itertools.product(range(2), repeat=3):
                            g[t % 2][u, pl.ds((2 * k + a) * RU + lo, RD), pl.ds((2 * v + b) * FC // 4, FC // 4)] = (
                                _gelu2(gate(pre[t * R3 // (2 * RU) + k][u, v, a, b][lo:lo + RD])))

                    return _jobs(job, range(R3 // (2 * RU)), range(2), range(0, RU, RD))

                def down(t, *side):
                    for s in range(R3 // (2 * RD)):
                        for i in _ORDER:
                            outer = functools.cache(lambda a, b: _combine(_LHS[i], lambda u, v: g[t % 2][
                                u, pl.ds((2 * s + a) * RD, RD), pl.ds((2 * v + b) * FC // 4, FC // 4)]))
                            where = {
                                (a, b): (i, pl.ds(t * R3 + (2 * s + a) * RD, RD), pl.ds(b * HD // 2, HD // 2))
                                for a in range(2) for b in range(2)
                            }
                            acc = {k: macc[idx] for k, idx in where.items()}
                            for j in _ORDER:
                                a = _combine(_LHS[j], outer).astype(BF16)
                                _scatter(acc, _OUT[j], pacer.dot(a, _get_wide(w4c, 7 * i + j)))
                            for k, idx in where.items():
                                macc[idx] = acc[k]
                    pacer.run(*side)

                side = [qkv_jobs(f), [job for k in range(NG) for job in wo_jobs(f, k)]]
                w3j = w3_jobs(f + 1)
                total = sum(PREP_SHARE)

                def prep(k):
                    lo, hi = sum(PREP_SHARE[:k]), sum(PREP_SHARE[:k + 1])
                    return [l[len(l) * lo // total:len(l) * hi // total] for l in side]

                up(0, _rhs2_jobs(w4c, r4.at[f % 2]), *prep(0))
                up(1, activating(0), *prep(1))
                down(0, _share(w3j, 0, 3))
                up(2, activating(1), *prep(2))
                down(1, _share(w3j, 1, 3))
                up(3, activating(2), *prep(3))
                down(2, activating(3), *prep(4))
                down(3, _share(w3j, 2, 3))
                return carry

            lax.fori_loop(0, NF, chunk, 0)

        pl.run_scoped(
            token_mixing,
            pltpu.VMEM((2, D, D), BF16),
            pltpu.VMEM((2, T1, D), F32),
            pltpu.VMEM((2, R1, D), F32),
            pltpu.SemaphoreType.DMA((NT,)),
            pltpu.SemaphoreType.DMA((5,)),
        )
        pl.run_scoped(
            ffn,
            _words(49, NCB // 4, FC // 8),
            pltpu.VMEM((2, R3, FC), F32),
            pltpu.VMEM((2, R3, FC), F32),
        )

    def recurrence(res, partial, qkv, fresh, att, out_partial, out, sem_out):
        L = M + SEG
        PR = PERIOD * SEG
        QR = PR // 4
        NPER = (S // SEG - 1) // PERIOD
        assert NPER * PR + SEG == S
        scale = DH ** -0.5
        row = lax.broadcasted_iota(jnp.int32, (L, L), 0)
        col = lax.broadcasted_iota(jnp.int32, (L, L), 1)
        mask = (row < M) | (row >= col)

        def w_in(w, p, g):
            return _get(wqkv, (w, pl.ds(pl.multiple_of((p * NG + g) * (LANES // 2), LANES // 2), LANES // 2)))

        def out_copy(r0, n):
            return pltpu.make_async_copy(res.at[pl.ds(r0, n)], out_hbm.at[pl.ds(r0, n)], sem_out)

        def emit(r0, attended):
            c = {}
            for i in _ORDER:
                _scatter(c, _OUT[i], macc[i, pl.ds(pl.multiple_of(r0 // 2, PACK), PACK), :])
            ffn = jnp.concatenate([jnp.concatenate([c[u, 0], c[u, 1]], axis=1) for u in range(2)], axis=0)
            rows = pl.ds(pl.multiple_of(r0, 2 * PACK), 2 * PACK)
            res[rows, :] = (xb[rows, :].astype(F32) + base[rows, :] + 0.5 * ffn + attended).astype(BF16)

        def quarter(a, half):
            return slice((2 * half + a) * QR, (2 * half + a + 1) * QR)

        def tokens(it):
            return xn[pl.ds(pl.multiple_of(it * PR, PR), PR), :].astype(F32)

        def operand(entry, lead, token_block):
            p, halves, lead_lhs, _ = entry
            a = jnp.concatenate(([_combine(lead_lhs, lead)] if lead else []) + [
                _combine(_HK_LHS[p], lambda a, i: token_block(h, quarter(a, h), i)) for h in halves], axis=0)
            return a if a.shape[0] % PACK else a.astype(BF16)

        def fold(entry, r, lead_acc, token_acc, begun, old):
            p, halves, _, lead_out = entry
            n = r.shape[0] - len(halves) * QR
            if n:
                _scatter(lead_acc, lead_out, r[:n])
            for k, h in enumerate(halves):
                _scatter(token_acc, _HK_OUT[p], r[n + k * QR:n + (k + 1) * QR], (h,),
                         lambda a, j, h: old(quarter(a, h), j) if (a, j, h) in begun else None)

        def settle(acc, begun, step, old, keep, final):
            for a, j, h in sorted(begun | set(acc)):
                if step == _DUE[h]:
                    final(quarter(a, h), j, acc[a, j, h] if (a, j, h) in acc else old(quarter(a, h), j))
                elif (a, j, h) in acc:
                    keep(quarter(a, h), j, acc[a, j, h])

        def projecting(step, w, g, entries, lhs, mem_out):
            begun, mem_acc, token_acc = _begun(_PLAN_IN, step), {}, {}

            def old(r, j):
                return partial[w, g * NB + j, r, :]

            def one(a, e):
                fold(e, pacer.dot(a, w_in(w, e[0], g)), mem_acc, token_acc, begun, old)

            def finish():
                def keep(r, j, v):
                    partial[w, g * NB + j, r, :] = v

                def final(r, j, v):
                    now = min(max((step + 1) * SEG - r.start, 0), QR)
                    for k in range(0, now, SUB):
                        mem_out[w, g * NB + j, r.start + k] = v[k:k + SUB]
                    if now < QR:
                        qkv[w, g * NB + j, r.start + now:r.stop, :] = v[now:]

                settle(token_acc, begun, step, old, keep, final)
                for (j,), v in mem_acc.items():
                    mem_out[w, g * NB + j] = v

            return [functools.partial(one, a, e) for a, e in zip(lhs, entries)] + [finish]

        def segment_rows(step, found, w, h):
            return jnp.concatenate([
                found[w, h, r] if (w, h, r) in found else qkv[w, h, r:r + SUB, :]
                for r in range(step * SEG, (step + 1) * SEG, SUB)], axis=0)

        def out_old(r, j):
            return out_partial[r, pl.ds(j * LANES, LANES)]

        def out_store(ref, r, j, v):
            ref[r, pl.ds(j * LANES, LANES)] = v

        def only(entries, keep):
            return [(p, h, a, c) for p, halves, a, c in entries if (h := tuple(k for k in halves if k in keep))]

        def play(*lists):
            for job in _mix(*lists):
                job()

        wo_copy(NF).wait()
        qkv_wait(NF)
        mem_copy.wait()
        pacer = _Pacer(_never(xb))

        out_partial[...] = jnp.zeros(out_partial.shape, F32)
        entries = sorted(only(_PLAN_IN[1], (0,)) + _PLAN_IN[2], key=lambda e: e[1])

        def head_group(g, carry):
            first = tokens(0)
            lhs = [operand(e, None, lambda h, r, i: _lanes(first, i)[r]) for e in entries]
            att_g, partial_g = att.at[pl.ds(g * NB, NB)], partial.at[:, pl.ds(g * NB, NB)]

            def clear(h, gate):
                att_g[h] = gate(jnp.zeros((PR, DH), F32))

            values = [job for k in range(3) for job in regroup_jobs(NF, k, g // 2) + combine_jobs(NF, k, g)]
            side = ([_share(values, 0, 2)], [_share(values, 1, 2)], [wo_jobs(NF, g), _jobs(clear, range(NB))])
            for w in range(3):
                acc = {}
                for a, e in zip(lhs, entries):
                    fold(e, pacer.dot(a, w_in(w, e[0], g)), None, acc, (), None)
                for (a, j, h), v in acc.items():
                    partial_g[w, j, quarter(a, h), :] = v
                pacer.run(*side[w])
            return carry

        lax.fori_loop(0, NG, head_group, 0)

        def period(it, mem):
            done = pl.multiple_of(jnp.maximum(it - 1, 0) * PR, PR)
            this, following = tokens(it), tokens(it + 1)
            finished = _jobs(lambda r, gate: emit(done + r, gate(out[pl.ds(r, 2 * PACK), :])), range(0, PR, 2 * PACK))
            for step in range(PERIOD):
                mem = segment(step, this, following, mem, finished if step == PERIOD - 1 else [])

            @pl.when(it >= 1)
            def _():
                out_copy(done, PR).start()

            return mem

        def segment(step, this, following, mem, side):
            lhs = [
                operand(e, lambda i: _lanes(mem, i),
                        lambda h, r, i: _lanes(this if step <= _DUE[h] else following, i)[r])
                for e in _PLAN_IN[step]
            ]
            qkv_mem, prob, att_mem, new_mem, out_acc = {}, {}, {}, {}, {}
            begun = _begun(_PLAN_OUT, step)

            def part(w, h):
                return jnp.concatenate([qkv_mem[w, h], segment_rows(step, qkv_mem, w, h)], axis=0)

            def scores(h):
                prob[h] = _softmax_rows(part(0, h), part(1, h), mask, scale)

            def attend(h):
                o = _dot(prob[h], part(2, h))
                att_mem[h] = o[:M]
                lo, hi = hold(step - 1)
                if hi > lo:
                    att[h, lo:hi, :] = fresh[h, lo:hi, :]
                lo, hi = hold(step)
                if lo > step * SEG:
                    att[h, step * SEG:lo, :] = o[M:M + lo - step * SEG]
                if hi > lo:
                    fresh[h, lo:hi, :] = o[M + lo - step * SEG:]

            def hold(k):
                if k not in _DUE:
                    return (k + 1) * SEG, (k + 1) * SEG
                return max(k * SEG, _DUE.index(k) * 2 * QR), (k + 1) * SEG

            def outproj(g, e):
                a = operand(e, lambda i: att_mem[g * NB + i], lambda h, r, i: att[g * NB + i, r, :])
                fold(e, _dot(a, _get(wo, (e[0], g))), new_mem, out_acc, begun, out_old)

            def heads(fn, g):
                return _jobs(fn, range(g * NB, (g + 1) * NB))

            def project(g, w):
                return projecting(step, w, g, _PLAN_IN[step], lhs, qkv_mem)

            todo = _jobs(outproj, range(NG), _PLAN_OUT[step])
            early = len(todo) - NB * NB - sum(TAIL)
            at = 0
            for g in range(NG):
                play(project(g, 0))
                play(project(g, 1), heads(attend, g - 1) if g else [])
                values = project(g, 2)
                lead = len(values) // LEAD[g == NG - 1]
                pacer.run(_share(side, g, NG - 1) if g < NG - 1 else [])
                play(values[:lead])
                play(values[lead:lead + len(values) // 2], heads(scores, g))
                play(values[lead + len(values) // 2:])
                play(todo[at:min(early, g * NB * NB)])
                at = min(early, g * NB * NB)
            play(todo[at:at + TAIL[0]])
            play(todo[at + TAIL[0]:at + sum(TAIL)], heads(attend, NG - 1))
            play(todo[at + sum(TAIL):])
            settle(out_acc, begun, step, out_old,
                   functools.partial(out_store, out_partial), functools.partial(out_store, out))
            pacer.run()
            return jnp.concatenate([new_mem[j,] for j in range(NB)], axis=1)

        mem = lax.fori_loop(0, NPER, period, mem0[...].astype(F32))

        last = tokens(NPER)
        entries = [(p, tuple(k for k in halves if k == 0), a, c) for p, halves, a, c in _PLAN_IN[0]]
        lhs = [operand(e, lambda i: _lanes(mem, i), lambda h, r, i: _lanes(last, i)[r]) for e in entries]
        qkv_mem, prob, new, own, out_acc = {}, {}, {}, {}, {}
        begun = _begun(_PLAN_OUT, 0)

        def part(w, h):
            return jnp.concatenate([qkv_mem[w, h], segment_rows(0, qkv_mem, w, h)], axis=0)

        for t in range(NG + 2):
            if t < NG:
                for w in range(3):
                    play(projecting(0, w, t, entries, lhs, qkv_mem))
                for h in range(t * NB, (t + 1) * NB):
                    prob[h] = _softmax_rows(segment_rows(0, qkv_mem, 0, h), part(1, h), mask[M:], scale)
            if 0 <= t - 2:
                for lead, todo in ((None, only(_PLAN_OUT[1], (1,))), (lambda i: new[(t - 2) * NB + i], _PLAN_OUT[0])):
                    for e in todo:
                        a = operand(e, lead, lambda h, r, i: att[(t - 2) * NB + i, r, :])
                        fold(e, _dot(a, _get(wo, (e[0], t - 2))), own, out_acc, begun, out_old)
            if 0 <= t - 1 < NG:
                for h in range((t - 1) * NB, t * NB):
                    new[h] = _dot(prob[h], part(2, h))
        total = jnp.concatenate([
            jnp.concatenate([
                out_acc[a, j, h] if (a, j, h) in out_acc else out_old(quarter(a, h), j)
                for h in range(2) for a in range(2)] + [own[j,]], axis=0)
            for j in range(NB)], axis=1)
        r0 = (NPER - 1) * PR
        for r in range(0, PR + SEG, 2 * PACK):
            emit(r0 + r, total[r:r + 2 * PACK])
        out_copy(r0, PR + SEG).start()
        out_copy(0, S).wait()

    pl.run_scoped(
        mixer,
        _words(49, NCB // 4, S // 8),
        _words(2, 49, FC // 4 // LANES, HD // 4),
        pltpu.VMEM((2, D, FC), BF16),
        pltpu.VMEM((2, FC, D), BF16),
        pltpu.SemaphoreType.DMA((2, 2)),
    )
    pl.run_scoped(
        recurrence,
        pltpu.VMEM((S, D), BF16),
        pltpu.VMEM((3, H, PERIOD * SEG, DH), F32),
        pltpu.VMEM((3, H, PERIOD * SEG, DH), F32),
        pltpu.VMEM((H, PERIOD * SEG, DH), F32),
        pltpu.VMEM((H, PERIOD * SEG, DH), F32),
        pltpu.VMEM((PERIOD * SEG, D), F32),
        pltpu.VMEM((PERIOD * SEG, D), F32),
        pltpu.SemaphoreType.DMA(()),
    )


@functools.partial(jax.jit, static_argnames=("A_seg_len",))
def pallas_parallel_sum__memory_aug_recurrent_mem_tr__mixer_s_mlp__prompt_kernel(
    A_x: jax.Array,
    A_mem0: jax.Array,
    A_Wq: jax.Array,
    A_Wk: jax.Array,
    A_Wv: jax.Array,
    A_Wo: jax.Array,
    A_seg_len: int,
    B_x: jax.Array,
    B_w1: jax.Array,
    B_w2: jax.Array,
    B_w3: jax.Array,
    B_w4: jax.Array,
):
    del B_x
    B, S, D = A_x.shape
    _, H, DH = A_Wq.shape
    M = A_mem0.shape[1]
    F = B_w3.shape[1]
    SEG = int(A_seg_len)
    assert B == 1 and DH == LANES and D == NB * LANES

    hbm = pl.BlockSpec(memory_space=pl.ANY)
    out = pl.pallas_call(
        functools.partial(_kernel, S=S, D=D, H=H, DH=DH, M=M, SEG=SEG, F=F),
        out_shape=jax.ShapeDtypeStruct((S, D), A_x.dtype),
        in_specs=[hbm] * 10,
        out_specs=hbm,
        scratch_shapes=[
            pltpu.VMEM((S, D), BF16),
            pltpu.VMEM((S + (PERIOD - 1) * SEG, D), BF16),
            pltpu.VMEM((S, D), F32),
            pltpu.VMEM((7, S // 2, D // 2), F32),
            _words(3, NPROD * H // NB * LANES // 2),
            _words(NPROD, H // NB, LANES // 2),
            pltpu.VMEM((2, 3, NB, PACK * H, LANES), BF16),
            _words(3, H // PACK, NB, SUB * (PACK + 1)),
            pltpu.VMEM((2, H, PACK, D), BF16),
            pltpu.VMEM((M, D), BF16),
            pltpu.SemaphoreType.DMA(()),
            pltpu.SemaphoreType.DMA((2, 3)),
            pltpu.SemaphoreType.DMA((2,)),
        ],
        compiler_params=pltpu.CompilerParams(
            vmem_limit_bytes=127 * 1024 * 1024,
            disable_bounds_checks=True,
            flags={"XLA_TPU_EVENLY_DISTRIBUTE_CRITICAL_NODES": True},
        ),
    )(
        A_x.reshape(S, D),
        A_mem0.reshape(M, D),
        A_Wq.reshape(NB, LANES * H, DH),
        A_Wk.reshape(NB, LANES * H, DH),
        A_Wv.reshape(NB, LANES * H, DH),
        A_Wo,
        B_w1, B_w2, B_w3, B_w4,
    )
    return out.reshape(B, S, D)
```
